```python
import jax
import jax.numpy as jnp

def _softmax(x, axis=-1):
    return jax.nn.softmax(x, axis=axis)

def _gelu(x):
    return jax.nn.gelu(x, approximate=True)

def _silu(x):
    return jax.nn.silu(x)

def _sigmoid(x):
    return jax.nn.sigmoid(x)

def _layernorm(x, axis=-1, eps=1e-05):
    m = jnp.mean(x, axis=axis, keepdims=True)
    v = jnp.var(x, axis=axis, keepdims=True)
    return (x - m) / jnp.sqrt(v + eps)

def _scatter_add(tgt, idx, src, axis=0):
    return tgt.at[idx].add(src)

def _segment_sum(src, seg, n):
    return jax.ops.segment_sum(src, seg, n)

class _Rng:

    def __init__(self, key):
        self._k = key

    def _next(self):
        self._k, sub = jax.random.split(self._k)
        return sub

    def normal(self, shape):
        return jax.random.normal(self._next(), shape, dtype=jnp.bfloat16)

    def randint(self, lo, hi, shape):
        return jax.random.randint(self._next(), shape, lo, hi, dtype=jnp.int32)

    def uniform(self, shape, lo=0.0, hi=1.0):
        return jax.random.uniform(self._next(), shape, jnp.bfloat16, lo, hi)

    def permutation(self, n):
        return jax.random.permutation(self._next(), n)
kernel_name = 'sequential_preLN__memory_aug_recurrent_mem_tr__mixer_s_mlp__prompt'

def setup_inputs():
    _rng = _Rng(jax.random.key(int.from_bytes(__import__("os").urandom(4), "little")))
    _w = lambda a: (lambda t: t.astype(jnp.bfloat16) if jnp.issubdtype(t.dtype, jnp.floating) else t)(jnp.asarray(a))

    def _A_setup():
        B, S, Dm = (1, 2048, 1024)
        H, Dh = (32, 128)
        M, seg = (8, 32)
        seg = min(seg, S)
        S = S // seg * seg
        return {'x': _w((lambda *s: _rng.normal(s) * 0.05)(B, S, Dm)), 'mem0': _w((lambda *s: _rng.normal(s) * 0.05)(B, M, Dm)), 'Wq': _w((lambda *s: _rng.normal(s) * 0.05)(Dm, H, Dh) * Dm ** (-0.5)), 'Wk': _w((lambda *s: _rng.normal(s) * 0.05)(Dm, H, Dh) * Dm ** (-0.5)), 'Wv': _w((lambda *s: _rng.normal(s) * 0.05)(Dm, H, Dh) * Dm ** (-0.5)), 'Wo': _w((lambda *s: _rng.normal(s) * 0.05)(H, Dh, Dm) * (H * Dh) ** (-0.5)), 'seg_len': seg}
    _A_in = _A_setup()

    def _B_setup():
        B, S, D, F = (1, 2048, 1024, 3584)
        return {'x': _w((lambda *s: _rng.normal(s) * 0.05)(B, S, D)), 'w1': _w((lambda *s: _rng.normal(s) * 0.05)(D, D) * D ** (-0.5)), 'w2': _w((lambda *s: _rng.normal(s) * 0.05)(D, D) * D ** (-0.5)), 'w3': _w((lambda *s: _rng.normal(s) * 0.05)(D, F) * D ** (-0.5)), 'w4': _w((lambda *s: _rng.normal(s) * 0.05)(F, D) * F ** (-0.5))}
    _B_in = _B_setup()
    return {'A_x': _A_in['x'], 'A_mem0': _A_in['mem0'], 'A_Wq': _A_in['Wq'], 'A_Wk': _A_in['Wk'], 'A_Wv': _A_in['Wv'], 'A_Wo': _A_in['Wo'], 'A_seg_len': _A_in['seg_len'], 'B_x': _B_in['x'], 'B_w1': _B_in['w1'], 'B_w2': _B_in['w2'], 'B_w3': _B_in['w3'], 'B_w4': _B_in['w4']}

def reference(A_x, A_mem0, A_Wq, A_Wk, A_Wv, A_Wo, A_seg_len, B_x, B_w1, B_w2, B_w3, B_w4):

    def _A_ref(x, mem0, Wq, Wk, Wv, Wo, seg_len):
        B, S, Dm = x.shape
        H, Dh = (Wq.shape[1], Wq.shape[2])
        M = mem0.shape[1]
        scale = Dh ** (-0.5)
        n_seg = S // seg_len
        L = M + seg_len
        idx = jnp.arange(L)
        mask = (idx[:, None] < M) | (idx[:, None] >= idx[None, :])
        mem = mem0
        outs = []
        for s in range(n_seg):
            xs = x[:, s * seg_len:(s + 1) * seg_len, :].copy()
            h = jnp.concatenate([mem, xs], axis=1)
            q = jnp.einsum('btd,dhe->bhte', h, Wq)
            k = jnp.einsum('btd,dhe->bhte', h, Wk)
            v = jnp.einsum('btd,dhe->bhte', h, Wv)
            scores = jnp.einsum('bhqe,bhke->bhqk', q, k) * scale
            scores = jnp.where(mask[None, None], scores, -1000000000.0)
            p = _softmax(scores, axis=-1)
            o = jnp.einsum('bhqk,bhke->bhqe', p, v)
            o = jnp.einsum('bhte,hed->btd', o, Wo)
            mem = o[:, :M, :].copy()
            outs.append(o[:, M:, :])
        return jnp.concatenate(outs, axis=1)

    def _B_ref(x, w1, w2, w3, w4):
        B, S, D = x.shape
        h = _gelu(_layernorm(x, axis=-1) @ w1)
        c = D // 4
        g0 = jnp.pad(h[:, :, 0 * c:1 * c], ((0, 0), (1, 0), (0, 0)))[:, :S, :]
        g1 = jnp.pad(h[:, :, 1 * c:2 * c], ((0, 0), (0, 1), (0, 0)))[:, 1:, :]
        g2 = jnp.pad(h[:, :, 2 * c:3 * c], ((0, 0), (2, 0), (0, 0)))[:, :S, :]
        g3 = jnp.pad(h[:, :, 3 * c:], ((0, 0), (0, 2), (0, 0)))[:, 2:, :]
        hs = jnp.concatenate([g0, g1, g2, g3], axis=-1) @ w2
        x1 = x + hs
        h2 = _gelu(_layernorm(x1, axis=-1) @ w3) @ w4
        return x1 + h2
    x = A_x
    h = x + _A_ref(_layernorm(x, axis=-1), A_mem0, A_Wq, A_Wk, A_Wv, A_Wo, A_seg_len)
    h2 = h + _B_ref(_layernorm(h, axis=-1), B_w1, B_w2, B_w3, B_w4)
    return h2
```

```python
import functools

import jax
import jax.numpy as jnp
import jax.experimental.pallas as pl
import jax.experimental.pallas.tpu as pltpu

F32 = jnp.float32
BF16 = jnp.bfloat16
U32 = jnp.uint32

S = 2048
D = 1024
H = 32
E = 128
M = 8
SEG = 32
NSEG = S // SEG
FF = 3584
TPS = 24
P0 = S - TPS * (NSEG - 1)
PPAD = 544
RING = 576
OTAIL = TPS * (NSEG - 1)
CH = 256
EPS = 1e-5
NEG = -1000000000.0


def _ln(x):
    m = jnp.mean(x, axis=-1, keepdims=True)
    xc = x - m
    v = jnp.mean(xc * xc, axis=-1, keepdims=True)
    return xc * jax.lax.rsqrt(v + EPS)


def _gelu(x):
    return jax.nn.gelu(x, approximate=True)


def _dot(a, b):
    return jnp.dot(a, b, preferred_element_type=F32)


def _w(u32_val):
    return pltpu.bitcast(u32_val, BF16)


def _kernel(x_hbm, mem0_ref, wq_hbm, wk_hbm, wv_hbm, wo_hbm, w1_hbm, w2_hbm,
            w3_hbm, w4_hbm, out_hbm,
            wqkv, wo, w1, w2, w3, w4, xbuf, lnx, ring, obuf, hbuf, mem, h1buf,
            outbuf, sem_x, sem_qkv, sem_w, sem_out):
    def x_copy(i):
        lo, n = ((0, PPAD), (PPAD, S - PPAD))[i]
        return pltpu.make_async_copy(x_hbm.at[pl.ds(lo, n), :],
                                     xbuf.at[pl.ds(lo, n), :], sem_x.at[i])

    def qkv_copies(p):
        cps = []
        for wi, w_hbm in enumerate((wq_hbm, wk_hbm, wv_hbm)):
            wu = w_hbm.bitcast(U32)
            for par in range(2):
                cps.append(pltpu.make_async_copy(
                    wu.at[:, par, p, :], wqkv.at[wi * H + 2 * p + par],
                    sem_qkv.at[p]))
        return cps

    def w_copy(i):
        src, dst = ((wo_hbm, wo), (w1_hbm, w1), (w2_hbm, w2), (w3_hbm, w3),
                    (w4_hbm, w4))[i]
        return pltpu.make_async_copy(src.bitcast(U32), dst, sem_w.at[i])

    x_copy(0).start()
    for p in range(2):
        for c in qkv_copies(p):
            c.start()
    x_copy(1).start()
    for p in range(2, H // 2):
        for c in qkv_copies(p):
            c.start()
    for i in range(5):
        w_copy(i).start()

    mem[...] = mem0_ref[...].astype(F32)
    obuf[:, 0:TPS, :] = jnp.zeros((H, TPS, E), BF16)

    x_copy(0).wait()
    lnx[0:PPAD, :] = _ln(xbuf[0:PPAD, :].astype(F32)).astype(BF16)

    def prologue(p, carry):
        for c in qkv_copies(p):
            c.wait()
        xp = lnx[0:PPAD, :]
        for wi in range(3):
            s0 = wi * H + 2 * p
            a = wqkv[s0]
            b = wqkv[s0 + 1]
            c0 = (a & jnp.uint32(0xFFFF)) | (b << 16)
            c1 = (a >> 16) | (b & jnp.uint32(0xFFFF0000))
            wqkv[s0] = c0
            wqkv[s0 + 1] = c1
            ring[s0, 0:PPAD, :] = _dot(xp, _w(c0)).astype(BF16)
            ring[s0 + 1, 0:PPAD, :] = _dot(xp, _w(c1)).astype(BF16)
        return carry

    jax.lax.fori_loop(0, H // 2, prologue, 0)

    x_copy(1).wait()

    def ln_rest(i, carry):
        r = pl.ds(pl.multiple_of(PPAD + i * 376, 8), 376)
        lnx[r, :] = _ln(xbuf[r, :].astype(F32)).astype(BF16)
        return carry

    jax.lax.fori_loop(0, 4, ln_rest, 0)
    w_copy(0).wait()

    LP = 48
    row = jax.lax.broadcasted_iota(jnp.int32, (LP, LP), 0)
    col = jax.lax.broadcasted_iota(jnp.int32, (LP, LP), 1)
    allowed = (col < SEG + M) & ((col >= SEG) | (row >= SEG) | (col <= row))
    scale = E ** (-0.5)

    def step(s, carry):
        t0 = pl.multiple_of(jnp.minimum(P0 + TPS * s, S - TPS), 8)
        tok = lnx[pl.ds(t0, TPS), :].astype(F32)
        xs = jnp.concatenate([mem[...], tok], axis=0).astype(BF16)
        wpos = [pl.multiple_of((t0 + 8 * g) % RING, 8) for g in range(3)]
        rpos = pl.multiple_of((SEG * s) % RING, SEG)
        opos = pl.multiple_of(SEG * s, SEG)
        ord_ = pl.multiple_of(jnp.maximum(s - 1, 0) * TPS, 8)
        zpad = jnp.zeros((8, E), F32)
        lhs_o = []
        for h in range(H):
            parts = []
            for wi in range(3):
                y = _dot(xs, _w(wqkv[wi * H + h]))
                tokpart = ring[wi * H + h, pl.ds(rpos, SEG), :]
                for g in range(3):
                    ring[wi * H + h, pl.ds(wpos[g], 8), :] = (
                        y[8 + 8 * g:16 + 8 * g].astype(BF16))
                mpart = jnp.concatenate([y[0:8], zpad], axis=0).astype(BF16)
                parts.append(jnp.concatenate([tokpart, mpart], axis=0))
            q, k, v = parts
            sc = jax.lax.dot_general(q, k, (((1,), (1,)), ((), ())),
                                     preferred_element_type=F32) * scale
            sc = jnp.where(allowed, sc, NEG)
            mx = jnp.max(sc, axis=-1, keepdims=True)
            pe = jnp.exp(sc - mx)
            pr = pe / jnp.sum(pe, axis=-1, keepdims=True)
            o = _dot(pr.astype(BF16), v)
            oprev = obuf[h, pl.ds(ord_, TPS), :].astype(F32)
            obuf[h, pl.ds(opos, SEG), :] = o[0:SEG].astype(BF16)
            lhs_o.append(jnp.concatenate([o[SEG:SEG + M], oprev], axis=0)
                         .astype(BF16))
        split = 28
        la = jnp.concatenate(lhs_o[:split], axis=1)
        lb = jnp.concatenate(lhs_o[split:], axis=1)
        res = (_dot(la, _w(wo[0:split * E // 2, :]))
               + _dot(lb, _w(wo[split * E // 2:, :])))
        mem[...] = res[0:M]
        hbuf[pl.ds(ord_, TPS), :] = res[M:]
        return carry

    jax.lax.fori_loop(0, NSEG, step, 0)

    NT = S - OTAIL
    lo_ = jnp.concatenate([obuf[h, OTAIL - 8:S, :] for h in range(H)], axis=1)
    hbuf[OTAIL - 8:S, :] = _dot(lo_, _w(wo[...]))

    for i in range(1, 5):
        w_copy(i).wait()

    h1buf[0:8, :] = jnp.zeros((8, D), F32)
    h1buf[S + 8:S + 16, :] = jnp.zeros((8, D), F32)

    def pass1(c, carry):
        r = pl.ds(pl.multiple_of(c * CH, CH), CH)
        hh = xbuf[r, :].astype(F32) + hbuf[r, :]
        hbuf[r, :] = hh
        t = _ln(_ln(hh)).astype(BF16)
        h1buf[pl.ds(pl.multiple_of(c * CH + 8, 8), CH), :] = _gelu(
            _dot(t, _w(w1[...])))
        return carry

    jax.lax.fori_loop(0, S // CH, pass1, 0)

    def out_copy(c):
        r = pl.ds(pl.multiple_of(c * CH, CH), CH)
        return pltpu.make_async_copy(outbuf.at[r, :], out_hbm.at[r, :],
                                     sem_out.at[c])

    def pass2(c, carry):
        r = pl.ds(pl.multiple_of(c * CH, CH), CH)
        win = h1buf[pl.ds(pl.multiple_of(c * CH, 8), CH + 16), :]
        qd = D // 4
        g = jnp.concatenate([
            win[7:7 + CH, 0 * qd:1 * qd],
            win[9:9 + CH, 1 * qd:2 * qd],
            win[6:6 + CH, 2 * qd:3 * qd],
            win[10:10 + CH, 3 * qd:4 * qd]], axis=1).astype(BF16)
        hh = hbuf[r, :]
        x1 = _ln(hh) + _dot(g, _w(w2[...]))
        t = _ln(x1).astype(BF16)
        u = _gelu(_dot(t, _w(w3[...]))).astype(BF16)
        y = _dot(u, _w(w4[...]))
        outbuf[r, :] = (hh + (x1 + y)).astype(BF16)
        out_copy(c).start()
        return carry

    jax.lax.fori_loop(0, S // CH, pass2, 0)
    for c in range(S // CH):
        out_copy(c).wait()


@functools.partial(jax.jit, static_argnames=("A_seg_len",))
def pallas_sequential_preLN__memory_aug_recurrent_mem_tr__mixer_s_mlp__prompt_kernel(
    A_x: jax.Array,
    A_mem0: jax.Array,
    A_Wq: jax.Array,
    A_Wk: jax.Array,
    A_Wv: jax.Array,
    A_Wo: jax.Array,
    A_seg_len,
    B_x: jax.Array,
    B_w1: jax.Array,
    B_w2: jax.Array,
    B_w3: jax.Array,
    B_w4: jax.Array,
):
    assert A_seg_len == SEG and A_x.shape == (1, S, D)
    x = A_x.reshape(S, D)
    mem0 = A_mem0.reshape(M, D)
    wq = A_Wq.reshape(D // 2, 2, H, E)
    wk = A_Wk.reshape(D // 2, 2, H, E)
    wv = A_Wv.reshape(D // 2, 2, H, E)
    wo = A_Wo.reshape(H * E, D)

    hbm = pl.BlockSpec(memory_space=pl.ANY)
    vmem = pl.BlockSpec(memory_space=pltpu.VMEM)
    out = pl.pallas_call(
        _kernel,
        out_shape=jax.ShapeDtypeStruct((S, D), BF16),
        in_specs=[hbm, vmem] + [hbm] * 8,
        out_specs=hbm,
        scratch_shapes=[
            pltpu.VMEM((3 * H, D // 2, E), U32),
            pltpu.VMEM((H * E // 2, D), U32),
            pltpu.VMEM((D // 2, D), U32),
            pltpu.VMEM((D // 2, D), U32),
            pltpu.VMEM((D // 2, FF), U32),
            pltpu.VMEM((FF // 2, D), U32),
            pltpu.VMEM((S, D), BF16),
            pltpu.VMEM((S, D), BF16),
            pltpu.VMEM((3 * H, RING, E), BF16),
            pltpu.VMEM((H, S, E), BF16),
            pltpu.VMEM((S, D), F32),
            pltpu.VMEM((M, D), F32),
            pltpu.VMEM((S + 16, D), F32),
            pltpu.VMEM((S, D), BF16),
            pltpu.SemaphoreType.DMA((2,)),
            pltpu.SemaphoreType.DMA((H // 2,)),
            pltpu.SemaphoreType.DMA((5,)),
            pltpu.SemaphoreType.DMA((S // CH,)),
        ],
        compiler_params=pltpu.CompilerParams(
            vmem_limit_bytes=126 * 1024 * 1024),
    )(x, mem0, wq, wk, wv, wo, B_w1, B_w2, B_w3, B_w4)
    return out.reshape(1, S, D)
```

```python
import functools

import jax
import jax.numpy as jnp
import jax.experimental.pallas as pl
import jax.experimental.pallas.tpu as pltpu

F32 = jnp.float32
BF16 = jnp.bfloat16
U32 = jnp.uint32

S = 2048
D = 1024
H = 32
E = 128
M = 8
SEG = 32
NSEG = S // SEG
FF = 3584
TPS = 24
P0 = S - TPS * (NSEG - 1)
PPAD = 544
RING = 576
OTAIL = TPS * (NSEG - 1)
CH = 256
EPS = 1e-5
LAG_S = 2
LAG_P = 2
LAG_W = 1
WO_CHUNK = 4
NEG = -1000000000.0


def _ln(x):
    m = jnp.mean(x, axis=-1, keepdims=True)
    xc = x - m
    v = jnp.mean(xc * xc, axis=-1, keepdims=True)
    return xc * jax.lax.rsqrt(v + EPS)


def _gelu(x):
    return jax.nn.gelu(x, approximate=True)


def _dot(a, b):
    return jnp.dot(a, b, preferred_element_type=F32)


def _w(u32_val):
    return pltpu.bitcast(u32_val, BF16)


def _kernel(x_hbm, mem0_ref, wq_hbm, wk_hbm, wv_hbm, wo_hbm, w1_hbm, w2_hbm,
            w3_hbm, w4_hbm, out_hbm,
            wqkv, wo, w1, w2, w3, w4, xbuf, lnx, ring, obuf, hbuf, mem, h1buf,
            outbuf, sem_x, sem_qkv, sem_w, sem_out):
    def x_copy(i):
        lo, n = ((0, PPAD), (PPAD, S - PPAD))[i]
        return pltpu.make_async_copy(x_hbm.at[pl.ds(lo, n), :],
                                     xbuf.at[pl.ds(lo, n), :], sem_x.at[i])

    def qkv_copies(p):
        cps = []
        for wi, w_hbm in enumerate((wq_hbm, wk_hbm, wv_hbm)):
            wu = w_hbm.bitcast(U32)
            for par in range(2):
                cps.append(pltpu.make_async_copy(
                    wu.at[:, par, p, :], wqkv.at[wi * H + 2 * p + par],
                    sem_qkv.at[p]))
        return cps

    def w_copy(i):
        src, dst = ((wo_hbm, wo), (w1_hbm, w1), (w2_hbm, w2), (w3_hbm, w3),
                    (w4_hbm, w4))[i]
        return pltpu.make_async_copy(src.bitcast(U32), dst, sem_w.at[i])

    x_copy(0).start()
    for p in range(2):
        for c in qkv_copies(p):
            c.start()
    x_copy(1).start()
    for p in range(2, H // 2):
        for c in qkv_copies(p):
            c.start()
    for i in range(5):
        w_copy(i).start()

    mem[...] = mem0_ref[...].astype(F32)
    obuf[:, 0:TPS, :] = jnp.zeros((H, TPS, E), BF16)

    x_copy(0).wait()
    lnx[0:PPAD, :] = _ln(xbuf[0:PPAD, :].astype(F32)).astype(BF16)

    def prologue(p, carry):
        for c in qkv_copies(p):
            c.wait()
        xp = lnx[0:PPAD, :]
        for wi in range(3):
            s0 = wi * H + 2 * p
            a = wqkv[s0]
            b = wqkv[s0 + 1]
            c0 = (a & jnp.uint32(0xFFFF)) | (b << 16)
            c1 = (a >> 16) | (b & jnp.uint32(0xFFFF0000))
            wqkv[s0] = c0
            wqkv[s0 + 1] = c1
            ring[s0, 0:PPAD, :] = _dot(xp, _w(c0)).astype(BF16)
            ring[s0 + 1, 0:PPAD, :] = _dot(xp, _w(c1)).astype(BF16)
        return carry

    with jax.named_scope('ph1_prologue'):
        jax.lax.fori_loop(0, H // 2, prologue, 0)

    x_copy(1).wait()

    def ln_rest(i, carry):
        r = pl.ds(pl.multiple_of(PPAD + i * 376, 8), 376)
        lnx[r, :] = _ln(xbuf[r, :].astype(F32)).astype(BF16)
        return carry

    with jax.named_scope('ph1_lnrest'):
        jax.lax.fori_loop(0, 4, ln_rest, 0)
    w_copy(0).wait()

    LP = 48
    row = jax.lax.broadcasted_iota(jnp.int32, (LP, LP), 0)
    col = jax.lax.broadcasted_iota(jnp.int32, (LP, LP), 1)
    allowed = (col < SEG + M) & ((col >= SEG) | (row >= SEG) | (col <= row))
    scale = E ** (-0.5)

    def step(s, carry):
        t0 = pl.multiple_of(jnp.minimum(P0 + TPS * s, S - TPS), 8)
        tok = lnx[pl.ds(t0, TPS), :].astype(F32)
        xs = jnp.concatenate([mem[...], tok], axis=0).astype(BF16)
        wpos = [pl.multiple_of((t0 + 8 * g) % RING, 8) for g in range(3)]
        rpos = pl.multiple_of((SEG * s) % RING, SEG)
        opos = pl.multiple_of(SEG * s, SEG)
        ord_ = pl.multiple_of(jnp.maximum(s - 1, 0) * TPS, 8)
        zpad = jnp.zeros((8, E), F32)
        qkv = {}
        soft = {}
        lhs_o = {}

        def do_qkv(h):
            parts = []
            for wi in range(3):
                y = _dot(xs, _w(wqkv[wi * H + h]))
                tokpart = ring[wi * H + h, pl.ds(rpos, SEG), :]
                for g in range(3):
                    ring[wi * H + h, pl.ds(wpos[g], 8), :] = (
                        y[8 + 8 * g:16 + 8 * g].astype(BF16))
                mpart = jnp.concatenate([y[0:8], zpad], axis=0).astype(BF16)
                parts.append(jnp.concatenate([tokpart, mpart], axis=0))
            qkv[h] = parts

        def do_scores(h):
            q, k, _ = qkv[h]
            sc = jax.lax.dot_general(q, k, (((1,), (1,)), ((), ())),
                                     preferred_element_type=F32) * scale
            sc = jnp.where(allowed, sc, NEG)
            mx = jnp.max(sc, axis=-1, keepdims=True)
            pe = jnp.exp(sc - mx)
            inv = 1.0 / jnp.sum(pe, axis=-1, keepdims=True)
            soft[h] = (pe.astype(BF16), inv)

        def do_pv(h):
            pe, inv = soft[h]
            o = _dot(pe, qkv[h][2]) * inv
            oprev = obuf[h, pl.ds(ord_, TPS), :].astype(F32)
            obuf[h, pl.ds(opos, SEG), :] = o[0:SEG].astype(BF16)
            lhs_o[h] = (jnp.concatenate([o[SEG:SEG + M], oprev], axis=0)
                        .astype(BF16))

        def do_wo(h0, h1):
            la = jnp.concatenate([lhs_o[h] for h in range(h0, h1)], axis=1)
            return _dot(la, _w(wo[h0 * E // 2:h1 * E // 2, :]))

        for i in range(H):
            do_qkv(i)
            if i - LAG_S >= 0:
                do_scores(i - LAG_S)
            if i - LAG_S - LAG_P >= 0:
                do_pv(i - LAG_S - LAG_P)
        ns = H - LAG_S
        npv = H - LAG_S - LAG_P
        res = None
        done = 0
        while done < H:
            avail = npv - LAG_W
            if npv >= H:
                avail = H
            if ns < H:
                chunk = min(WO_CHUNK, avail - done)
            else:
                chunk = min(WO_CHUNK, avail - done)
            if chunk > 0:
                r = do_wo(done, done + chunk)
                res = r if res is None else res + r
                done += chunk
            if ns < H:
                do_scores(ns)
                ns += 1
            if npv < H:
                do_pv(npv)
                npv += 1
        mem[...] = res[0:M]
        hbuf[pl.ds(ord_, TPS), :] = res[M:]
        return carry

    with jax.named_scope('ph2_steps'):
        jax.lax.fori_loop(0, NSEG, step, 0)

    NT = S - OTAIL
    with jax.named_scope('ph3_wo'):
        lo_ = jnp.concatenate([obuf[h, OTAIL - 8:S, :] for h in range(H)], axis=1)
        hbuf[OTAIL - 8:S, :] = _dot(lo_, _w(wo[...]))

    for i in range(1, 5):
        w_copy(i).wait()

    h1buf[0:8, :] = jnp.zeros((8, D), F32)
    h1buf[S + 8:S + 16, :] = jnp.zeros((8, D), F32)

    def pass1(c, carry):
        r = pl.ds(pl.multiple_of(c * CH, CH), CH)
        hh = xbuf[r, :].astype(F32) + hbuf[r, :]
        hbuf[r, :] = hh
        t = _ln(_ln(hh)).astype(BF16)
        h1buf[pl.ds(pl.multiple_of(c * CH + 8, 8), CH), :] = _gelu(
            _dot(t, _w(w1[...])))
        return carry

    with jax.named_scope('ph3_pass1'):
        jax.lax.fori_loop(0, S // CH, pass1, 0)

    def out_copy(c):
        r = pl.ds(pl.multiple_of(c * CH, CH), CH)
        return pltpu.make_async_copy(outbuf.at[r, :], out_hbm.at[r, :],
                                     sem_out.at[c])

    def pass2(c, carry):
        r = pl.ds(pl.multiple_of(c * CH, CH), CH)
        win = h1buf[pl.ds(pl.multiple_of(c * CH, 8), CH + 16), :]
        qd = D // 4
        g = jnp.concatenate([
            win[7:7 + CH, 0 * qd:1 * qd],
            win[9:9 + CH, 1 * qd:2 * qd],
            win[6:6 + CH, 2 * qd:3 * qd],
            win[10:10 + CH, 3 * qd:4 * qd]], axis=1).astype(BF16)
        hh = hbuf[r, :]
        x1 = _ln(hh) + _dot(g, _w(w2[...]))
        t = _ln(x1).astype(BF16)
        u = _gelu(_dot(t, _w(w3[...]))).astype(BF16)
        y = _dot(u, _w(w4[...]))
        outbuf[r, :] = (hh + (x1 + y)).astype(BF16)
        out_copy(c).start()
        return carry

    with jax.named_scope('ph3_pass2'):
        jax.lax.fori_loop(0, S // CH, pass2, 0)
    for c in range(S // CH):
        out_copy(c).wait()


@functools.partial(jax.jit, static_argnames=("A_seg_len",))
def pallas_sequential_preLN__memory_aug_recurrent_mem_tr__mixer_s_mlp__prompt_kernel(
    A_x: jax.Array,
    A_mem0: jax.Array,
    A_Wq: jax.Array,
    A_Wk: jax.Array,
    A_Wv: jax.Array,
    A_Wo: jax.Array,
    A_seg_len,
    B_x: jax.Array,
    B_w1: jax.Array,
    B_w2: jax.Array,
    B_w3: jax.Array,
    B_w4: jax.Array,
):
    assert A_seg_len == SEG and A_x.shape == (1, S, D)
    x = A_x.reshape(S, D)
    mem0 = A_mem0.reshape(M, D)
    wq = A_Wq.reshape(D // 2, 2, H, E)
    wk = A_Wk.reshape(D // 2, 2, H, E)
    wv = A_Wv.reshape(D // 2, 2, H, E)
    wo = A_Wo.reshape(H * E, D)

    hbm = pl.BlockSpec(memory_space=pl.ANY)
    vmem = pl.BlockSpec(memory_space=pltpu.VMEM)
    out = pl.pallas_call(
        _kernel,
        out_shape=jax.ShapeDtypeStruct((S, D), BF16),
        in_specs=[hbm, vmem] + [hbm] * 8,
        out_specs=hbm,
        scratch_shapes=[
            pltpu.VMEM((3 * H, D // 2, E), U32),
            pltpu.VMEM((H * E // 2, D), U32),
            pltpu.VMEM((D // 2, D), U32),
            pltpu.VMEM((D // 2, D), U32),
            pltpu.VMEM((D // 2, FF), U32),
            pltpu.VMEM((FF // 2, D), U32),
            pltpu.VMEM((S, D), BF16),
            pltpu.VMEM((S, D), BF16),
            pltpu.VMEM((3 * H, RING, E), BF16),
            pltpu.VMEM((H, S, E), BF16),
            pltpu.VMEM((S, D), F32),
            pltpu.VMEM((M, D), F32),
            pltpu.VMEM((S + 16, D), F32),
            pltpu.VMEM((S, D), BF16),
            pltpu.SemaphoreType.DMA((2,)),
            pltpu.SemaphoreType.DMA((H // 2,)),
            pltpu.SemaphoreType.DMA((5,)),
            pltpu.SemaphoreType.DMA((S // CH,)),
        ],
        compiler_params=pltpu.CompilerParams(
            vmem_limit_bytes=126 * 1024 * 1024),
    )(x, mem0, wq, wk, wv, wo, B_w1, B_w2, B_w3, B_w4)
    return out.reshape(1, S, D)
```

```python
import functools

import jax
import jax.numpy as jnp
import jax.experimental.pallas as pl
import jax.experimental.pallas.tpu as pltpu

F32 = jnp.float32
BF16 = jnp.bfloat16
U32 = jnp.uint32

S = 2048
D = 1024
H = 32
E = 128
M = 8
SEG = 32
NSEG = S // SEG
FF = 3584
TPS = 24
P0 = S - TPS * (NSEG - 1)
PPAD = 544
RING = 576
OTAIL = TPS * (NSEG - 1)
CH = 256
EPS = 1e-5
LAG_S = 2
LAG_P = 2
LAG_W = 1
WO_CHUNK = 4
NEG = -1000000000.0


def _ln(x):
    m = jnp.mean(x, axis=-1, keepdims=True)
    xc = x - m
    v = jnp.mean(xc * xc, axis=-1, keepdims=True)
    return xc * jax.lax.rsqrt(v + EPS)


def _gelu(x):
    return jax.nn.gelu(x, approximate=True)


def _dot(a, b):
    return jnp.dot(a, b, preferred_element_type=F32)


def _w(u32_val):
    return pltpu.bitcast(u32_val, BF16)


def _kernel(x_hbm, mem0_ref, wq_hbm, wk_hbm, wv_hbm, wo_hbm, w1_hbm, w2_hbm,
            w3_hbm, w4_hbm, out_hbm,
            wqkv, wo, w1, w2, w3, w4, xbuf, lnx, ring, obuf, hbuf, mem, h1buf,
            outbuf, sem_x, sem_qkv, sem_w, sem_out):
    def x_copy(i):
        lo, n = ((0, PPAD), (PPAD, S - PPAD))[i]
        return pltpu.make_async_copy(x_hbm.at[pl.ds(lo, n), :],
                                     xbuf.at[pl.ds(lo, n), :], sem_x.at[i])

    def qkv_copies(p):
        cps = []
        for wi, w_hbm in enumerate((wq_hbm, wk_hbm, wv_hbm)):
            wu = w_hbm.bitcast(U32)
            for par in range(2):
                cps.append(pltpu.make_async_copy(
                    wu.at[:, par, p, :], wqkv.at[wi * H + 2 * p + par],
                    sem_qkv.at[p]))
        return cps

    def w_copy(i):
        src, dst = ((wo_hbm, wo), (w1_hbm, w1), (w2_hbm, w2), (w3_hbm, w3),
                    (w4_hbm, w4))[i]
        return pltpu.make_async_copy(src.bitcast(U32), dst, sem_w.at[i])

    x_copy(0).start()
    for p in range(2):
        for c in qkv_copies(p):
            c.start()
    x_copy(1).start()

    mem[...] = mem0_ref[...].astype(F32)
    obuf[:, 0:TPS, :] = jnp.zeros((H, TPS, E), BF16)

    x_copy(0).wait()
    lnx[0:PPAD, :] = _ln(xbuf[0:PPAD, :].astype(F32)).astype(BF16)

    def prologue(p, carry):
        @pl.when(p + 2 < H // 2)
        def _():
            for c in qkv_copies(p + 2):
                c.start()

        for i, at in enumerate((13, 14, 14, 15, 15)):
            @pl.when(p == at)
            def _():
                w_copy(i).start()

        for c in qkv_copies(p):
            c.wait()
        xp = lnx[0:PPAD, :]
        for wi in range(3):
            s0 = wi * H + 2 * p
            a = wqkv[s0]
            b = wqkv[s0 + 1]
            c0 = (a & jnp.uint32(0xFFFF)) | (b << 16)
            c1 = (a >> 16) | (b & jnp.uint32(0xFFFF0000))
            wqkv[s0] = c0
            wqkv[s0 + 1] = c1
            ring[s0, 0:PPAD, :] = _dot(xp, _w(c0)).astype(BF16)
            ring[s0 + 1, 0:PPAD, :] = _dot(xp, _w(c1)).astype(BF16)
        return carry

    with jax.named_scope('ph1_prologue'):
        jax.lax.fori_loop(0, H // 2, prologue, 0)

    x_copy(1).wait()

    def ln_rest(i, carry):
        r = pl.ds(pl.multiple_of(PPAD + i * 376, 8), 376)
        lnx[r, :] = _ln(xbuf[r, :].astype(F32)).astype(BF16)
        return carry

    with jax.named_scope('ph1_lnrest'):
        jax.lax.fori_loop(0, 4, ln_rest, 0)
    w_copy(0).wait()

    LP = 48
    row = jax.lax.broadcasted_iota(jnp.int32, (LP, LP), 0)
    col = jax.lax.broadcasted_iota(jnp.int32, (LP, LP), 1)
    allowed = (col < SEG + M) & ((col >= SEG) | (row >= SEG) | (col <= row))
    scale = E ** (-0.5)

    def step(s, carry):
        t0 = pl.multiple_of(jnp.minimum(P0 + TPS * s, S - TPS), 8)
        tok = lnx[pl.ds(t0, TPS), :].astype(F32)
        xs = jnp.concatenate([mem[...], tok], axis=0).astype(BF16)
        wpos = [pl.multiple_of((t0 + 8 * g) % RING, 8) for g in range(3)]
        rpos = pl.multiple_of((SEG * s) % RING, SEG)
        opos = pl.multiple_of(SEG * s, SEG)
        ord_ = pl.multiple_of(jnp.maximum(s - 1, 0) * TPS, 8)
        zpad = jnp.zeros((8, E), F32)
        qkv = {}
        soft = {}
        lhs_o = {}

        def do_qkv(h):
            parts = []
            for wi in range(3):
                y = _dot(xs, _w(wqkv[wi * H + h]))
                tokpart = ring[wi * H + h, pl.ds(rpos, SEG), :]
                for g in range(3):
                    ring[wi * H + h, pl.ds(wpos[g], 8), :] = (
                        y[8 + 8 * g:16 + 8 * g].astype(BF16))
                mpart = jnp.concatenate([y[0:8], zpad], axis=0).astype(BF16)
                parts.append(jnp.concatenate([tokpart, mpart], axis=0))
            qkv[h] = parts

        def do_scores(h):
            q, k, _ = qkv[h]
            sc = jax.lax.dot_general(q, k, (((1,), (1,)), ((), ())),
                                     preferred_element_type=F32) * scale
            sc = jnp.where(allowed, sc, NEG)
            mx = jnp.max(sc, axis=-1, keepdims=True)
            pe = jnp.exp(sc - mx)
            inv = 1.0 / jnp.sum(pe, axis=-1, keepdims=True)
            soft[h] = (pe.astype(BF16), inv)

        def do_pv(h):
            pe, inv = soft[h]
            o = _dot(pe, qkv[h][2]) * inv
            oprev = obuf[h, pl.ds(ord_, TPS), :].astype(F32)
            obuf[h, pl.ds(opos, SEG), :] = o[0:SEG].astype(BF16)
            lhs_o[h] = (jnp.concatenate([o[SEG:SEG + M], oprev], axis=0)
                        .astype(BF16))

        def do_wo(h0, h1):
            la = jnp.concatenate([lhs_o[h] for h in range(h0, h1)], axis=1)
            return _dot(la, _w(wo[h0 * E // 2:h1 * E // 2, :]))

        for i in range(H):
            do_qkv(i)
            if i - LAG_S >= 0:
                do_scores(i - LAG_S)
            if i - LAG_S - LAG_P >= 0:
                do_pv(i - LAG_S - LAG_P)
        ns = H - LAG_S
        npv = H - LAG_S - LAG_P
        res = None
        done = 0
        while done < H:
            avail = npv - LAG_W
            if npv >= H:
                avail = H
            if ns < H:
                chunk = min(WO_CHUNK, avail - done)
            else:
                chunk = min(WO_CHUNK, avail - done)
            if chunk > 0:
                r = do_wo(done, done + chunk)
                res = r if res is None else res + r
                done += chunk
            if ns < H:
                do_scores(ns)
                ns += 1
            if npv < H:
                do_pv(npv)
                npv += 1
        mem[...] = res[0:M]
        hbuf[pl.ds(ord_, TPS), :] = res[M:]
        return carry

    with jax.named_scope('ph2_steps'):
        jax.lax.fori_loop(0, NSEG, step, 0)

    NT = S - OTAIL
    def wo_tail(j, carry):
        cs = pl.ds(pl.multiple_of(j * 128, 128), 128)
        lo_ = jnp.concatenate([obuf[h, OTAIL - 8:S, :] for h in range(H)], axis=1)
        hbuf[OTAIL - 8:S, cs] = _dot(lo_, _w(wo[:, cs]))
        return carry

    with jax.named_scope('ph3_wo'):
        jax.lax.fori_loop(0, D // 128, wo_tail, 0)

    for i in range(1, 5):
        w_copy(i).wait()

    h1buf[0:8, :] = jnp.zeros((8, D), F32)
    h1buf[S + 8:S + 16, :] = jnp.zeros((8, D), F32)

    def pass1(c, carry):
        r = pl.ds(pl.multiple_of(c * CH, CH), CH)
        hh = xbuf[r, :].astype(F32) + hbuf[r, :]
        hbuf[r, :] = hh
        t = _ln(_ln(hh)).astype(BF16)
        h1buf[pl.ds(pl.multiple_of(c * CH + 8, 8), CH), :] = _gelu(
            _dot(t, _w(w1[...])))
        return carry

    with jax.named_scope('ph3_pass1'):
        jax.lax.fori_loop(0, S // CH, pass1, 0)

    def out_copy(c):
        r = pl.ds(pl.multiple_of(c * CH, CH), CH)
        return pltpu.make_async_copy(outbuf.at[r, :], out_hbm.at[r, :],
                                     sem_out.at[c])

    def pass2(c, carry):
        r = pl.ds(pl.multiple_of(c * CH, CH), CH)
        win = h1buf[pl.ds(pl.multiple_of(c * CH, 8), CH + 16), :]
        qd = D // 4
        g = jnp.concatenate([
            win[7:7 + CH, 0 * qd:1 * qd],
            win[9:9 + CH, 1 * qd:2 * qd],
            win[6:6 + CH, 2 * qd:3 * qd],
            win[10:10 + CH, 3 * qd:4 * qd]], axis=1).astype(BF16)
        hh = hbuf[r, :]
        x1 = _ln(hh) + _dot(g, _w(w2[...]))
        t = _ln(x1).astype(BF16)
        u = _gelu(_dot(t, _w(w3[...]))).astype(BF16)
        y = _dot(u, _w(w4[...]))
        outbuf[r, :] = (hh + (x1 + y)).astype(BF16)
        out_copy(c).start()
        return carry

    with jax.named_scope('ph3_pass2'):
        jax.lax.fori_loop(0, S // CH, pass2, 0)
    for c in range(S // CH):
        out_copy(c).wait()


@functools.partial(jax.jit, static_argnames=("A_seg_len",))
def pallas_sequential_preLN__memory_aug_recurrent_mem_tr__mixer_s_mlp__prompt_kernel(
    A_x: jax.Array,
    A_mem0: jax.Array,
    A_Wq: jax.Array,
    A_Wk: jax.Array,
    A_Wv: jax.Array,
    A_Wo: jax.Array,
    A_seg_len,
    B_x: jax.Array,
    B_w1: jax.Array,
    B_w2: jax.Array,
    B_w3: jax.Array,
    B_w4: jax.Array,
):
    assert A_seg_len == SEG and A_x.shape == (1, S, D)
    x = A_x.reshape(S, D)
    mem0 = A_mem0.reshape(M, D)
    wq = A_Wq.reshape(D // 2, 2, H, E)
    wk = A_Wk.reshape(D // 2, 2, H, E)
    wv = A_Wv.reshape(D // 2, 2, H, E)
    wo = A_Wo.reshape(H * E, D)

    hbm = pl.BlockSpec(memory_space=pl.ANY)
    vmem = pl.BlockSpec(memory_space=pltpu.VMEM)
    out = pl.pallas_call(
        _kernel,
        out_shape=jax.ShapeDtypeStruct((S, D), BF16),
        in_specs=[hbm, vmem] + [hbm] * 8,
        out_specs=hbm,
        scratch_shapes=[
            pltpu.VMEM((3 * H, D // 2, E), U32),
            pltpu.VMEM((H * E // 2, D), U32),
            pltpu.VMEM((D // 2, D), U32),
            pltpu.VMEM((D // 2, D), U32),
            pltpu.VMEM((D // 2, FF), U32),
            pltpu.VMEM((FF // 2, D), U32),
            pltpu.VMEM((S, D), BF16),
            pltpu.VMEM((S, D), BF16),
            pltpu.VMEM((3 * H, RING, E), BF16),
            pltpu.VMEM((H, S, E), BF16),
            pltpu.VMEM((S, D), F32),
            pltpu.VMEM((M, D), F32),
            pltpu.VMEM((S + 16, D), F32),
            pltpu.VMEM((S, D), BF16),
            pltpu.SemaphoreType.DMA((2,)),
            pltpu.SemaphoreType.DMA((H // 2,)),
            pltpu.SemaphoreType.DMA((5,)),
            pltpu.SemaphoreType.DMA((S // CH,)),
        ],
        compiler_params=pltpu.CompilerParams(
            vmem_limit_bytes=126 * 1024 * 1024),
    )(x, mem0, wq, wk, wv, wo, B_w1, B_w2, B_w3, B_w4)
    return out.reshape(1, S, D)
```

```python
import functools

import jax
import jax.numpy as jnp
import jax.experimental.pallas as pl
import jax.experimental.pallas.tpu as pltpu

F32 = jnp.float32
BF16 = jnp.bfloat16
U32 = jnp.uint32

S = 2048
D = 1024
H = 32
E = 128
M = 8
SEG = 32
NSEG = S // SEG
FF = 3584
TPS = 24
P0 = S - TPS * (NSEG - 1)
PPAD = 544
RING = 576
OTAIL = TPS * (NSEG - 1)
CH = 256
EPS = 1e-5
LAG_S = 1
LAG_P = 2
TAIL = (('w', 0, 8), ('p', 13, 0), ('s', 15, 0), ('w', 8, 16), ('p', 14, 0),
        ('w', 16, 24), ('p', 15, 0), ('w', 24, 28), ('w', 28, 32))
NEG = -1000000000.0


def _ln(x):
    m = jnp.mean(x, axis=-1, keepdims=True)
    xc = x - m
    v = jnp.mean(xc * xc, axis=-1, keepdims=True)
    return xc * jax.lax.rsqrt(v + EPS)


def _recip(x):
    r = pl.reciprocal(x, approx=True)
    return r * (2.0 - x * r)


def _gelu(x):
    return jax.nn.gelu(x, approximate=True)


def _dot(a, b):
    return jnp.dot(a, b, preferred_element_type=F32)


def _w(u32_val):
    return pltpu.bitcast(u32_val, BF16)


def _kernel(x_hbm, mem0_ref, wq_hbm, wk_hbm, wv_hbm, wo_hbm, w1_hbm, w2_hbm,
            w3_hbm, w4_hbm, out_hbm,
            wqkv, wo, w1, w2, w3, w4, xbuf, lnx, ring, obuf, hbuf, mem, h1buf,
            outbuf, sem_x, sem_qkv, sem_w, sem_out):
    def x_copy(i):
        lo, n = ((0, PPAD), (PPAD, S - PPAD))[i]
        return pltpu.make_async_copy(x_hbm.at[pl.ds(lo, n), :],
                                     xbuf.at[pl.ds(lo, n), :], sem_x.at[i])

    def qkv_copies(p):
        cps = []
        for wi, w_hbm in enumerate((wq_hbm, wk_hbm, wv_hbm)):
            wu = w_hbm.bitcast(U32)
            for par in range(2):
                cps.append(pltpu.make_async_copy(
                    wu.at[:, par, p, :], wqkv.at[wi * H + 2 * p + par],
                    sem_qkv.at[p]))
        return cps

    def w_copy(i):
        src, dst = ((wo_hbm, wo), (w1_hbm, w1), (w2_hbm, w2), (w3_hbm, w3),
                    (w4_hbm, w4))[i]
        return pltpu.make_async_copy(src.bitcast(U32), dst, sem_w.at[i])

    x_copy(0).start()
    for p in range(2):
        for c in qkv_copies(p):
            c.start()
    x_copy(1).start()

    mem[...] = mem0_ref[...].astype(F32)
    obuf[:, 0:TPS, :] = jnp.zeros((H, TPS, E), BF16)

    x_copy(0).wait()
    lnx[0:PPAD, :] = _ln(xbuf[0:PPAD, :].astype(F32)).astype(BF16)

    def prologue(p, carry):
        @pl.when(p + 2 < H // 2)
        def _():
            for c in qkv_copies(p + 2):
                c.start()

        for i, at in enumerate((13, 14, 14, 15, 15)):
            @pl.when(p == at)
            def _():
                w_copy(i).start()

        for c in qkv_copies(p):
            c.wait()
        xp = lnx[0:PPAD, :]
        for wi in range(3):
            s0 = wi * H + 2 * p
            a = wqkv[s0]
            b = wqkv[s0 + 1]
            c0 = (a & jnp.uint32(0xFFFF)) | (b << 16)
            c1 = (a >> 16) | (b & jnp.uint32(0xFFFF0000))
            wqkv[s0] = c0
            wqkv[s0 + 1] = c1
            ring[s0, 0:PPAD, :] = _dot(xp, _w(c0)).astype(BF16)
            ring[s0 + 1, 0:PPAD, :] = _dot(xp, _w(c1)).astype(BF16)
        return carry

    with jax.named_scope('ph1_prologue'):
        jax.lax.fori_loop(0, H // 2, prologue, 0)

    x_copy(1).wait()

    def ln_rest(i, carry):
        r = pl.ds(pl.multiple_of(PPAD + i * 376, 8), 376)
        lnx[r, :] = _ln(xbuf[r, :].astype(F32)).astype(BF16)
        return carry

    with jax.named_scope('ph1_lnrest'):
        jax.lax.fori_loop(0, 4, ln_rest, 0)
    w_copy(0).wait()

    LP = 2 * (SEG + M)
    row = jax.lax.broadcasted_iota(jnp.int32, (LP, LP), 0)
    col = jax.lax.broadcasted_iota(jnp.int32, (LP, LP), 1)

    def head_of(i):
        return jnp.where(i < 2 * SEG, i // SEG, (i - 2 * SEG) // M)

    same_head = head_of(row) == head_of(col)
    allowed = same_head & ((col >= 2 * SEG) | (row >= 2 * SEG)
                           | (col % SEG <= row % SEG))
    scale = E ** (-0.5)
    bias = jnp.where(allowed, 0.0,
                     jnp.where(same_head, NEG / scale, -jnp.inf)).astype(F32)
    exp_c = scale * 1.4426950408889634

    def step(s, carry):
        t0 = pl.multiple_of(jnp.minimum(P0 + TPS * s, S - TPS), 8)
        tok = lnx[pl.ds(t0, TPS), :].astype(F32)
        xs = jnp.concatenate([mem[...], tok], axis=0).astype(BF16)
        wpos = [pl.multiple_of((t0 + 8 * g) % RING, 8) for g in range(3)]
        rpos = pl.multiple_of((SEG * s) % RING, SEG)
        opos = pl.multiple_of(SEG * s, SEG)
        ord_ = pl.multiple_of(jnp.maximum(s - 1, 0) * TPS, 8)
        qkv = {}
        soft = {}
        lhs_o = {}
        NP = H // 2

        def do_qkv(j):
            parts = []
            for wi in range(3):
                toks, mems = [], []
                for h in (2 * j, 2 * j + 1):
                    y = _dot(xs, _w(wqkv[wi * H + h]))
                    toks.append(ring[wi * H + h, pl.ds(rpos, SEG), :])
                    for g in range(3):
                        ring[wi * H + h, pl.ds(wpos[g], 8), :] = (
                            y[8 + 8 * g:16 + 8 * g].astype(BF16))
                    mems.append(y[0:8])
                mpart = jnp.concatenate(mems, axis=0).astype(BF16)
                parts.append(jnp.concatenate(toks + [mpart], axis=0))
            qkv[j] = parts

        def do_scores(j):
            q, k, _ = qkv[j]
            sc = jax.lax.dot_general(q, k, (((1,), (1,)), ((), ())),
                                     preferred_element_type=F32) + bias
            mx = jnp.max(sc, axis=-1, keepdims=True)
            pe = jnp.exp2((sc - mx) * exp_c)
            inv = _recip(jnp.sum(pe, axis=-1, keepdims=True))
            soft[j] = (pe.astype(BF16), inv)

        def do_pv(j):
            pe, inv = soft[j]
            o = _dot(pe, qkv[j][2]) * inv
            for i, h in enumerate((2 * j, 2 * j + 1)):
                oprev = obuf[h, pl.ds(ord_, TPS), :].astype(F32)
                obuf[h, pl.ds(opos, SEG), :] = (
                    o[i * SEG:(i + 1) * SEG].astype(BF16))
                om = o[2 * SEG + i * M:2 * SEG + (i + 1) * M]
                lhs_o[h] = jnp.concatenate([om, oprev], axis=0).astype(BF16)

        def do_wo(h0, h1):
            la = jnp.concatenate([lhs_o[h] for h in range(h0, h1)], axis=1)
            return _dot(la, _w(wo[h0 * E // 2:h1 * E // 2, :]))

        for i in range(NP):
            do_qkv(i)
            if i - LAG_S >= 0:
                do_scores(i - LAG_S)
            if i - LAG_S - LAG_P >= 0:
                do_pv(i - LAG_S - LAG_P)
        res = None
        for kind, a, b in TAIL:
            if kind == 's':
                do_scores(a)
            elif kind == 'p':
                do_pv(a)
            else:
                r = do_wo(a, b)
                res = r if res is None else res + r
        mem[...] = res[0:M]
        hbuf[pl.ds(ord_, TPS), :] = res[M:]
        return carry

    with jax.named_scope('ph2_steps'):
        jax.lax.fori_loop(0, NSEG, step, 0)

    NT = S - OTAIL
    def wo_tail(j, carry):
        cs = pl.ds(pl.multiple_of(j * 128, 128), 128)
        lo_ = jnp.concatenate([obuf[h, OTAIL - 8:S, :] for h in range(H)], axis=1)
        hbuf[OTAIL - 8:S, cs] = _dot(lo_, _w(wo[:, cs]))
        return carry

    with jax.named_scope('ph3_wo'):
        jax.lax.fori_loop(0, D // 128, wo_tail, 0)

    for i in range(1, 5):
        w_copy(i).wait()

    h1buf[0:8, :] = jnp.zeros((8, D), F32)
    h1buf[S + 8:S + 16, :] = jnp.zeros((8, D), F32)

    def pass1(c, carry):
        r = pl.ds(pl.multiple_of(c * CH, CH), CH)
        hh = xbuf[r, :].astype(F32) + hbuf[r, :]
        hbuf[r, :] = hh
        t = _ln(_ln(hh)).astype(BF16)
        h1buf[pl.ds(pl.multiple_of(c * CH + 8, 8), CH), :] = _gelu(
            _dot(t, _w(w1[...])))
        return carry

    with jax.named_scope('ph3_pass1'):
        jax.lax.fori_loop(0, S // CH, pass1, 0)

    def out_copy(c):
        r = pl.ds(pl.multiple_of(c * CH, CH), CH)
        return pltpu.make_async_copy(outbuf.at[r, :], out_hbm.at[r, :],
                                     sem_out.at[c])

    def pass2(c, carry):
        r = pl.ds(pl.multiple_of(c * CH, CH), CH)
        win = h1buf[pl.ds(pl.multiple_of(c * CH, 8), CH + 16), :]
        qd = D // 4
        g = jnp.concatenate([
            win[7:7 + CH, 0 * qd:1 * qd],
            win[9:9 + CH, 1 * qd:2 * qd],
            win[6:6 + CH, 2 * qd:3 * qd],
            win[10:10 + CH, 3 * qd:4 * qd]], axis=1).astype(BF16)
        hh = hbuf[r, :]
        x1 = _ln(hh) + _dot(g, _w(w2[...]))
        t = _ln(x1).astype(BF16)
        u = _gelu(_dot(t, _w(w3[...]))).astype(BF16)
        y = _dot(u, _w(w4[...]))
        outbuf[r, :] = (hh + (x1 + y)).astype(BF16)
        out_copy(c).start()
        return carry

    with jax.named_scope('ph3_pass2'):
        jax.lax.fori_loop(0, S // CH, pass2, 0)
    for c in range(S // CH):
        out_copy(c).wait()


@functools.partial(jax.jit, static_argnames=("A_seg_len",))
def pallas_sequential_preLN__memory_aug_recurrent_mem_tr__mixer_s_mlp__prompt_kernel(
    A_x: jax.Array,
    A_mem0: jax.Array,
    A_Wq: jax.Array,
    A_Wk: jax.Array,
    A_Wv: jax.Array,
    A_Wo: jax.Array,
    A_seg_len,
    B_x: jax.Array,
    B_w1: jax.Array,
    B_w2: jax.Array,
    B_w3: jax.Array,
    B_w4: jax.Array,
):
    assert A_seg_len == SEG and A_x.shape == (1, S, D)
    x = A_x.reshape(S, D)
    mem0 = A_mem0.reshape(M, D)
    wq = A_Wq.reshape(D // 2, 2, H, E)
    wk = A_Wk.reshape(D // 2, 2, H, E)
    wv = A_Wv.reshape(D // 2, 2, H, E)
    wo = A_Wo.reshape(H * E, D)

    hbm = pl.BlockSpec(memory_space=pl.ANY)
    vmem = pl.BlockSpec(memory_space=pltpu.VMEM)
    out = pl.pallas_call(
        _kernel,
        out_shape=jax.ShapeDtypeStruct((S, D), BF16),
        in_specs=[hbm, vmem] + [hbm] * 8,
        out_specs=hbm,
        scratch_shapes=[
            pltpu.VMEM((3 * H, D // 2, E), U32),
            pltpu.VMEM((H * E // 2, D), U32),
            pltpu.VMEM((D // 2, D), U32),
            pltpu.VMEM((D // 2, D), U32),
            pltpu.VMEM((D // 2, FF), U32),
            pltpu.VMEM((FF // 2, D), U32),
            pltpu.VMEM((S, D), BF16),
            pltpu.VMEM((S, D), BF16),
            pltpu.VMEM((3 * H, RING, E), BF16),
            pltpu.VMEM((H, S, E), BF16),
            pltpu.VMEM((S, D), F32),
            pltpu.VMEM((M, D), F32),
            pltpu.VMEM((S + 16, D), F32),
            pltpu.VMEM((S, D), BF16),
            pltpu.SemaphoreType.DMA((2,)),
            pltpu.SemaphoreType.DMA((H // 2,)),
            pltpu.SemaphoreType.DMA((5,)),
            pltpu.SemaphoreType.DMA((S // CH,)),
        ],
        compiler_params=pltpu.CompilerParams(
            vmem_limit_bytes=126 * 1024 * 1024),
    )(x, mem0, wq, wk, wv, wo, B_w1, B_w2, B_w3, B_w4)
    return out.reshape(1, S, D)
```

```python
import functools

import jax
import jax.numpy as jnp
import jax.experimental.pallas as pl
import jax.experimental.pallas.tpu as pltpu

F32 = jnp.float32
BF16 = jnp.bfloat16
U32 = jnp.uint32

S = 2048
D = 1024
H = 32
E = 128
M = 8
SEG = 32
NSEG = S // SEG
FF = 3584
TPS = 24
P0 = S - TPS * (NSEG - 1)
PPAD = 544
RING = 576
OTAIL = TPS * (NSEG - 1)
CH = 256
EPS = 1e-5
LAG_S = 1
LAG_P = 2
TAIL = (('w', 0, 8), ('p', 13, 0), ('s', 15, 0), ('w', 8, 16), ('p', 14, 0),
        ('w', 16, 24), ('p', 15, 0), ('w', 24, 28), ('w', 28, 32))
NEG = -1000000000.0


def _ln(x):
    m = jnp.mean(x, axis=-1, keepdims=True)
    xc = x - m
    v = jnp.mean(xc * xc, axis=-1, keepdims=True)
    return xc * jax.lax.rsqrt(v + EPS)


def _recip(x):
    r = pl.reciprocal(x, approx=True)
    return r * (2.0 - x * r)


def _gelu(x):
    return jax.nn.gelu(x, approximate=True)


def _dot(a, b):
    return jnp.dot(a, b, preferred_element_type=F32)


def _w(u32_val):
    return pltpu.bitcast(u32_val, BF16)


def _kernel(x_hbm, mem0_ref, wq_hbm, wk_hbm, wv_hbm, wo_hbm, w1_hbm, w2_hbm,
            w3_hbm, w4_hbm, out_hbm,
            wqkv, wo, w1, w2, w3, w4, xbuf, lnx, ring, obuf, hbuf, mem, h1buf,
            outbuf, sem_x, sem_qkv, sem_wo, sem_w, sem_out):
    def x_copy(i):
        lo, n = ((0, PPAD), (PPAD, S - PPAD))[i]
        return pltpu.make_async_copy(x_hbm.at[pl.ds(lo, n), :],
                                     xbuf.at[pl.ds(lo, n), :], sem_x.at[i])

    def qkv_copies(p):
        cps = []
        for wi, w_hbm in enumerate((wq_hbm, wk_hbm, wv_hbm)):
            wu = w_hbm.bitcast(U32)
            for par in range(2):
                cps.append(pltpu.make_async_copy(
                    wu.at[:, par, p, :], wqkv.at[wi * H + 2 * p + par],
                    sem_qkv.at[p]))
        return cps

    def w_copy(i):
        src, dst = ((w1_hbm, w1), (w2_hbm, w2), (w3_hbm, w3), (w4_hbm, w4))[i]
        return pltpu.make_async_copy(src.bitcast(U32), dst, sem_w.at[i])

    WO_PIECES = 8
    WO_ROWS = H * E // 2 // WO_PIECES

    def wo_copy(i):
        r = pl.ds(pl.multiple_of(i * WO_ROWS, WO_ROWS), WO_ROWS)
        return pltpu.make_async_copy(wo_hbm.bitcast(U32).at[r, :], wo.at[r, :],
                                     sem_wo.at[i])

    x_copy(0).start()
    for c in qkv_copies(0):
        c.start(priority=1)

    mem[...] = mem0_ref[...].astype(F32)
    obuf[:, 0:TPS, :] = jnp.zeros((H, TPS, E), BF16)

    x_copy(0).wait()
    lnx[0:PPAD, :] = _ln(xbuf[0:PPAD, :].astype(F32)).astype(BF16)

    def prologue(p, carry):
        for c in qkv_copies(p):
            c.wait()

        @pl.when(p == 0)
        def _():
            for c in qkv_copies(1):
                c.start()

        @pl.when(p + 2 < H // 2)
        def _():
            for c in qkv_copies(p + 2):
                c.start()

        @pl.when((p >= 2) & (p < 2 + WO_PIECES))
        def _():
            wo_copy(p - 2).start()

        @pl.when(p == 10)
        def _():
            x_copy(1).start()

        xp = lnx[0:PPAD, :]
        for wi in range(3):
            s0 = wi * H + 2 * p
            a = wqkv[s0]
            b = wqkv[s0 + 1]
            c0 = (a & jnp.uint32(0xFFFF)) | (b << 16)
            c1 = (a >> 16) | (b & jnp.uint32(0xFFFF0000))
            wqkv[s0] = c0
            wqkv[s0 + 1] = c1
            ring[s0, 0:PPAD, :] = _dot(xp, _w(c0)).astype(BF16)
            ring[s0 + 1, 0:PPAD, :] = _dot(xp, _w(c1)).astype(BF16)
        return carry

    with jax.named_scope('ph1_prologue'):
        jax.lax.fori_loop(0, H // 2, prologue, 0)

    x_copy(1).wait()

    def ln_rest(i, carry):
        r = pl.ds(pl.multiple_of(PPAD + i * 376, 8), 376)
        lnx[r, :] = _ln(xbuf[r, :].astype(F32)).astype(BF16)
        return carry

    with jax.named_scope('ph1_lnrest'):
        jax.lax.fori_loop(0, 4, ln_rest, 0)
    for i in range(WO_PIECES):
        wo_copy(i).wait()
    for i in range(4):
        w_copy(i).start()

    LP = 2 * (SEG + M)
    row = jax.lax.broadcasted_iota(jnp.int32, (LP, LP), 0)
    col = jax.lax.broadcasted_iota(jnp.int32, (LP, LP), 1)

    def head_of(i):
        return jnp.where(i < 2 * SEG, i // SEG, (i - 2 * SEG) // M)

    same_head = head_of(row) == head_of(col)
    allowed = same_head & ((col >= 2 * SEG) | (row >= 2 * SEG)
                           | (col % SEG <= row % SEG))
    scale = E ** (-0.5)
    bias = jnp.where(allowed, 0.0,
                     jnp.where(same_head, NEG / scale, -jnp.inf)).astype(F32)
    exp_c = scale * 1.4426950408889634

    def step(s, carry):
        t0 = pl.multiple_of(jnp.minimum(P0 + TPS * s, S - TPS), 8)
        tok = lnx[pl.ds(t0, TPS), :].astype(F32)
        xs = jnp.concatenate([mem[...], tok], axis=0).astype(BF16)
        wpos = [pl.multiple_of((t0 + 8 * g) % RING, 8) for g in range(3)]
        rpos = pl.multiple_of((SEG * s) % RING, SEG)
        opos = pl.multiple_of(SEG * s, SEG)
        ord_ = pl.multiple_of(jnp.maximum(s - 1, 0) * TPS, 8)
        qkv = {}
        soft = {}
        lhs_o = {}
        NP = H // 2

        def do_qkv(j):
            parts = []
            for wi in range(3):
                toks, mems = [], []
                for h in (2 * j, 2 * j + 1):
                    y = _dot(xs, _w(wqkv[wi * H + h]))
                    toks.append(ring[wi * H + h, pl.ds(rpos, SEG), :])
                    for g in range(3):
                        ring[wi * H + h, pl.ds(wpos[g], 8), :] = (
                            y[8 + 8 * g:16 + 8 * g].astype(BF16))
                    mems.append(y[0:8])
                mpart = jnp.concatenate(mems, axis=0).astype(BF16)
                parts.append(jnp.concatenate(toks + [mpart], axis=0))
            qkv[j] = parts

        def do_scores(j):
            q, k, _ = qkv[j]
            sc = jax.lax.dot_general(q, k, (((1,), (1,)), ((), ())),
                                     preferred_element_type=F32) + bias
            mx = jnp.max(sc, axis=-1, keepdims=True)
            pe = jnp.exp2((sc - mx) * exp_c)
            inv = _recip(jnp.sum(pe, axis=-1, keepdims=True))
            soft[j] = (pe.astype(BF16), inv)

        def do_pv(j):
            pe, inv = soft[j]
            o = _dot(pe, qkv[j][2]) * inv
            for i, h in enumerate((2 * j, 2 * j + 1)):
                oprev = obuf[h, pl.ds(ord_, TPS), :].astype(F32)
                obuf[h, pl.ds(opos, SEG), :] = (
                    o[i * SEG:(i + 1) * SEG].astype(BF16))
                om = o[2 * SEG + i * M:2 * SEG + (i + 1) * M]
                lhs_o[h] = jnp.concatenate([om, oprev], axis=0).astype(BF16)

        def do_wo(h0, h1):
            la = jnp.concatenate([lhs_o[h] for h in range(h0, h1)], axis=1)
            return _dot(la, _w(wo[h0 * E // 2:h1 * E // 2, :]))

        for i in range(NP):
            do_qkv(i)
            if i - LAG_S >= 0:
                do_scores(i - LAG_S)
            if i - LAG_S - LAG_P >= 0:
                do_pv(i - LAG_S - LAG_P)
        res = None
        for kind, a, b in TAIL:
            if kind == 's':
                do_scores(a)
            elif kind == 'p':
                do_pv(a)
            else:
                r = do_wo(a, b)
                res = r if res is None else res + r
        mem[...] = res[0:M]
        hbuf[pl.ds(ord_, TPS), :] = res[M:]
        return carry

    with jax.named_scope('ph2_steps'):
        jax.lax.fori_loop(0, NSEG, step, 0)

    NT = S - OTAIL
    def wo_tail(j, carry):
        cs = pl.ds(pl.multiple_of(j * 128, 128), 128)
        lo_ = jnp.concatenate([obuf[h, OTAIL - 8:S, :] for h in range(H)], axis=1)
        hbuf[OTAIL - 8:S, cs] = _dot(lo_, _w(wo[:, cs]))
        return carry

    with jax.named_scope('ph3_wo'):
        jax.lax.fori_loop(0, D // 128, wo_tail, 0)

    for i in range(4):
        w_copy(i).wait()

    h1buf[0:8, :] = jnp.zeros((8, D), F32)
    h1buf[S + 8:S + 16, :] = jnp.zeros((8, D), F32)

    def pass1(c, carry):
        r = pl.ds(pl.multiple_of(c * CH, CH), CH)
        hh = xbuf[r, :].astype(F32) + hbuf[r, :]
        hbuf[r, :] = hh
        t = _ln(_ln(hh)).astype(BF16)
        h1buf[pl.ds(pl.multiple_of(c * CH + 8, 8), CH), :] = _gelu(
            _dot(t, _w(w1[...])))
        return carry

    with jax.named_scope('ph3_pass1'):
        jax.lax.fori_loop(0, S // CH, pass1, 0)

    def out_copy(c):
        r = pl.ds(pl.multiple_of(c * CH, CH), CH)
        return pltpu.make_async_copy(outbuf.at[r, :], out_hbm.at[r, :],
                                     sem_out.at[c])

    def pass2(c, carry):
        r = pl.ds(pl.multiple_of(c * CH, CH), CH)
        win = h1buf[pl.ds(pl.multiple_of(c * CH, 8), CH + 16), :]
        qd = D // 4
        g = jnp.concatenate([
            win[7:7 + CH, 0 * qd:1 * qd],
            win[9:9 + CH, 1 * qd:2 * qd],
            win[6:6 + CH, 2 * qd:3 * qd],
            win[10:10 + CH, 3 * qd:4 * qd]], axis=1).astype(BF16)
        hh = hbuf[r, :]
        x1 = _ln(hh) + _dot(g, _w(w2[...]))
        t = _ln(x1).astype(BF16)
        u = _gelu(_dot(t, _w(w3[...]))).astype(BF16)
        y = _dot(u, _w(w4[...]))
        outbuf[r, :] = (hh + (x1 + y)).astype(BF16)
        out_copy(c).start()
        return carry

    with jax.named_scope('ph3_pass2'):
        jax.lax.fori_loop(0, S // CH, pass2, 0)
    for c in range(S // CH):
        out_copy(c).wait()


@functools.partial(jax.jit, static_argnames=("A_seg_len",))
def pallas_sequential_preLN__memory_aug_recurrent_mem_tr__mixer_s_mlp__prompt_kernel(
    A_x: jax.Array,
    A_mem0: jax.Array,
    A_Wq: jax.Array,
    A_Wk: jax.Array,
    A_Wv: jax.Array,
    A_Wo: jax.Array,
    A_seg_len,
    B_x: jax.Array,
    B_w1: jax.Array,
    B_w2: jax.Array,
    B_w3: jax.Array,
    B_w4: jax.Array,
):
    assert A_seg_len == SEG and A_x.shape == (1, S, D)
    x = A_x.reshape(S, D)
    mem0 = A_mem0.reshape(M, D)
    wq = A_Wq.reshape(D // 2, 2, H, E)
    wk = A_Wk.reshape(D // 2, 2, H, E)
    wv = A_Wv.reshape(D // 2, 2, H, E)
    wo = A_Wo.reshape(H * E, D)

    hbm = pl.BlockSpec(memory_space=pl.ANY)
    vmem = pl.BlockSpec(memory_space=pltpu.VMEM)
    out = pl.pallas_call(
        _kernel,
        out_shape=jax.ShapeDtypeStruct((S, D), BF16),
        in_specs=[hbm, vmem] + [hbm] * 8,
        out_specs=hbm,
        scratch_shapes=[
            pltpu.VMEM((3 * H, D // 2, E), U32),
            pltpu.VMEM((H * E // 2, D), U32),
            pltpu.VMEM((D // 2, D), U32),
            pltpu.VMEM((D // 2, D), U32),
            pltpu.VMEM((D // 2, FF), U32),
            pltpu.VMEM((FF // 2, D), U32),
            pltpu.VMEM((S, D), BF16),
            pltpu.VMEM((S, D), BF16),
            pltpu.VMEM((3 * H, RING, E), BF16),
            pltpu.VMEM((H, S, E), BF16),
            pltpu.VMEM((S, D), F32),
            pltpu.VMEM((M, D), F32),
            pltpu.VMEM((S + 16, D), F32),
            pltpu.VMEM((S, D), BF16),
            pltpu.SemaphoreType.DMA((2,)),
            pltpu.SemaphoreType.DMA((H // 2,)),
            pltpu.SemaphoreType.DMA((8,)),
            pltpu.SemaphoreType.DMA((4,)),
            pltpu.SemaphoreType.DMA((S // CH,)),
        ],
        compiler_params=pltpu.CompilerParams(
            vmem_limit_bytes=126 * 1024 * 1024),
    )(x, mem0, wq, wk, wv, wo, B_w1, B_w2, B_w3, B_w4)
    return out.reshape(1, S, D)
```

```python
import functools

import jax
import jax.numpy as jnp
import jax.experimental.pallas as pl
import jax.experimental.pallas.tpu as pltpu

F32 = jnp.float32
BF16 = jnp.bfloat16
U32 = jnp.uint32

S = 2048
D = 1024
H = 32
E = 128
M = 8
SEG = 32
NSEG = S // SEG
FF = 3584
TPS = 24
P0 = S - TPS * (NSEG - 1)
PPAD = 544
RING = 576
OTAIL = TPS * (NSEG - 1)
CH = 256
HC = CH // 2
EPS = 1e-5
LAG_S = 1
LAG_P = 2
TAIL = (('w', 0, 8), ('p', 13, 0), ('s', 15, 0), ('w', 8, 16), ('p', 14, 0),
        ('w', 16, 24), ('p', 15, 0), ('w', 24, 28), ('w', 28, 32))
NEG = -1000000000.0


def _ln(x):
    m = jnp.mean(x, axis=-1, keepdims=True)
    xc = x - m
    v = jnp.mean(xc * xc, axis=-1, keepdims=True)
    return xc * jax.lax.rsqrt(v + EPS)


def _recip(x):
    r = pl.reciprocal(x, approx=True)
    return r * (2.0 - x * r)


def _gelu(x):
    return jax.nn.gelu(x, approximate=True)


def _dot(a, b):
    return jnp.dot(a, b, preferred_element_type=F32)


def _w(u32_val):
    return pltpu.bitcast(u32_val, BF16)


def _kernel(x_hbm, mem0_ref, wq_hbm, wk_hbm, wv_hbm, wo_hbm, w1_hbm, w2_hbm,
            w3_hbm, w4_hbm, out_hbm,
            wqkv, wo, w1, w2, w3, w4, xbuf, lnx, ring, obuf, abuf, mem, h1buf,
            outbuf, sem_x, sem_qkv, sem_wo, sem_w, sem_out):
    def x_copy(i):
        lo, n = ((0, PPAD), (PPAD, S - PPAD))[i]
        return pltpu.make_async_copy(x_hbm.at[pl.ds(lo, n), :],
                                     xbuf.at[pl.ds(lo, n), :], sem_x.at[i])

    def qkv_copies(p):
        cps = []
        for wi, w_hbm in enumerate((wq_hbm, wk_hbm, wv_hbm)):
            wu = w_hbm.bitcast(U32)
            for par in range(2):
                cps.append(pltpu.make_async_copy(
                    wu.at[:, par, p, :], wqkv.at[wi * H + 2 * p + par],
                    sem_qkv.at[p]))
        return cps

    def w_copy(i):
        src, dst = ((w1_hbm, w1), (w2_hbm, w2), (w3_hbm, w3), (w4_hbm, w4))[i]
        return pltpu.make_async_copy(src.bitcast(U32), dst, sem_w.at[i])

    WO_PIECES = 8
    WO_ROWS = H * E // 2 // WO_PIECES

    def wo_copy(i):
        r = pl.ds(pl.multiple_of(i * WO_ROWS, WO_ROWS), WO_ROWS)
        return pltpu.make_async_copy(wo_hbm.bitcast(U32).at[r, :], wo.at[r, :],
                                     sem_wo.at[i])

    x_copy(0).start()
    for c in qkv_copies(0):
        c.start(priority=1)

    mem[...] = mem0_ref[...].astype(F32)
    obuf[:, 0:TPS, :] = jnp.zeros((H, TPS, E), BF16)

    x_copy(0).wait()
    lnx[...] = _ln(xbuf[0:PPAD, :].astype(F32)).astype(BF16)

    def prologue(p, carry):
        for c in qkv_copies(p):
            c.wait()

        @pl.when(p == 0)
        def _():
            for c in qkv_copies(1):
                c.start()

        @pl.when(p + 2 < H // 2)
        def _():
            for c in qkv_copies(p + 2):
                c.start()

        @pl.when((p >= 2) & (p < 2 + WO_PIECES))
        def _():
            wo_copy(p - 2).start()

        @pl.when(p == 10)
        def _():
            x_copy(1).start()

        xp = lnx[...]
        for wi in range(3):
            s0 = wi * H + 2 * p
            a = wqkv[s0]
            b = wqkv[s0 + 1]
            c0 = (a & jnp.uint32(0xFFFF)) | (b << 16)
            c1 = (a >> 16) | (b & jnp.uint32(0xFFFF0000))
            wqkv[s0] = c0
            wqkv[s0 + 1] = c1
            ring[s0, 0:PPAD, :] = _dot(xp, _w(c0)).astype(BF16)
            ring[s0 + 1, 0:PPAD, :] = _dot(xp, _w(c1)).astype(BF16)
        return carry

    with jax.named_scope('ph1_prologue'):
        jax.lax.fori_loop(0, H // 2, prologue, 0)

    x_copy(1).wait()
    for i in range(WO_PIECES):
        wo_copy(i).wait()
    for i in range(4):
        w_copy(i).start()

    LP = 2 * (SEG + M)
    row = jax.lax.broadcasted_iota(jnp.int32, (LP, LP), 0)
    col = jax.lax.broadcasted_iota(jnp.int32, (LP, LP), 1)

    def head_of(i):
        return jnp.where(i < 2 * SEG, i // SEG, (i - 2 * SEG) // M)

    same_head = head_of(row) == head_of(col)
    allowed = same_head & ((col >= 2 * SEG) | (row >= 2 * SEG)
                           | (col % SEG <= row % SEG))
    scale = E ** (-0.5)
    bias = jnp.where(allowed, 0.0,
                     jnp.where(same_head, NEG / scale, -jnp.inf)).astype(F32)
    exp_c = scale * 1.4426950408889634

    def step_tokens(s):
        t0 = pl.multiple_of(jnp.minimum(P0 + TPS * s, S - TPS), 8)
        return t0, _ln(xbuf[pl.ds(t0, TPS), :].astype(F32))

    def step(s, tok):
        t0, tok_next = step_tokens(s + 1)
        t0 = pl.multiple_of(jnp.minimum(P0 + TPS * s, S - TPS), 8)
        xs = jnp.concatenate([mem[...], tok], axis=0).astype(BF16)
        wpos = [pl.multiple_of((t0 + 8 * g) % RING, 8) for g in range(3)]
        rpos = pl.multiple_of((SEG * s) % RING, SEG)
        opos = pl.multiple_of(SEG * s, SEG)
        ord_ = pl.multiple_of(jnp.maximum(s - 1, 0) * TPS, 8)
        qkv = {}
        soft = {}
        lhs_o = {}
        NP = H // 2

        def do_qkv(j):
            parts = []
            for wi in range(3):
                toks, mems = [], []
                for h in (2 * j, 2 * j + 1):
                    y = _dot(xs, _w(wqkv[wi * H + h]))
                    toks.append(ring[wi * H + h, pl.ds(rpos, SEG), :])
                    for g in range(3):
                        ring[wi * H + h, pl.ds(wpos[g], 8), :] = (
                            y[8 + 8 * g:16 + 8 * g].astype(BF16))
                    mems.append(y[0:8])
                mpart = jnp.concatenate(mems, axis=0).astype(BF16)
                parts.append(jnp.concatenate(toks + [mpart], axis=0))
            qkv[j] = parts

        def do_scores(j):
            q, k, _ = qkv[j]
            sc = jax.lax.dot_general(q, k, (((1,), (1,)), ((), ())),
                                     preferred_element_type=F32) + bias
            mx = jnp.max(sc, axis=-1, keepdims=True)
            pe = jnp.exp2((sc - mx) * exp_c)
            inv = _recip(jnp.sum(pe, axis=-1, keepdims=True))
            soft[j] = (pe.astype(BF16), inv)

        def do_pv(j):
            pe, inv = soft[j]
            o = _dot(pe, qkv[j][2]) * inv
            for i, h in enumerate((2 * j, 2 * j + 1)):
                oprev = obuf[h, pl.ds(ord_, TPS), :].astype(F32)
                obuf[h, pl.ds(opos, SEG), :] = (
                    o[i * SEG:(i + 1) * SEG].astype(BF16))
                om = o[2 * SEG + i * M:2 * SEG + (i + 1) * M]
                lhs_o[h] = jnp.concatenate([om, oprev], axis=0).astype(BF16)

        def do_wo(h0, h1):
            la = jnp.concatenate([lhs_o[h] for h in range(h0, h1)], axis=1)
            return _dot(la, _w(wo[h0 * E // 2:h1 * E // 2, :]))

        for i in range(NP):
            do_qkv(i)
            if i - LAG_S >= 0:
                do_scores(i - LAG_S)
            if i - LAG_S - LAG_P >= 0:
                do_pv(i - LAG_S - LAG_P)
        res = None
        for kind, a, b in TAIL:
            if kind == 's':
                do_scores(a)
            elif kind == 'p':
                do_pv(a)
            else:
                r = do_wo(a, b)
                res = r if res is None else res + r
        mem[...] = res[0:M]
        abuf[pl.ds(ord_, TPS), :] = res[M:]
        return tok_next

    with jax.named_scope('ph2_steps'):
        jax.lax.fori_loop(0, NSEG, step, step_tokens(0)[1])

    NT = S - OTAIL
    def wo_tail(j, carry):
        cs = pl.ds(pl.multiple_of(j * 128, 128), 128)
        lo_ = jnp.concatenate([obuf[h, OTAIL - 8:S, :] for h in range(H)], axis=1)
        abuf[OTAIL - 8:S, cs] = _dot(lo_, _w(wo[:, cs]))
        return carry

    with jax.named_scope('ph3_wo'):
        jax.lax.fori_loop(0, D // 128, wo_tail, 0)

    for i in range(4):
        w_copy(i).wait()

    h1buf[0:8, :] = jnp.zeros((8, D), F32)
    h1buf[S + 8:S + 16, :] = jnp.zeros((8, D), F32)

    def resid(r):
        return xbuf[r, :].astype(F32) + abuf[r, :]

    def pass1_input(c):
        r = pl.ds(pl.multiple_of(c * CH, CH), CH)
        return _ln(_ln(resid(r))).astype(BF16)

    def pass1(c, t):
        y = _dot(t, _w(w1[...]))
        t_next = pass1_input(jnp.minimum(c + 1, S // CH - 1))
        h1buf[pl.ds(pl.multiple_of(c * CH + 8, 8), CH), :] = _gelu(y)
        return t_next

    with jax.named_scope('ph3_pass1'):
        jax.lax.fori_loop(0, S // CH, pass1, pass1_input(0))

    def out_copy(c):
        r = pl.ds(pl.multiple_of(c * HC, HC), HC)
        return pltpu.make_async_copy(outbuf.at[r, :], out_hbm.at[r, :],
                                     sem_out.at[c])

    def shifted(c0):
        win = h1buf[pl.ds(pl.multiple_of(c0, 8), HC + 16), :]
        qd = D // 4
        return jnp.concatenate([
            win[7:7 + HC, 0 * qd:1 * qd],
            win[9:9 + HC, 1 * qd:2 * qd],
            win[6:6 + HC, 2 * qd:3 * qd],
            win[10:10 + HC, 3 * qd:4 * qd]], axis=1).astype(BF16)

    def pass2(c, carry):
        halves = (2 * c, 2 * c + 1)
        rows = [pl.ds(pl.multiple_of(i * HC, HC), HC) for i in halves]
        hs = [_dot(shifted(i * HC), _w(w2[...])) for i in halves]
        hh = [resid(r) for r in rows]
        x1 = [_ln(h) + d for h, d in zip(hh, hs)]
        u = [_gelu(_dot(_ln(v).astype(BF16), _w(w3[...]))).astype(BF16)
             for v in x1]
        for i in range(2):
            y = _dot(u[i], _w(w4[...]))
            outbuf[rows[i], :] = (hh[i] + (x1[i] + y)).astype(BF16)
            out_copy(halves[i]).start()
        return carry

    with jax.named_scope('ph3_pass2'):
        jax.lax.fori_loop(0, S // CH, pass2, 0)
    for c in range(S // HC):
        out_copy(c).wait()


@functools.partial(jax.jit, static_argnames=("A_seg_len",))
def pallas_sequential_preLN__memory_aug_recurrent_mem_tr__mixer_s_mlp__prompt_kernel(
    A_x: jax.Array,
    A_mem0: jax.Array,
    A_Wq: jax.Array,
    A_Wk: jax.Array,
    A_Wv: jax.Array,
    A_Wo: jax.Array,
    A_seg_len,
    B_x: jax.Array,
    B_w1: jax.Array,
    B_w2: jax.Array,
    B_w3: jax.Array,
    B_w4: jax.Array,
):
    assert A_seg_len == SEG and A_x.shape == (1, S, D)
    x = A_x.reshape(S, D)
    mem0 = A_mem0.reshape(M, D)
    wq = A_Wq.reshape(D // 2, 2, H, E)
    wk = A_Wk.reshape(D // 2, 2, H, E)
    wv = A_Wv.reshape(D // 2, 2, H, E)
    wo = A_Wo.reshape(H * E, D)

    hbm = pl.BlockSpec(memory_space=pl.ANY)
    vmem = pl.BlockSpec(memory_space=pltpu.VMEM)
    out = pl.pallas_call(
        _kernel,
        out_shape=jax.ShapeDtypeStruct((S, D), BF16),
        in_specs=[hbm, vmem] + [hbm] * 8,
        out_specs=hbm,
        scratch_shapes=[
            pltpu.VMEM((3 * H, D // 2, E), U32),
            pltpu.VMEM((H * E // 2, D), U32),
            pltpu.VMEM((D // 2, D), U32),
            pltpu.VMEM((D // 2, D), U32),
            pltpu.VMEM((D // 2, FF), U32),
            pltpu.VMEM((FF // 2, D), U32),
            pltpu.VMEM((S, D), BF16),
            pltpu.VMEM((PPAD, D), BF16),
            pltpu.VMEM((3 * H, RING, E), BF16),
            pltpu.VMEM((H, S, E), BF16),
            pltpu.VMEM((S, D), F32),
            pltpu.VMEM((M, D), F32),
            pltpu.VMEM((S + 16, D), F32),
            pltpu.VMEM((S, D), BF16),
            pltpu.SemaphoreType.DMA((2,)),
            pltpu.SemaphoreType.DMA((H // 2,)),
            pltpu.SemaphoreType.DMA((8,)),
            pltpu.SemaphoreType.DMA((4,)),
            pltpu.SemaphoreType.DMA((S // HC,)),
        ],
        compiler_params=pltpu.CompilerParams(
            vmem_limit_bytes=126 * 1024 * 1024),
    )(x, mem0, wq, wk, wv, wo, B_w1, B_w2, B_w3, B_w4)
    return out.reshape(1, S, D)
```

```python
import functools

import jax
import jax.numpy as jnp
import jax.experimental.pallas as pl
import jax.experimental.pallas.tpu as pltpu

F32 = jnp.float32
BF16 = jnp.bfloat16
U32 = jnp.uint32

S = 2048
D = 1024
H = 32
E = 128
M = 8
SEG = 32
NSEG = S // SEG
FF = 3584
TPS = 24
P0 = S - TPS * (NSEG - 1)
PPAD = 544
RING = 576
OTAIL = TPS * (NSEG - 1)
CH = 256
HC = CH // 2
EPS = 1e-5
STEP_UNROLL = 2
LAG_S = 1
LAG_P = 2
TAIL = (('w', 0, 8), ('p', 13, 0), ('s', 15, 0), ('w', 8, 16), ('p', 14, 0),
        ('w', 16, 24), ('p', 15, 0), ('w', 24, 28), ('w', 28, 32))
NEG = -1000000000.0


def _ln(x):
    m = jnp.mean(x, axis=-1, keepdims=True)
    xc = x - m
    v = jnp.mean(xc * xc, axis=-1, keepdims=True)
    return xc * jax.lax.rsqrt(v + EPS)


def _recip(x):
    r = pl.reciprocal(x, approx=True)
    return r * (2.0 - x * r)


def _gelu(x):
    return jax.nn.gelu(x, approximate=True)


def _dot(a, b):
    return jnp.dot(a, b, preferred_element_type=F32)


def _w(u32_val):
    return pltpu.bitcast(u32_val, BF16)


def _kernel(x_hbm, mem0_ref, wq_hbm, wk_hbm, wv_hbm, wo_hbm, w1_hbm, w2_hbm,
            w3_hbm, w4_hbm, out_hbm,
            wqkv, wo, w1, w2, w3, w4, xbuf, lnx, ring, obuf, abuf, mem, h1buf,
            outbuf, sem_x, sem_qkv, sem_wo, sem_w, sem_out):
    def x_copy(i):
        lo, n = ((0, PPAD), (PPAD, S - PPAD))[i]
        return pltpu.make_async_copy(x_hbm.at[pl.ds(lo, n), :],
                                     xbuf.at[pl.ds(lo, n), :], sem_x.at[i])

    def qkv_copies(p):
        cps = []
        for wi, w_hbm in enumerate((wq_hbm, wk_hbm, wv_hbm)):
            wu = w_hbm.bitcast(U32)
            for par in range(2):
                cps.append(pltpu.make_async_copy(
                    wu.at[:, par, p, :], wqkv.at[wi * H + 2 * p + par],
                    sem_qkv.at[p]))
        return cps

    def w_copy(i):
        src, dst = ((w1_hbm, w1), (w2_hbm, w2), (w3_hbm, w3), (w4_hbm, w4))[i]
        return pltpu.make_async_copy(src.bitcast(U32), dst, sem_w.at[i])

    WO_PIECES = 8
    WO_ROWS = H * E // 2 // WO_PIECES

    def wo_copy(i):
        r = pl.ds(pl.multiple_of(i * WO_ROWS, WO_ROWS), WO_ROWS)
        return pltpu.make_async_copy(wo_hbm.bitcast(U32).at[r, :], wo.at[r, :],
                                     sem_wo.at[i])

    x_copy(0).start()
    for c in qkv_copies(0):
        c.start(priority=1)

    mem[...] = mem0_ref[...].astype(F32)
    obuf[:, 0:TPS, :] = jnp.zeros((H, TPS, E), BF16)

    x_copy(0).wait()
    lnx[...] = _ln(xbuf[0:PPAD, :].astype(F32)).astype(BF16)

    def prologue(p, carry):
        for c in qkv_copies(p):
            c.wait()

        @pl.when(p == 0)
        def _():
            for c in qkv_copies(1):
                c.start()

        @pl.when(p + 2 < H // 2)
        def _():
            for c in qkv_copies(p + 2):
                c.start()

        @pl.when((p >= 2) & (p < 2 + WO_PIECES))
        def _():
            wo_copy(p - 2).start()

        @pl.when(p == 10)
        def _():
            x_copy(1).start()

        xp = lnx[...]
        for wi in range(3):
            s0 = wi * H + 2 * p
            a = wqkv[s0]
            b = wqkv[s0 + 1]
            c0 = (a & jnp.uint32(0xFFFF)) | (b << 16)
            c1 = (a >> 16) | (b & jnp.uint32(0xFFFF0000))
            wqkv[s0] = c0
            wqkv[s0 + 1] = c1
            ring[s0, 0:PPAD, :] = _dot(xp, _w(c0)).astype(BF16)
            ring[s0 + 1, 0:PPAD, :] = _dot(xp, _w(c1)).astype(BF16)
        return carry

    with jax.named_scope('ph1_prologue'):
        jax.lax.fori_loop(0, H // 2, prologue, 0)

    x_copy(1).wait()
    for i in range(WO_PIECES):
        wo_copy(i).wait()
    for i in range(4):
        w_copy(i).start()

    LP = 2 * (SEG + M)
    row = jax.lax.broadcasted_iota(jnp.int32, (LP, LP), 0)
    col = jax.lax.broadcasted_iota(jnp.int32, (LP, LP), 1)

    def head_of(i):
        return jnp.where(i < 2 * SEG, i // SEG, (i - 2 * SEG) // M)

    same_head = head_of(row) == head_of(col)
    allowed = same_head & ((col >= 2 * SEG) | (row >= 2 * SEG)
                           | (col % SEG <= row % SEG))
    scale = E ** (-0.5)
    bias = jnp.where(allowed, 0.0,
                     jnp.where(same_head, NEG / scale, -jnp.inf)).astype(F32)
    exp_c = scale * 1.4426950408889634

    def step_tokens(s):
        t0 = pl.multiple_of(jnp.minimum(P0 + TPS * s, S - TPS), 8)
        return t0, _ln(xbuf[pl.ds(t0, TPS), :].astype(F32))

    def step(s, tok):
        t0, tok_next = step_tokens(s + 1)
        t0 = pl.multiple_of(jnp.minimum(P0 + TPS * s, S - TPS), 8)
        xs = jnp.concatenate([mem[...], tok], axis=0).astype(BF16)
        wpos = [pl.multiple_of((t0 + 8 * g) % RING, 8) for g in range(3)]
        rpos = pl.multiple_of((SEG * s) % RING, SEG)
        opos = pl.multiple_of(SEG * s, SEG)
        ord_ = pl.multiple_of(jnp.maximum(s - 1, 0) * TPS, 8)
        qkv = {}
        soft = {}
        lhs_o = {}
        NP = H // 2

        def do_qkv(j):
            parts = []
            for wi in range(3):
                toks, mems = [], []
                for h in (2 * j, 2 * j + 1):
                    y = _dot(xs, _w(wqkv[wi * H + h]))
                    toks.append(ring[wi * H + h, pl.ds(rpos, SEG), :])
                    for g in range(3):
                        ring[wi * H + h, pl.ds(wpos[g], 8), :] = (
                            y[8 + 8 * g:16 + 8 * g].astype(BF16))
                    mems.append(y[0:8])
                mpart = jnp.concatenate(mems, axis=0).astype(BF16)
                parts.append(jnp.concatenate(toks + [mpart], axis=0))
            qkv[j] = parts

        def do_scores(j):
            q, k, _ = qkv[j]
            sc = jax.lax.dot_general(q, k, (((1,), (1,)), ((), ())),
                                     preferred_element_type=F32) + bias
            mx = jnp.max(sc, axis=-1, keepdims=True)
            pe = jnp.exp2((sc - mx) * exp_c)
            inv = _recip(jnp.sum(pe, axis=-1, keepdims=True))
            soft[j] = (pe.astype(BF16), inv)

        def do_pv(j):
            pe, inv = soft[j]
            o = _dot(pe, qkv[j][2]) * inv
            for i, h in enumerate((2 * j, 2 * j + 1)):
                oprev = obuf[h, pl.ds(ord_, TPS), :].astype(F32)
                obuf[h, pl.ds(opos, SEG), :] = (
                    o[i * SEG:(i + 1) * SEG].astype(BF16))
                om = o[2 * SEG + i * M:2 * SEG + (i + 1) * M]
                lhs_o[h] = jnp.concatenate([om, oprev], axis=0).astype(BF16)

        def do_wo(h0, h1):
            la = jnp.concatenate([lhs_o[h] for h in range(h0, h1)], axis=1)
            return _dot(la, _w(wo[h0 * E // 2:h1 * E // 2, :]))

        for i in range(NP):
            do_qkv(i)
            if i - LAG_S >= 0:
                do_scores(i - LAG_S)
            if i - LAG_S - LAG_P >= 0:
                do_pv(i - LAG_S - LAG_P)
        res = None
        for kind, a, b in TAIL:
            if kind == 's':
                do_scores(a)
            elif kind == 'p':
                do_pv(a)
            else:
                r = do_wo(a, b)
                res = r if res is None else res + r
        mem[...] = res[0:M]
        abuf[pl.ds(ord_, TPS), :] = res[M:]
        return tok_next

    with jax.named_scope('ph2_steps'):
        jax.lax.fori_loop(0, NSEG, step, step_tokens(0)[1], unroll=STEP_UNROLL)

    NT = S - OTAIL
    def wo_tail(j, carry):
        cs = pl.ds(pl.multiple_of(j * 128, 128), 128)
        lo_ = jnp.concatenate([obuf[h, OTAIL - 8:S, :] for h in range(H)], axis=1)
        abuf[OTAIL - 8:S, cs] = _dot(lo_, _w(wo[:, cs]))
        return carry

    with jax.named_scope('ph3_wo'):
        jax.lax.fori_loop(0, D // 128, wo_tail, 0)

    for i in range(4):
        w_copy(i).wait()

    h1buf[0:8, :] = jnp.zeros((8, D), F32)
    h1buf[S + 8:S + 16, :] = jnp.zeros((8, D), F32)

    def resid(r):
        return xbuf[r, :].astype(F32) + abuf[r, :]

    QC = CH // 4

    def pass1_input(q):
        r = pl.ds(pl.multiple_of(q * QC, QC), QC)
        return _ln(_ln(resid(r))).astype(BF16)

    def pass1(c, t):
        for j in range(4):
            q = 4 * c + j
            y = _dot(t, _w(w1[...]))
            t = pass1_input(jnp.minimum(q + 1, S // QC - 1))
            h1buf[pl.ds(pl.multiple_of(q * QC + 8, 8), QC), :] = _gelu(y)
        return t

    with jax.named_scope('ph3_pass1'):
        jax.lax.fori_loop(0, S // CH, pass1, pass1_input(0))

    def out_copy(c):
        r = pl.ds(pl.multiple_of(c * HC, HC), HC)
        return pltpu.make_async_copy(outbuf.at[r, :], out_hbm.at[r, :],
                                     sem_out.at[c])

    def shifted(c0):
        win = h1buf[pl.ds(pl.multiple_of(c0, 8), HC + 16), :]
        qd = D // 4
        return jnp.concatenate([
            win[7:7 + HC, 0 * qd:1 * qd],
            win[9:9 + HC, 1 * qd:2 * qd],
            win[6:6 + HC, 2 * qd:3 * qd],
            win[10:10 + HC, 3 * qd:4 * qd]], axis=1).astype(BF16)

    def pass2(c, carry):
        halves = (2 * c, 2 * c + 1)
        rows = [pl.ds(pl.multiple_of(i * HC, HC), HC) for i in halves]
        hs = [_dot(shifted(i * HC), _w(w2[...])) for i in halves]
        hh = [resid(r) for r in rows]
        x1 = [_ln(h) + d for h, d in zip(hh, hs)]
        u = [_gelu(_dot(_ln(v).astype(BF16), _w(w3[...]))).astype(BF16)
             for v in x1]
        for i in range(2):
            y = _dot(u[i], _w(w4[...]))
            outbuf[rows[i], :] = (hh[i] + (x1[i] + y)).astype(BF16)
            out_copy(halves[i]).start()
        return carry

    with jax.named_scope('ph3_pass2'):
        jax.lax.fori_loop(0, S // CH, pass2, 0)
    for c in range(S // HC):
        out_copy(c).wait()


@functools.partial(jax.jit, static_argnames=("A_seg_len",))
def pallas_sequential_preLN__memory_aug_recurrent_mem_tr__mixer_s_mlp__prompt_kernel(
    A_x: jax.Array,
    A_mem0: jax.Array,
    A_Wq: jax.Array,
    A_Wk: jax.Array,
    A_Wv: jax.Array,
    A_Wo: jax.Array,
    A_seg_len,
    B_x: jax.Array,
    B_w1: jax.Array,
    B_w2: jax.Array,
    B_w3: jax.Array,
    B_w4: jax.Array,
):
    assert A_seg_len == SEG and A_x.shape == (1, S, D)
    x = A_x.reshape(S, D)
    mem0 = A_mem0.reshape(M, D)
    wq = A_Wq.reshape(D // 2, 2, H, E)
    wk = A_Wk.reshape(D // 2, 2, H, E)
    wv = A_Wv.reshape(D // 2, 2, H, E)
    wo = A_Wo.reshape(H * E, D)

    hbm = pl.BlockSpec(memory_space=pl.ANY)
    vmem = pl.BlockSpec(memory_space=pltpu.VMEM)
    out = pl.pallas_call(
        _kernel,
        out_shape=jax.ShapeDtypeStruct((S, D), BF16),
        in_specs=[hbm, vmem] + [hbm] * 8,
        out_specs=hbm,
        scratch_shapes=[
            pltpu.VMEM((3 * H, D // 2, E), U32),
            pltpu.VMEM((H * E // 2, D), U32),
            pltpu.VMEM((D // 2, D), U32),
            pltpu.VMEM((D // 2, D), U32),
            pltpu.VMEM((D // 2, FF), U32),
            pltpu.VMEM((FF // 2, D), U32),
            pltpu.VMEM((S, D), BF16),
            pltpu.VMEM((PPAD, D), BF16),
            pltpu.VMEM((3 * H, RING, E), BF16),
            pltpu.VMEM((H, S, E), BF16),
            pltpu.VMEM((S, D), F32),
            pltpu.VMEM((M, D), F32),
            pltpu.VMEM((S + 16, D), F32),
            pltpu.VMEM((S, D), BF16),
            pltpu.SemaphoreType.DMA((2,)),
            pltpu.SemaphoreType.DMA((H // 2,)),
            pltpu.SemaphoreType.DMA((8,)),
            pltpu.SemaphoreType.DMA((4,)),
            pltpu.SemaphoreType.DMA((S // HC,)),
        ],
        compiler_params=pltpu.CompilerParams(
            vmem_limit_bytes=126 * 1024 * 1024),
    )(x, mem0, wq, wk, wv, wo, B_w1, B_w2, B_w3, B_w4)
    return out.reshape(1, S, D)
```

```python
import functools

import jax
import jax.numpy as jnp
import jax.experimental.pallas as pl
import jax.experimental.pallas.tpu as pltpu

F32 = jnp.float32
BF16 = jnp.bfloat16
U32 = jnp.uint32

S = 2048
D = 1024
H = 32
E = 128
M = 8
SEG = 32
NSEG = S // SEG
FF = 3584
TPS = 24
P0 = S - TPS * NSEG
RING = 544
OTAIL = TPS * NSEG
CH = 256
HC = CH // 2
EPS = 1e-5
STEP_UNROLL = 2
LAG_S = 1
LAG_P = 2
TAIL = (('w', 0, 4), ('s', 15, 0), ('w', 4, 8), ('p', 13, 0), ('w', 8, 16),
        ('p', 14, 0), ('w', 16, 24), ('p', 15, 0), ('w', 24, 30), ('w', 30, 32))
NEG = -1000000000.0


def _ln(x):
    m = jnp.mean(x, axis=-1, keepdims=True)
    xc = x - m
    v = jnp.mean(xc * xc, axis=-1, keepdims=True)
    return xc * jax.lax.rsqrt(v + EPS)


def _recip(x):
    r = pl.reciprocal(x, approx=True)
    return r * (2.0 - x * r)


def _gelu(x):
    return jax.nn.gelu(x, approximate=True)


def _dot(a, b):
    return jnp.dot(a, b, preferred_element_type=F32)


def _w(u32_val):
    return pltpu.bitcast(u32_val, BF16)


def _kernel(x_hbm, mem0_ref, wq_hbm, wk_hbm, wv_hbm, wo_hbm, w1_hbm, w2_hbm,
            w3_hbm, w4_hbm, out_hbm,
            wqkv, wo, w1, w2, w3, w4, xbuf, lnx, ring, obuf, abuf, mem, h1buf,
            outbuf, sem_x, sem_qkv, sem_wo, sem_w, sem_out):
    def x_copy(i):
        lo, n = ((0, P0), (P0, S - P0))[i]
        return pltpu.make_async_copy(x_hbm.at[pl.ds(lo, n), :],
                                     xbuf.at[pl.ds(lo, n), :], sem_x.at[i])

    def qkv_copies(p):
        cps = []
        for wi, w_hbm in enumerate((wq_hbm, wk_hbm, wv_hbm)):
            wu = w_hbm.bitcast(U32)
            for par in range(2):
                cps.append(pltpu.make_async_copy(
                    wu.at[:, par, p, :], wqkv.at[wi * H + 2 * p + par],
                    sem_qkv.at[p]))
        return cps

    def w_copy(i):
        src, dst = ((w1_hbm, w1), (w2_hbm, w2), (w3_hbm, w3), (w4_hbm, w4))[i]
        return pltpu.make_async_copy(src.bitcast(U32), dst, sem_w.at[i])

    WO_PIECES = 8
    WO_ROWS = H * E // 2 // WO_PIECES

    def wo_copy(i):
        r = pl.ds(pl.multiple_of(i * WO_ROWS, WO_ROWS), WO_ROWS)
        return pltpu.make_async_copy(wo_hbm.bitcast(U32).at[r, :], wo.at[r, :],
                                     sem_wo.at[i])

    x_copy(0).start()
    for c in qkv_copies(0):
        c.start(priority=1)

    mem[...] = mem0_ref[...].astype(F32)

    x_copy(0).wait()
    lnx[...] = _ln(xbuf[0:P0, :].astype(F32)).astype(BF16)

    def prologue(p, carry):
        for c in qkv_copies(p):
            c.wait()

        @pl.when(p == 0)
        def _():
            for c in qkv_copies(1):
                c.start()

        @pl.when(p + 2 < H // 2)
        def _():
            for c in qkv_copies(p + 2):
                c.start()

        @pl.when((p >= 2) & (p < 2 + WO_PIECES))
        def _():
            wo_copy(p - 2).start()

        @pl.when(p == 10)
        def _():
            x_copy(1).start()

        xp = lnx[...]
        for wi in range(3):
            s0 = wi * H + 2 * p
            a = wqkv[s0]
            b = wqkv[s0 + 1]
            c0 = (a & jnp.uint32(0xFFFF)) | (b << 16)
            c1 = (a >> 16) | (b & jnp.uint32(0xFFFF0000))
            wqkv[s0] = c0
            wqkv[s0 + 1] = c1
            ring[s0, 0:P0, :] = _dot(xp, _w(c0)).astype(BF16)
            ring[s0 + 1, 0:P0, :] = _dot(xp, _w(c1)).astype(BF16)
        return carry

    with jax.named_scope('ph1_prologue'):
        jax.lax.fori_loop(0, H // 2, prologue, 0)

    x_copy(1).wait()
    for i in range(WO_PIECES):
        wo_copy(i).wait()
    for i in range(4):
        w_copy(i).start()

    LP = 2 * (SEG + M)
    row = jax.lax.broadcasted_iota(jnp.int32, (LP, LP), 0)
    col = jax.lax.broadcasted_iota(jnp.int32, (LP, LP), 1)

    def head_of(i):
        return jnp.where(i < 2 * SEG, i // SEG, (i - 2 * SEG) // M)

    same_head = head_of(row) == head_of(col)
    allowed = same_head & ((col >= 2 * SEG) | (row >= 2 * SEG)
                           | (col % SEG <= row % SEG))
    scale = E ** (-0.5)
    bias = jnp.where(allowed, 0.0,
                     jnp.where(same_head, NEG / scale, -jnp.inf)).astype(F32)
    exp_c = scale * 1.4426950408889634

    def step_tokens(s):
        t0 = pl.multiple_of(jnp.minimum(P0 + TPS * s, S - TPS), 8)
        return t0, _ln(xbuf[pl.ds(t0, TPS), :].astype(F32))

    def step(s, tok):
        _, tok_next = step_tokens(s + 1)
        t0 = pl.multiple_of(P0 + TPS * s, 8)
        xs = jnp.concatenate([mem[...], tok], axis=0).astype(BF16)
        wpos = [pl.multiple_of((t0 + 8 * g) % RING, 8) for g in range(3)]
        rpos = pl.multiple_of((SEG * s) % RING, SEG)
        opos = pl.multiple_of(SEG * s, SEG)
        ord_ = pl.multiple_of(s * TPS, 8)
        qkv = {}
        soft = {}
        lhs_o = {}
        NP = H // 2

        def do_qkv(j):
            parts = []
            for wi in range(3):
                toks, mems = [], []
                for h in (2 * j, 2 * j + 1):
                    y = _dot(xs, _w(wqkv[wi * H + h]))
                    for g in range(3):
                        ring[wi * H + h, pl.ds(wpos[g], 8), :] = (
                            y[8 + 8 * g:16 + 8 * g].astype(BF16))
                    toks.append(ring[wi * H + h, pl.ds(rpos, SEG), :])
                    mems.append(y[0:8])
                mpart = jnp.concatenate(mems, axis=0).astype(BF16)
                parts.append(jnp.concatenate(toks + [mpart], axis=0))
            qkv[j] = parts

        def do_scores(j):
            q, k, _ = qkv[j]
            sc = jax.lax.dot_general(q, k, (((1,), (1,)), ((), ())),
                                     preferred_element_type=F32) + bias
            mx = jnp.max(sc, axis=-1, keepdims=True)
            pe = jnp.exp2((sc - mx) * exp_c)
            inv = _recip(jnp.sum(pe, axis=-1, keepdims=True))
            soft[j] = (pe.astype(BF16), inv)

        def do_pv(j):
            pe, inv = soft[j]
            o = _dot(pe, qkv[j][2]) * inv
            for i, h in enumerate((2 * j, 2 * j + 1)):
                obuf[h, pl.ds(opos, SEG), :] = (
                    o[i * SEG:(i + 1) * SEG].astype(BF16))
                oprev = obuf[h, pl.ds(ord_, TPS), :].astype(F32)
                om = o[2 * SEG + i * M:2 * SEG + (i + 1) * M]
                lhs_o[h] = jnp.concatenate([om, oprev], axis=0).astype(BF16)

        def do_wo(h0, h1):
            la = jnp.concatenate([lhs_o[h] for h in range(h0, h1)], axis=1)
            return _dot(la, _w(wo[h0 * E // 2:h1 * E // 2, :]))

        for i in range(NP):
            do_qkv(i)
            if i - LAG_S >= 0:
                do_scores(i - LAG_S)
            if i - LAG_S - LAG_P >= 0:
                do_pv(i - LAG_S - LAG_P)
        res = None
        for kind, a, b in TAIL:
            if kind == 's':
                do_scores(a)
            elif kind == 'p':
                do_pv(a)
            else:
                r = do_wo(a, b)
                res = r if res is None else res + r
        mem[...] = res[0:M]
        abuf[pl.ds(ord_, TPS), :] = res[M:]
        return tok_next

    with jax.named_scope('ph2_steps'):
        jax.lax.fori_loop(0, NSEG, step, step_tokens(0)[1], unroll=STEP_UNROLL)

    def wo_tail(j, carry):
        cs = pl.ds(pl.multiple_of(j * 128, 128), 128)
        lo_ = jnp.concatenate([obuf[h, OTAIL:S, :] for h in range(H)], axis=1)
        abuf[OTAIL:S, cs] = _dot(lo_, _w(wo[:, cs]))
        return carry

    with jax.named_scope('ph3_wo'):
        jax.lax.fori_loop(0, D // 128, wo_tail, 0)

    for i in range(4):
        w_copy(i).wait()

    h1buf[0:8, :] = jnp.zeros((8, D), F32)
    h1buf[S + 8:S + 16, :] = jnp.zeros((8, D), F32)

    def resid(r):
        return xbuf[r, :].astype(F32) + abuf[r, :]

    QC = CH // 4

    def pass1_input(q):
        r = pl.ds(pl.multiple_of(q * QC, QC), QC)
        return _ln(_ln(resid(r))).astype(BF16)

    def pass1(c, t):
        for j in range(4):
            q = 4 * c + j
            y = _dot(t, _w(w1[...]))
            t = pass1_input(jnp.minimum(q + 1, S // QC - 1))
            h1buf[pl.ds(pl.multiple_of(q * QC + 8, 8), QC), :] = _gelu(y)
        return t

    with jax.named_scope('ph3_pass1'):
        jax.lax.fori_loop(0, S // CH, pass1, pass1_input(0))

    def out_copy(c):
        r = pl.ds(pl.multiple_of(c * HC, HC), HC)
        return pltpu.make_async_copy(outbuf.at[r, :], out_hbm.at[r, :],
                                     sem_out.at[c])

    def shifted(c0):
        win = h1buf[pl.ds(pl.multiple_of(c0, 8), HC + 16), :]
        qd = D // 4
        return jnp.concatenate([
            win[7:7 + HC, 0 * qd:1 * qd],
            win[9:9 + HC, 1 * qd:2 * qd],
            win[6:6 + HC, 2 * qd:3 * qd],
            win[10:10 + HC, 3 * qd:4 * qd]], axis=1).astype(BF16)

    def pass2(c, carry):
        halves = (2 * c, 2 * c + 1)
        rows = [pl.ds(pl.multiple_of(i * HC, HC), HC) for i in halves]
        hs = [_dot(shifted(i * HC), _w(w2[...])) for i in halves]
        hh = [resid(r) for r in rows]
        x1 = [_ln(h) + d for h, d in zip(hh, hs)]
        u = [_gelu(_dot(_ln(v).astype(BF16), _w(w3[...]))).astype(BF16)
             for v in x1]
        for i in range(2):
            y = _dot(u[i], _w(w4[...]))
            outbuf[rows[i], :] = (hh[i] + (x1[i] + y)).astype(BF16)
            out_copy(halves[i]).start()
        return carry

    with jax.named_scope('ph3_pass2'):
        jax.lax.fori_loop(0, S // CH, pass2, 0)
    for c in range(S // HC):
        out_copy(c).wait()


@functools.partial(jax.jit, static_argnames=("A_seg_len",))
def pallas_sequential_preLN__memory_aug_recurrent_mem_tr__mixer_s_mlp__prompt_kernel(
    A_x: jax.Array,
    A_mem0: jax.Array,
    A_Wq: jax.Array,
    A_Wk: jax.Array,
    A_Wv: jax.Array,
    A_Wo: jax.Array,
    A_seg_len,
    B_x: jax.Array,
    B_w1: jax.Array,
    B_w2: jax.Array,
    B_w3: jax.Array,
    B_w4: jax.Array,
):
    assert A_seg_len == SEG and A_x.shape == (1, S, D)
    x = A_x.reshape(S, D)
    mem0 = A_mem0.reshape(M, D)
    wq = A_Wq.reshape(D // 2, 2, H, E)
    wk = A_Wk.reshape(D // 2, 2, H, E)
    wv = A_Wv.reshape(D // 2, 2, H, E)
    wo = A_Wo.reshape(H * E, D)

    hbm = pl.BlockSpec(memory_space=pl.ANY)
    vmem = pl.BlockSpec(memory_space=pltpu.VMEM)
    out = pl.pallas_call(
        _kernel,
        out_shape=jax.ShapeDtypeStruct((S, D), BF16),
        in_specs=[hbm, vmem] + [hbm] * 8,
        out_specs=hbm,
        scratch_shapes=[
            pltpu.VMEM((3 * H, D // 2, E), U32),
            pltpu.VMEM((H * E // 2, D), U32),
            pltpu.VMEM((D // 2, D), U32),
            pltpu.VMEM((D // 2, D), U32),
            pltpu.VMEM((D // 2, FF), U32),
            pltpu.VMEM((FF // 2, D), U32),
            pltpu.VMEM((S, D), BF16),
            pltpu.VMEM((P0, D), BF16),
            pltpu.VMEM((3 * H, RING, E), BF16),
            pltpu.VMEM((H, S, E), BF16),
            pltpu.VMEM((S, D), F32),
            pltpu.VMEM((M, D), F32),
            pltpu.VMEM((S + 16, D), F32),
            pltpu.VMEM((S, D), BF16),
            pltpu.SemaphoreType.DMA((2,)),
            pltpu.SemaphoreType.DMA((H // 2,)),
            pltpu.SemaphoreType.DMA((8,)),
            pltpu.SemaphoreType.DMA((4,)),
            pltpu.SemaphoreType.DMA((S // HC,)),
        ],
        compiler_params=pltpu.CompilerParams(
            vmem_limit_bytes=126 * 1024 * 1024,
            disable_bounds_checks=True),
    )(x, mem0, wq, wk, wv, wo, B_w1, B_w2, B_w3, B_w4)
    return out.reshape(1, S, D)
```

```python
import functools

import jax
import jax.numpy as jnp
import jax.experimental.pallas as pl
import jax.experimental.pallas.tpu as pltpu

F32 = jnp.float32
BF16 = jnp.bfloat16
U32 = jnp.uint32

S = 2048
D = 1024
H = 32
E = 128
M = 8
SEG = 32
NSEG = S // SEG
FF = 3584
TPS = 24
P0 = S - TPS * NSEG
RING = 544
OTAIL = TPS * NSEG
CH = 256
HC = CH // 2
EPS = 1e-5
STEP_UNROLL = 2
LAG_S = 1
LAG_P = 2
TAIL = (('w', 0, 4), ('s', 15, 0), ('w', 4, 8), ('p', 13, 0), ('w', 8, 16),
        ('p', 14, 0), ('w', 16, 24), ('p', 15, 0), ('w', 24, 30), ('w', 30, 32))
NEG = -1000000000.0


def _ln(x):
    m = jnp.mean(x, axis=-1, keepdims=True)
    xc = x - m
    v = jnp.mean(xc * xc, axis=-1, keepdims=True)
    return xc * jax.lax.rsqrt(v + EPS)


def _recip(x):
    r = pl.reciprocal(x, approx=True)
    return r * (2.0 - x * r)


def _gelu(x):
    return jax.nn.gelu(x, approximate=True)


def _dot(a, b):
    return jnp.dot(a, b, preferred_element_type=F32)


def _w(u32_val):
    return pltpu.bitcast(u32_val, BF16)


def _kernel(x_hbm, mem0_ref, wq_hbm, wk_hbm, wv_hbm, wo_hbm, w1_hbm, w2_hbm,
            w3_hbm, w4_hbm, out_hbm,
            wqkv, wo, w1, w2, w3, w4, xbuf, lnx, ring, obuf, abuf, mem, h1buf,
            outbuf, sem_x, sem_qkv, sem_wo, sem_w, sem_out):
    NPAIR = H // 2
    XP = (S - P0) // NPAIR

    def x_head():
        return pltpu.make_async_copy(x_hbm.at[pl.ds(0, P0), :],
                                     xbuf.at[pl.ds(0, P0), :], sem_x.at[0])

    def x_piece(i):
        r = pl.ds(pl.multiple_of(P0 + i * XP, 8), XP)
        return pltpu.make_async_copy(x_hbm.at[r, :], xbuf.at[r, :], sem_x.at[1])

    def qkv_copies(p):
        real = p < NPAIR
        src_p = jnp.minimum(p, NPAIR - 1)
        cps = []
        for wi, w_hbm in enumerate((wq_hbm, wk_hbm, wv_hbm)):
            wu = w_hbm.bitcast(U32)
            for par in range(2):
                slot = jnp.where(real, wi * H + 2 * p + par,
                                 3 * H + (p - NPAIR) * 6 + 2 * wi + par)
                cps.append(pltpu.make_async_copy(
                    wu.at[:, par, src_p, :], wqkv.at[slot], sem_qkv.at[p]))
        return cps

    def w_copy(i):
        src, dst = ((w1_hbm, w1), (w2_hbm, w2), (w3_hbm, w3), (w4_hbm, w4))[i]
        return pltpu.make_async_copy(src.bitcast(U32), dst, sem_w.at[i])

    WO_ROWS = H * E // 2 // NPAIR

    def wo_piece(i):
        r = pl.ds(pl.multiple_of(i * WO_ROWS, WO_ROWS), WO_ROWS)
        return pltpu.make_async_copy(wo_hbm.bitcast(U32).at[r, :], wo.at[r, :],
                                     sem_wo.at[0])

    x_head().start()
    for c in qkv_copies(0):
        c.start(priority=1)

    mem[...] = mem0_ref[...].astype(F32)

    x_head().wait()
    for c in qkv_copies(1):
        c.start(priority=1)
    lnx[...] = _ln(xbuf[0:P0, :].astype(F32)).astype(BF16)

    def prologue(p, carry):
        for c in qkv_copies(p):
            c.wait()

        wo_piece(p).start()
        x_piece(p).start()
        xp = lnx[...]
        for wi in range(3):
            s0 = wi * H + 2 * p
            a = wqkv[s0]
            b = wqkv[s0 + 1]
            c0 = (a & jnp.uint32(0xFFFF)) | (b << 16)
            c1 = (a >> 16) | (b & jnp.uint32(0xFFFF0000))
            wqkv[s0] = c0
            wqkv[s0 + 1] = c1
            ring[s0, 0:P0, :] = _dot(xp, _w(c0)).astype(BF16)
            ring[s0 + 1, 0:P0, :] = _dot(xp, _w(c1)).astype(BF16)

        for c in qkv_copies(p + 2):
            c.start(priority=1)
        return carry

    with jax.named_scope('ph1_prologue'):
        jax.lax.fori_loop(0, NPAIR, prologue, 0)

    for i in range(NPAIR):
        x_piece(i).wait()
        wo_piece(i).wait()
    for i in range(4):
        w_copy(i).start()

    LP = 2 * (SEG + M)
    row = jax.lax.broadcasted_iota(jnp.int32, (LP, LP), 0)
    col = jax.lax.broadcasted_iota(jnp.int32, (LP, LP), 1)

    def head_of(i):
        return jnp.where(i < 2 * SEG, i // SEG, (i - 2 * SEG) // M)

    same_head = head_of(row) == head_of(col)
    allowed = same_head & ((col >= 2 * SEG) | (row >= 2 * SEG)
                           | (col % SEG <= row % SEG))
    scale = E ** (-0.5)
    bias = jnp.where(allowed, 0.0,
                     jnp.where(same_head, NEG / scale, -jnp.inf)).astype(F32)
    exp_c = scale * 1.4426950408889634

    def step_tokens(s):
        t0 = pl.multiple_of(jnp.minimum(P0 + TPS * s, S - TPS), 8)
        return t0, _ln(xbuf[pl.ds(t0, TPS), :].astype(F32))

    def step(s, tok):
        _, tok_next = step_tokens(s + 1)
        t0 = pl.multiple_of(P0 + TPS * s, 8)
        xs = jnp.concatenate([mem[...], tok], axis=0).astype(BF16)
        wpos = [pl.multiple_of((t0 + 8 * g) % RING, 8) for g in range(3)]
        rpos = pl.multiple_of((SEG * s) % RING, SEG)
        opos = pl.multiple_of(SEG * s, SEG)
        ord_ = pl.multiple_of(s * TPS, 8)
        qkv = {}
        soft = {}
        lhs_o = {}
        NP = H // 2

        def do_qkv(j):
            parts = []
            for wi in range(3):
                toks, mems = [], []
                for h in (2 * j, 2 * j + 1):
                    y = _dot(xs, _w(wqkv[wi * H + h]))
                    for g in range(3):
                        ring[wi * H + h, pl.ds(wpos[g], 8), :] = (
                            y[8 + 8 * g:16 + 8 * g].astype(BF16))
                    toks.append(ring[wi * H + h, pl.ds(rpos, SEG), :])
                    mems.append(y[0:8])
                mpart = jnp.concatenate(mems, axis=0).astype(BF16)
                parts.append(jnp.concatenate(toks + [mpart], axis=0))
            qkv[j] = parts

        def do_scores(j):
            q, k, _ = qkv[j]
            sc = jax.lax.dot_general(q, k, (((1,), (1,)), ((), ())),
                                     preferred_element_type=F32) + bias
            mx = jnp.max(sc, axis=-1, keepdims=True)
            pe = jnp.exp2((sc - mx) * exp_c)
            inv = _recip(jnp.sum(pe, axis=-1, keepdims=True))
            soft[j] = (pe.astype(BF16), inv)

        def do_pv(j):
            pe, inv = soft[j]
            o = _dot(pe, qkv[j][2]) * inv
            for i, h in enumerate((2 * j, 2 * j + 1)):
                obuf[h, pl.ds(opos, SEG), :] = (
                    o[i * SEG:(i + 1) * SEG].astype(BF16))
                oprev = obuf[h, pl.ds(ord_, TPS), :].astype(F32)
                om = o[2 * SEG + i * M:2 * SEG + (i + 1) * M]
                lhs_o[h] = jnp.concatenate([om, oprev], axis=0).astype(BF16)

        def do_wo(h0, h1):
            la = jnp.concatenate([lhs_o[h] for h in range(h0, h1)], axis=1)
            return _dot(la, _w(wo[h0 * E // 2:h1 * E // 2, :]))

        for i in range(NP):
            do_qkv(i)
            if i - LAG_S >= 0:
                do_scores(i - LAG_S)
            if i - LAG_S - LAG_P >= 0:
                do_pv(i - LAG_S - LAG_P)
        res = None
        for kind, a, b in TAIL:
            if kind == 's':
                do_scores(a)
            elif kind == 'p':
                do_pv(a)
            else:
                r = do_wo(a, b)
                res = r if res is None else res + r
        mem[...] = res[0:M]
        abuf[pl.ds(ord_, TPS), :] = res[M:]
        return tok_next

    with jax.named_scope('ph2_steps'):
        jax.lax.fori_loop(0, NSEG, step, step_tokens(0)[1], unroll=STEP_UNROLL)

    def wo_tail(j, carry):
        cs = pl.ds(pl.multiple_of(j * 128, 128), 128)
        lo_ = jnp.concatenate([obuf[h, OTAIL:S, :] for h in range(H)], axis=1)
        abuf[OTAIL:S, cs] = _dot(lo_, _w(wo[:, cs]))
        return carry

    with jax.named_scope('ph3_wo'):
        jax.lax.fori_loop(0, D // 128, wo_tail, 0, unroll=2)

    for i in range(4):
        w_copy(i).wait()
    for p in range(NPAIR, NPAIR + 2):
        for c in qkv_copies(p):
            c.wait()

    h1buf[0:8, :] = jnp.zeros((8, D), F32)
    h1buf[S + 8:S + 16, :] = jnp.zeros((8, D), F32)

    def resid(r):
        return xbuf[r, :].astype(F32) + abuf[r, :]

    QC = CH // 4

    def pass1_input(q):
        r = pl.ds(pl.multiple_of(q * QC, QC), QC)
        return _ln(_ln(resid(r))).astype(BF16)

    def pass1(c, t):
        for j in range(4):
            q = 4 * c + j
            y = _dot(t, _w(w1[...]))
            t = pass1_input(jnp.minimum(q + 1, S // QC - 1))
            h1buf[pl.ds(pl.multiple_of(q * QC + 8, 8), QC), :] = _gelu(y)
        return t

    with jax.named_scope('ph3_pass1'):
        jax.lax.fori_loop(0, S // CH, pass1, pass1_input(0))

    def out_copy(c):
        r = pl.ds(pl.multiple_of(c * HC, HC), HC)
        return pltpu.make_async_copy(outbuf.at[r, :], out_hbm.at[r, :],
                                     sem_out.at[c])

    def shifted(c0):
        win = h1buf[pl.ds(pl.multiple_of(c0, 8), HC + 16), :]
        qd = D // 4
        return jnp.concatenate([
            win[7:7 + HC, 0 * qd:1 * qd],
            win[9:9 + HC, 1 * qd:2 * qd],
            win[6:6 + HC, 2 * qd:3 * qd],
            win[10:10 + HC, 3 * qd:4 * qd]], axis=1).astype(BF16)

    def pass2(c, carry):
        halves = (2 * c, 2 * c + 1)
        rows = [pl.ds(pl.multiple_of(i * HC, HC), HC) for i in halves]
        hs = [_dot(shifted(i * HC), _w(w2[...])) for i in halves]
        hh = [resid(r) for r in rows]
        x1 = [_ln(h) + d for h, d in zip(hh, hs)]
        u = [_gelu(_dot(_ln(v).astype(BF16), _w(w3[...]))).astype(BF16)
             for v in x1]
        for i in range(2):
            y = _dot(u[i], _w(w4[...]))
            outbuf[rows[i], :] = (hh[i] + (x1[i] + y)).astype(BF16)
            out_copy(halves[i]).start()
        return carry

    with jax.named_scope('ph3_pass2'):
        jax.lax.fori_loop(0, S // CH, pass2, 0)
    for c in range(S // HC):
        out_copy(c).wait()


@functools.partial(jax.jit, static_argnames=("A_seg_len",))
def pallas_sequential_preLN__memory_aug_recurrent_mem_tr__mixer_s_mlp__prompt_kernel(
    A_x: jax.Array,
    A_mem0: jax.Array,
    A_Wq: jax.Array,
    A_Wk: jax.Array,
    A_Wv: jax.Array,
    A_Wo: jax.Array,
    A_seg_len,
    B_x: jax.Array,
    B_w1: jax.Array,
    B_w2: jax.Array,
    B_w3: jax.Array,
    B_w4: jax.Array,
):
    assert A_seg_len == SEG and A_x.shape == (1, S, D)
    x = A_x.reshape(S, D)
    mem0 = A_mem0.reshape(M, D)
    wq = A_Wq.reshape(D // 2, 2, H, E)
    wk = A_Wk.reshape(D // 2, 2, H, E)
    wv = A_Wv.reshape(D // 2, 2, H, E)
    wo = A_Wo.reshape(H * E, D)

    hbm = pl.BlockSpec(memory_space=pl.ANY)
    vmem = pl.BlockSpec(memory_space=pltpu.VMEM)
    out = pl.pallas_call(
        _kernel,
        out_shape=jax.ShapeDtypeStruct((S, D), BF16),
        in_specs=[hbm, vmem] + [hbm] * 8,
        out_specs=hbm,
        scratch_shapes=[
            pltpu.VMEM((3 * H + 12, D // 2, E), U32),
            pltpu.VMEM((H * E // 2, D), U32),
            pltpu.VMEM((D // 2, D), U32),
            pltpu.VMEM((D // 2, D), U32),
            pltpu.VMEM((D // 2, FF), U32),
            pltpu.VMEM((FF // 2, D), U32),
            pltpu.VMEM((S, D), BF16),
            pltpu.VMEM((P0, D), BF16),
            pltpu.VMEM((3 * H, RING, E), BF16),
            pltpu.VMEM((H, S, E), BF16),
            pltpu.VMEM((S, D), F32),
            pltpu.VMEM((M, D), F32),
            pltpu.VMEM((S + 16, D), F32),
            pltpu.VMEM((S, D), BF16),
            pltpu.SemaphoreType.DMA((2,)),
            pltpu.SemaphoreType.DMA((H // 2 + 2,)),
            pltpu.SemaphoreType.DMA((1,)),
            pltpu.SemaphoreType.DMA((4,)),
            pltpu.SemaphoreType.DMA((S // HC,)),
        ],
        compiler_params=pltpu.CompilerParams(
            vmem_limit_bytes=126 * 1024 * 1024,
            disable_bounds_checks=True),
    )(x, mem0, wq, wk, wv, wo, B_w1, B_w2, B_w3, B_w4)
    return out.reshape(1, S, D)
```

```python
import functools

import jax
import jax.numpy as jnp
import jax.experimental.pallas as pl
import jax.experimental.pallas.tpu as pltpu

F32 = jnp.float32
BF16 = jnp.bfloat16
U32 = jnp.uint32

S = 2048
D = 1024
H = 32
E = 128
M = 8
SEG = 32
NSEG = S // SEG
FF = 3584
TPS = 24
P0 = S - TPS * NSEG
RING = 544
OTAIL = TPS * NSEG
CH = 256
HC = CH // 2
EPS = 1e-5
STEP_UNROLL = 2
LAG_S = 1
LAG_P = 2
TAIL = (('w', 0, 4), ('s', 15, 0), ('w', 4, 8), ('p', 13, 0), ('w', 8, 16),
        ('p', 14, 0), ('w', 16, 24), ('p', 15, 0), ('w', 24, 30), ('w', 30, 32))
NEG = -1000000000.0


def _ln(x):
    m = jnp.mean(x, axis=-1, keepdims=True)
    xc = x - m
    v = jnp.mean(xc * xc, axis=-1, keepdims=True)
    return xc * jax.lax.rsqrt(v + EPS)


def _recip(x):
    r = pl.reciprocal(x, approx=True)
    return r * (2.0 - x * r)


def _gelu(x):
    return jax.nn.gelu(x, approximate=True)


def _dot(a, b):
    return jnp.dot(a, b, preferred_element_type=F32)


def _w(u32_val):
    return pltpu.bitcast(u32_val, BF16)


def _kernel(x_hbm, mem0_ref, wq_hbm, wk_hbm, wv_hbm, wo_hbm, w1_hbm, w2_hbm,
            w3_hbm, w4_hbm, out_hbm,
            wqkv, wo, w1, w2, w3, w4, xbuf, lnx, ring, obuf, abuf, mem, h1buf,
            outbuf, sem_x, sem_qkv, sem_wo, sem_w, sem_out):
    NPAIR = H // 2
    XP = (S - P0) // NPAIR

    def x_head():
        return pltpu.make_async_copy(x_hbm.at[pl.ds(0, P0), :],
                                     xbuf.at[pl.ds(0, P0), :], sem_x.at[0])

    def x_piece(i):
        r = pl.ds(pl.multiple_of(P0 + i * XP, 8), XP)
        return pltpu.make_async_copy(x_hbm.at[r, :], xbuf.at[r, :], sem_x.at[1])

    def qkv_copies(p):
        real = p < NPAIR
        src_p = jnp.minimum(p, NPAIR - 1)
        cps = []
        for wi, w_hbm in enumerate((wq_hbm, wk_hbm, wv_hbm)):
            wu = w_hbm.bitcast(U32)
            for par in range(2):
                slot = jnp.where(real, wi * H + 2 * p + par,
                                 3 * H + (p - NPAIR) * 6 + 2 * wi + par)
                cps.append(pltpu.make_async_copy(
                    wu.at[:, par, src_p, :], wqkv.at[slot], sem_qkv.at[p]))
        return cps

    def w_copy(i):
        src, dst = ((w1_hbm, w1), (w2_hbm, w2), (w3_hbm, w3), (w4_hbm, w4))[i]
        return pltpu.make_async_copy(src.bitcast(U32), dst, sem_w.at[i])

    WO_ROWS = H * E // 2 // NPAIR

    def wo_piece(i):
        r = pl.ds(pl.multiple_of(i * WO_ROWS, WO_ROWS), WO_ROWS)
        return pltpu.make_async_copy(wo_hbm.bitcast(U32).at[r, :], wo.at[r, :],
                                     sem_wo.at[0])

    x_head().start()
    for c in qkv_copies(0):
        c.start(priority=1)

    mem[...] = mem0_ref[...].astype(F32)

    x_head().wait()
    for c in qkv_copies(1):
        c.start(priority=1)
    lnx[...] = _ln(xbuf[0:P0, :].astype(F32)).astype(BF16)

    def prologue(p, carry):
        for c in qkv_copies(p):
            c.wait()

        wo_piece(p).start()
        x_piece(p).start()
        xp = lnx[...]
        for wi in range(3):
            s0 = wi * H + 2 * p
            a = wqkv[s0]
            b = wqkv[s0 + 1]
            c0 = (a & jnp.uint32(0xFFFF)) | (b << 16)
            c1 = (a >> 16) | (b & jnp.uint32(0xFFFF0000))
            wqkv[s0] = c0
            wqkv[s0 + 1] = c1
            ring[s0, 0:P0, :] = _dot(xp, _w(c0)).astype(BF16)
            ring[s0 + 1, 0:P0, :] = _dot(xp, _w(c1)).astype(BF16)

        for c in qkv_copies(p + 2):
            c.start(priority=1)
        return carry

    with jax.named_scope('ph1_prologue'):
        jax.lax.fori_loop(0, NPAIR, prologue, 0)

    for i in range(NPAIR):
        x_piece(i).wait()
        wo_piece(i).wait()
    for i in range(4):
        w_copy(i).start()

    LP = 2 * (SEG + M)
    row = jax.lax.broadcasted_iota(jnp.int32, (LP, LP), 0)
    col = jax.lax.broadcasted_iota(jnp.int32, (LP, LP), 1)

    def head_of(i):
        return jnp.where(i < 2 * SEG, i // SEG, (i - 2 * SEG) // M)

    same_head = head_of(row) == head_of(col)
    allowed = same_head & ((col >= 2 * SEG) | (row >= 2 * SEG)
                           | (col % SEG <= row % SEG))
    scale = E ** (-0.5)
    bias = jnp.where(allowed, 0.0,
                     jnp.where(same_head, NEG / scale, -jnp.inf)).astype(F32)
    exp_c = scale * 1.4426950408889634

    ring_u = ring.bitcast(U32)
    obuf_u = obuf.bitcast(U32)

    def rows16(ref_u, slot, start, n):
        if isinstance(start, int):
            r = pl.ds(start // 2, n // 2)
        else:
            r = pl.ds(pl.multiple_of(start // 2, 8), n // 2)
        return pltpu.bitcast(ref_u[slot, r, :], BF16)

    def step_tokens(s):
        t0 = pl.multiple_of(jnp.minimum(P0 + TPS * s, S - TPS), 8)
        return t0, _ln(xbuf[pl.ds(t0, TPS), :].astype(F32))

    def step(s, tok):
        _, tok_next = step_tokens(s + 1)
        t0 = pl.multiple_of(P0 + TPS * s, 8)
        xs = jnp.concatenate([mem[...], tok], axis=0).astype(BF16)
        wpos = [pl.multiple_of((t0 + 8 * g) % RING, 8) for g in range(3)]
        rpos = pl.multiple_of((SEG * s) % RING, SEG)
        opos = pl.multiple_of(SEG * s, SEG)
        ord_ = pl.multiple_of(s * TPS, 8)
        qkv = {}
        soft = {}
        lhs_o = {}
        NP = H // 2

        def do_qkv(j):
            parts = []
            for wi in range(3):
                toks, mems = [], []
                for h in (2 * j, 2 * j + 1):
                    y = _dot(xs, _w(wqkv[wi * H + h]))
                    for g in range(3):
                        ring[wi * H + h, pl.ds(wpos[g], 8), :] = (
                            y[8 + 8 * g:16 + 8 * g].astype(BF16))
                    toks.append(rows16(ring_u, wi * H + h, rpos, SEG))
                    mems.append(y[0:8])
                mpart = jnp.concatenate(mems, axis=0).astype(BF16)
                parts.append(jnp.concatenate(toks + [mpart], axis=0))
            qkv[j] = parts

        def do_scores(j):
            q, k, _ = qkv[j]
            sc = jax.lax.dot_general(q, k, (((1,), (1,)), ((), ())),
                                     preferred_element_type=F32) + bias
            mx = jnp.max(sc, axis=-1, keepdims=True)
            pe = jnp.exp2((sc - mx) * exp_c)
            inv = _recip(jnp.sum(pe, axis=-1, keepdims=True))
            soft[j] = (pe.astype(BF16), inv)

        def do_pv(j):
            pe, inv = soft[j]
            o = _dot(pe, qkv[j][2]) * inv
            for i, h in enumerate((2 * j, 2 * j + 1)):
                obuf[h, pl.ds(opos, SEG), :] = (
                    o[i * SEG:(i + 1) * SEG].astype(BF16))
                oprev = obuf[h, pl.ds(ord_, TPS), :].astype(F32)
                om = o[2 * SEG + i * M:2 * SEG + (i + 1) * M]
                lhs_o[h] = jnp.concatenate([om, oprev], axis=0).astype(BF16)

        def do_wo(h0, h1):
            la = jnp.concatenate([lhs_o[h] for h in range(h0, h1)], axis=1)
            return _dot(la, _w(wo[h0 * E // 2:h1 * E // 2, :]))

        for i in range(NP):
            do_qkv(i)
            if i - LAG_S >= 0:
                do_scores(i - LAG_S)
            if i - LAG_S - LAG_P >= 0:
                do_pv(i - LAG_S - LAG_P)
        res = None
        for kind, a, b in TAIL:
            if kind == 's':
                do_scores(a)
            elif kind == 'p':
                do_pv(a)
            else:
                r = do_wo(a, b)
                res = r if res is None else res + r
        mem[...] = res[0:M]
        abuf[pl.ds(ord_, TPS), :] = res[M:]
        return tok_next

    with jax.named_scope('ph2_steps'):
        jax.lax.fori_loop(0, NSEG, step, step_tokens(0)[1], unroll=STEP_UNROLL)

    def wo_tail(j, carry):
        cs = pl.ds(pl.multiple_of(j * 128, 128), 128)
        lo_ = jnp.concatenate([rows16(obuf_u, h, OTAIL, S - OTAIL)
                               for h in range(H)], axis=1)
        abuf[OTAIL:S, cs] = _dot(lo_, _w(wo[:, cs]))
        return carry

    with jax.named_scope('ph3_wo'):
        jax.lax.fori_loop(0, D // 128, wo_tail, 0, unroll=2)

    for i in range(4):
        w_copy(i).wait()
    for p in range(NPAIR, NPAIR + 2):
        for c in qkv_copies(p):
            c.wait()

    h1buf[0:8, :] = jnp.zeros((8, D), F32)
    h1buf[S + 8:S + 16, :] = jnp.zeros((8, D), F32)

    def resid(r):
        return xbuf[r, :].astype(F32) + abuf[r, :]

    QC = CH // 4

    def pass1_input(q):
        r = pl.ds(pl.multiple_of(q * QC, QC), QC)
        return _ln(_ln(resid(r))).astype(BF16)

    def pass1(c, t):
        for j in range(4):
            q = 4 * c + j
            y = _dot(t, _w(w1[...]))
            t = pass1_input(jnp.minimum(q + 1, S // QC - 1))
            h1buf[pl.ds(pl.multiple_of(q * QC + 8, 8), QC), :] = _gelu(y)
        return t

    with jax.named_scope('ph3_pass1'):
        jax.lax.fori_loop(0, S // CH, pass1, pass1_input(0))

    def out_copy(c):
        r = pl.ds(pl.multiple_of(c * HC, HC), HC)
        return pltpu.make_async_copy(outbuf.at[r, :], out_hbm.at[r, :],
                                     sem_out.at[c])

    def shifted(c0):
        win = h1buf[pl.ds(pl.multiple_of(c0, 8), HC + 16), :]
        qd = D // 4
        return jnp.concatenate([
            win[7:7 + HC, 0 * qd:1 * qd],
            win[9:9 + HC, 1 * qd:2 * qd],
            win[6:6 + HC, 2 * qd:3 * qd],
            win[10:10 + HC, 3 * qd:4 * qd]], axis=1).astype(BF16)

    def pass2(c, carry):
        halves = (2 * c, 2 * c + 1)
        rows = [pl.ds(pl.multiple_of(i * HC, HC), HC) for i in halves]
        hs = [_dot(shifted(i * HC), _w(w2[...])) for i in halves]
        hh = [resid(r) for r in rows]
        x1 = [_ln(h) + d for h, d in zip(hh, hs)]
        u = [_gelu(_dot(_ln(v).astype(BF16), _w(w3[...]))).astype(BF16)
             for v in x1]
        for i in range(2):
            y = _dot(u[i], _w(w4[...]))
            outbuf[rows[i], :] = (hh[i] + (x1[i] + y)).astype(BF16)
            out_copy(halves[i]).start()
        return carry

    with jax.named_scope('ph3_pass2'):
        jax.lax.fori_loop(0, S // CH, pass2, 0)
    for c in range(S // HC):
        out_copy(c).wait()


@functools.partial(jax.jit, static_argnames=("A_seg_len",))
def pallas_sequential_preLN__memory_aug_recurrent_mem_tr__mixer_s_mlp__prompt_kernel(
    A_x: jax.Array,
    A_mem0: jax.Array,
    A_Wq: jax.Array,
    A_Wk: jax.Array,
    A_Wv: jax.Array,
    A_Wo: jax.Array,
    A_seg_len,
    B_x: jax.Array,
    B_w1: jax.Array,
    B_w2: jax.Array,
    B_w3: jax.Array,
    B_w4: jax.Array,
):
    assert A_seg_len == SEG and A_x.shape == (1, S, D)
    x = A_x.reshape(S, D)
    mem0 = A_mem0.reshape(M, D)
    wq = A_Wq.reshape(D // 2, 2, H, E)
    wk = A_Wk.reshape(D // 2, 2, H, E)
    wv = A_Wv.reshape(D // 2, 2, H, E)
    wo = A_Wo.reshape(H * E, D)

    hbm = pl.BlockSpec(memory_space=pl.ANY)
    vmem = pl.BlockSpec(memory_space=pltpu.VMEM)
    out = pl.pallas_call(
        _kernel,
        out_shape=jax.ShapeDtypeStruct((S, D), BF16),
        in_specs=[hbm, vmem] + [hbm] * 8,
        out_specs=hbm,
        scratch_shapes=[
            pltpu.VMEM((3 * H + 12, D // 2, E), U32),
            pltpu.VMEM((H * E // 2, D), U32),
            pltpu.VMEM((D // 2, D), U32),
            pltpu.VMEM((D // 2, D), U32),
            pltpu.VMEM((D // 2, FF), U32),
            pltpu.VMEM((FF // 2, D), U32),
            pltpu.VMEM((S, D), BF16),
            pltpu.VMEM((P0, D), BF16),
            pltpu.VMEM((3 * H, RING, E), BF16),
            pltpu.VMEM((H, S, E), BF16),
            pltpu.VMEM((S, D), F32),
            pltpu.VMEM((M, D), F32),
            pltpu.VMEM((S + 16, D), F32),
            pltpu.VMEM((S, D), BF16),
            pltpu.SemaphoreType.DMA((2,)),
            pltpu.SemaphoreType.DMA((H // 2 + 2,)),
            pltpu.SemaphoreType.DMA((1,)),
            pltpu.SemaphoreType.DMA((4,)),
            pltpu.SemaphoreType.DMA((S // HC,)),
        ],
        compiler_params=pltpu.CompilerParams(
            vmem_limit_bytes=126 * 1024 * 1024,
            disable_bounds_checks=True),
    )(x, mem0, wq, wk, wv, wo, B_w1, B_w2, B_w3, B_w4)
    return out.reshape(1, S, D)
```

```python
import functools

import jax
import jax.numpy as jnp
import jax.experimental.pallas as pl
import jax.experimental.pallas.tpu as pltpu

F32 = jnp.float32
BF16 = jnp.bfloat16
U32 = jnp.uint32

S = 2048
D = 1024
H = 32
E = 128
M = 8
SEG = 32
NSEG = S // SEG
FF = 3584
TPS = 24
P0 = S - TPS * NSEG
RING = 544
OTAIL = TPS * NSEG
CH = 256
HC = CH // 2
EPS = 1e-5
STEP_UNROLL = 2
LAG_S = 1
LAG_P = 3
MAIN_W = {10: (0, 8), 14: (8, 12)}
TAIL = (('w', 12, 16), ('p', 12, 0), ('s', 15, 0), ('w', 16, 18), ('p', 13, 0),
        ('w', 18, 22), ('p', 14, 0), ('w', 22, 26), ('p', 15, 0), ('w', 26, 30),
        ('w', 30, 32))
NEG = -1000000000.0


def _ln(x):
    m = jnp.mean(x, axis=-1, keepdims=True)
    xc = x - m
    v = jnp.mean(xc * xc, axis=-1, keepdims=True)
    return xc * jax.lax.rsqrt(v + EPS)


def _recip(x):
    r = pl.reciprocal(x, approx=True)
    return r * (2.0 - x * r)


def _gelu(x):
    return jax.nn.gelu(x, approximate=True)


def _dot(a, b):
    return jnp.dot(a, b, preferred_element_type=F32)


def _w(u32_val):
    return pltpu.bitcast(u32_val, BF16)


def _kernel(x_hbm, mem0_ref, wq_hbm, wk_hbm, wv_hbm, wo_hbm, w1_hbm, w2_hbm,
            w3_hbm, w4_hbm, out_hbm,
            wqkv, wo, w1, w2, w3, w4, xbuf, lnx, ring, obuf, abuf, mem, h1buf,
            outbuf, sem_x, sem_qkv, sem_wo, sem_w, sem_out):
    NPAIR = H // 2
    XP = (S - P0) // NPAIR

    def x_head():
        return pltpu.make_async_copy(x_hbm.at[pl.ds(0, P0), :],
                                     xbuf.at[pl.ds(0, P0), :], sem_x.at[0])

    def x_piece(i):
        r = pl.ds(pl.multiple_of(P0 + i * XP, 8), XP)
        return pltpu.make_async_copy(x_hbm.at[r, :], xbuf.at[r, :], sem_x.at[1])

    def qkv_copies(p):
        real = p < NPAIR
        src_p = jnp.minimum(p, NPAIR - 1)
        cps = []
        for wi, w_hbm in enumerate((wq_hbm, wk_hbm, wv_hbm)):
            wu = w_hbm.bitcast(U32)
            for par in range(2):
                slot = jnp.where(real, wi * H + 2 * p + par,
                                 3 * H + (p - NPAIR) * 6 + 2 * wi + par)
                cps.append(pltpu.make_async_copy(
                    wu.at[:, par, src_p, :], wqkv.at[slot], sem_qkv.at[p]))
        return cps

    def w_copy(i):
        src, dst = ((w1_hbm, w1), (w2_hbm, w2), (w3_hbm, w3), (w4_hbm, w4))[i]
        return pltpu.make_async_copy(src.bitcast(U32), dst, sem_w.at[i])

    WO_ROWS = H * E // 2 // NPAIR

    def wo_piece(i):
        r = pl.ds(pl.multiple_of(i * WO_ROWS, WO_ROWS), WO_ROWS)
        return pltpu.make_async_copy(wo_hbm.bitcast(U32).at[r, :], wo.at[r, :],
                                     sem_wo.at[0])

    x_head().start()
    for c in qkv_copies(0):
        c.start(priority=1)

    mem[...] = mem0_ref[...].astype(F32)

    x_head().wait()
    for c in qkv_copies(1):
        c.start(priority=1)
    lnx[...] = _ln(xbuf[0:P0, :].astype(F32)).astype(BF16)

    def prologue(p, carry):
        for c in qkv_copies(p):
            c.wait()

        wo_piece(p).start()
        x_piece(p).start()
        xp = lnx[...]
        for wi in range(3):
            s0 = wi * H + 2 * p
            a = wqkv[s0]
            b = wqkv[s0 + 1]
            c0 = (a & jnp.uint32(0xFFFF)) | (b << 16)
            c1 = (a >> 16) | (b & jnp.uint32(0xFFFF0000))
            wqkv[s0] = c0
            wqkv[s0 + 1] = c1
            ring[s0, 0:P0, :] = _dot(xp, _w(c0)).astype(BF16)
            ring[s0 + 1, 0:P0, :] = _dot(xp, _w(c1)).astype(BF16)

        for c in qkv_copies(p + 2):
            c.start(priority=1)
        return carry

    with jax.named_scope('ph1_prologue'):
        jax.lax.fori_loop(0, NPAIR, prologue, 0)

    for i in range(NPAIR):
        x_piece(i).wait()
        wo_piece(i).wait()
    for i in range(4):
        w_copy(i).start()

    LP = 2 * (SEG + M)
    row = jax.lax.broadcasted_iota(jnp.int32, (LP, LP), 0)
    col = jax.lax.broadcasted_iota(jnp.int32, (LP, LP), 1)

    def head_of(i):
        return jnp.where(i < 2 * SEG, i // SEG, (i - 2 * SEG) // M)

    same_head = head_of(row) == head_of(col)
    allowed = same_head & ((col >= 2 * SEG) | (row >= 2 * SEG)
                           | (col % SEG <= row % SEG))
    scale = E ** (-0.5)
    bias = jnp.where(allowed, 0.0,
                     jnp.where(same_head, NEG / scale, -jnp.inf)).astype(F32)
    exp_c = scale * 1.4426950408889634

    ring_u = ring.bitcast(U32)
    obuf_u = obuf.bitcast(U32)

    def rows16(ref_u, slot, start, n):
        if isinstance(start, int):
            r = pl.ds(start // 2, n // 2)
        else:
            r = pl.ds(pl.multiple_of(start // 2, 8), n // 2)
        return pltpu.bitcast(ref_u[slot, r, :], BF16)

    def step_tokens(s):
        t0 = pl.multiple_of(jnp.minimum(P0 + TPS * s, S - TPS), 8)
        return t0, _ln(xbuf[pl.ds(t0, TPS), :].astype(F32))

    def step(s, tok):
        _, tok_next = step_tokens(s + 1)
        t0 = pl.multiple_of(P0 + TPS * s, 8)
        xs = jnp.concatenate([mem[...], tok], axis=0).astype(BF16)
        wpos = [pl.multiple_of((t0 + 8 * g) % RING, 8) for g in range(3)]
        rpos = pl.multiple_of((SEG * s) % RING, SEG)
        opos = pl.multiple_of(SEG * s, SEG)
        ord_ = pl.multiple_of(s * TPS, 8)
        qkv = {}
        soft = {}
        lhs_o = {}
        NP = H // 2

        def do_qkv(j):
            parts = []
            for wi in range(3):
                toks, mems = [], []
                for h in (2 * j, 2 * j + 1):
                    y = _dot(xs, _w(wqkv[wi * H + h]))
                    for g in range(3):
                        ring[wi * H + h, pl.ds(wpos[g], 8), :] = (
                            y[8 + 8 * g:16 + 8 * g].astype(BF16))
                    toks.append(rows16(ring_u, wi * H + h, rpos, SEG))
                    mems.append(y[0:8])
                mpart = jnp.concatenate(mems, axis=0).astype(BF16)
                parts.append(jnp.concatenate(toks + [mpart], axis=0))
            qkv[j] = parts

        def do_scores(j):
            q, k, _ = qkv[j]
            sc = jax.lax.dot_general(q, k, (((1,), (1,)), ((), ())),
                                     preferred_element_type=F32) + bias
            mx = jnp.max(sc, axis=-1, keepdims=True)
            pe = jnp.exp2((sc - mx) * exp_c)
            inv = _recip(jnp.sum(pe, axis=-1, keepdims=True))
            soft[j] = (pe.astype(BF16), inv)

        def do_pv(j):
            pe, inv = soft[j]
            o = _dot(pe, qkv[j][2]) * inv
            for i, h in enumerate((2 * j, 2 * j + 1)):
                obuf[h, pl.ds(opos, SEG), :] = (
                    o[i * SEG:(i + 1) * SEG].astype(BF16))
                oprev = obuf[h, pl.ds(ord_, TPS), :].astype(F32)
                om = o[2 * SEG + i * M:2 * SEG + (i + 1) * M]
                lhs_o[h] = jnp.concatenate([om, oprev], axis=0).astype(BF16)

        def do_wo(h0, h1):
            la = jnp.concatenate([lhs_o[h] for h in range(h0, h1)], axis=1)
            return _dot(la, _w(wo[h0 * E // 2:h1 * E // 2, :]))

        res = None
        for i in range(NP):
            do_qkv(i)
            if i - LAG_S >= 0:
                do_scores(i - LAG_S)
            if i - LAG_S - LAG_P >= 0:
                do_pv(i - LAG_S - LAG_P)
            if i in MAIN_W:
                r = do_wo(*MAIN_W[i])
                res = r if res is None else res + r
        for kind, a, b in TAIL:
            if kind == 's':
                do_scores(a)
            elif kind == 'p':
                do_pv(a)
            else:
                res = res + do_wo(a, b)
        mem[...] = res[0:M]
        abuf[pl.ds(ord_, TPS), :] = res[M:]
        return tok_next

    with jax.named_scope('ph2_steps'):
        jax.lax.fori_loop(0, NSEG, step, step_tokens(0)[1], unroll=STEP_UNROLL)

    def wo_tail(j, carry):
        cs = pl.ds(pl.multiple_of(j * 128, 128), 128)
        lo_ = jnp.concatenate([rows16(obuf_u, h, OTAIL, S - OTAIL)
                               for h in range(H)], axis=1)
        abuf[OTAIL:S, cs] = _dot(lo_, _w(wo[:, cs]))
        return carry

    with jax.named_scope('ph3_wo'):
        jax.lax.fori_loop(0, D // 128, wo_tail, 0, unroll=2)

    for i in range(4):
        w_copy(i).wait()
    for p in range(NPAIR, NPAIR + 2):
        for c in qkv_copies(p):
            c.wait()

    h1buf[0:8, :] = jnp.zeros((8, D), F32)
    h1buf[S + 8:S + 16, :] = jnp.zeros((8, D), F32)

    def resid(r):
        return xbuf[r, :].astype(F32) + abuf[r, :]

    QC = CH // 4

    def pass1_input(q):
        r = pl.ds(pl.multiple_of(q * QC, QC), QC)
        return _ln(_ln(resid(r))).astype(BF16)

    def pass1(c, t):
        for j in range(4):
            q = 4 * c + j
            y = _dot(t, _w(w1[...]))
            t = pass1_input(jnp.minimum(q + 1, S // QC - 1))
            h1buf[pl.ds(pl.multiple_of(q * QC + 8, 8), QC), :] = _gelu(y)
        return t

    with jax.named_scope('ph3_pass1'):
        jax.lax.fori_loop(0, S // CH, pass1, pass1_input(0))

    def out_copy(c):
        r = pl.ds(pl.multiple_of(c * HC, HC), HC)
        return pltpu.make_async_copy(outbuf.at[r, :], out_hbm.at[r, :],
                                     sem_out.at[c])

    def shifted(c0):
        win = h1buf[pl.ds(pl.multiple_of(c0, 8), HC + 16), :]
        qd = D // 4
        return jnp.concatenate([
            win[7:7 + HC, 0 * qd:1 * qd],
            win[9:9 + HC, 1 * qd:2 * qd],
            win[6:6 + HC, 2 * qd:3 * qd],
            win[10:10 + HC, 3 * qd:4 * qd]], axis=1).astype(BF16)

    def pass2(c, carry):
        halves = (2 * c, 2 * c + 1)
        rows = [pl.ds(pl.multiple_of(i * HC, HC), HC) for i in halves]
        hs = [_dot(shifted(i * HC), _w(w2[...])) for i in halves]
        hh = [resid(r) for r in rows]
        x1 = [_ln(h) + d for h, d in zip(hh, hs)]
        u = [_gelu(_dot(_ln(v).astype(BF16), _w(w3[...]))).astype(BF16)
             for v in x1]
        for i in range(2):
            y = _dot(u[i], _w(w4[...]))
            outbuf[rows[i], :] = (hh[i] + (x1[i] + y)).astype(BF16)
            out_copy(halves[i]).start()
        return carry

    with jax.named_scope('ph3_pass2'):
        jax.lax.fori_loop(0, S // CH, pass2, 0)
    for c in range(S // HC):
        out_copy(c).wait()


@functools.partial(jax.jit, static_argnames=("A_seg_len",))
def pallas_sequential_preLN__memory_aug_recurrent_mem_tr__mixer_s_mlp__prompt_kernel(
    A_x: jax.Array,
    A_mem0: jax.Array,
    A_Wq: jax.Array,
    A_Wk: jax.Array,
    A_Wv: jax.Array,
    A_Wo: jax.Array,
    A_seg_len,
    B_x: jax.Array,
    B_w1: jax.Array,
    B_w2: jax.Array,
    B_w3: jax.Array,
    B_w4: jax.Array,
):
    assert A_seg_len == SEG and A_x.shape == (1, S, D)
    x = A_x.reshape(S, D)
    mem0 = A_mem0.reshape(M, D)
    wq = A_Wq.reshape(D // 2, 2, H, E)
    wk = A_Wk.reshape(D // 2, 2, H, E)
    wv = A_Wv.reshape(D // 2, 2, H, E)
    wo = A_Wo.reshape(H * E, D)

    hbm = pl.BlockSpec(memory_space=pl.ANY)
    vmem = pl.BlockSpec(memory_space=pltpu.VMEM)
    out = pl.pallas_call(
        _kernel,
        out_shape=jax.ShapeDtypeStruct((S, D), BF16),
        in_specs=[hbm, vmem] + [hbm] * 8,
        out_specs=hbm,
        scratch_shapes=[
            pltpu.VMEM((3 * H + 12, D // 2, E), U32),
            pltpu.VMEM((H * E // 2, D), U32),
            pltpu.VMEM((D // 2, D), U32),
            pltpu.VMEM((D // 2, D), U32),
            pltpu.VMEM((D // 2, FF), U32),
            pltpu.VMEM((FF // 2, D), U32),
            pltpu.VMEM((S, D), BF16),
            pltpu.VMEM((P0, D), BF16),
            pltpu.VMEM((3 * H, RING, E), BF16),
            pltpu.VMEM((H, S, E), BF16),
            pltpu.VMEM((S, D), F32),
            pltpu.VMEM((M, D), F32),
            pltpu.VMEM((S + 16, D), F32),
            pltpu.VMEM((S, D), BF16),
            pltpu.SemaphoreType.DMA((2,)),
            pltpu.SemaphoreType.DMA((H // 2 + 2,)),
            pltpu.SemaphoreType.DMA((1,)),
            pltpu.SemaphoreType.DMA((4,)),
            pltpu.SemaphoreType.DMA((S // HC,)),
        ],
        compiler_params=pltpu.CompilerParams(
            vmem_limit_bytes=126 * 1024 * 1024,
            disable_bounds_checks=True),
    )(x, mem0, wq, wk, wv, wo, B_w1, B_w2, B_w3, B_w4)
    return out.reshape(1, S, D)
```

```python
import functools

import jax
import jax.numpy as jnp
import jax.experimental.pallas as pl
import jax.experimental.pallas.tpu as pltpu

F32 = jnp.float32
BF16 = jnp.bfloat16
U32 = jnp.uint32

S = 2048
D = 1024
H = 32
E = 128
M = 8
SEG = 32
NSEG = S // SEG
FF = 3584
TPS = 24
P0 = S - TPS * NSEG
RING = 544
OTAIL = TPS * NSEG
CH = 256
HC = CH // 2
EPS = 1e-5
STEP_UNROLL = 2
LAG_S = 1
LAG_P = 3
ORDER = 'qkspvw'
MAIN_W = {10: (0, 8), 14: (8, 12)}
TAIL = (('w', 12, 16), ('p', 12, 0), ('s', 15, 0), ('w', 16, 18), ('p', 13, 0),
        ('w', 18, 22), ('p', 14, 0), ('w', 22, 26), ('p', 15, 0), ('w', 26, 30),
        ('w', 30, 32))
NEG = -1000000000.0


def _ln(x):
    m = jnp.mean(x, axis=-1, keepdims=True)
    xc = x - m
    v = jnp.mean(xc * xc, axis=-1, keepdims=True)
    return xc * jax.lax.rsqrt(v + EPS)


def _recip(x):
    r = pl.reciprocal(x, approx=True)
    return r * (2.0 - x * r)


def _gelu(x):
    return jax.nn.gelu(x, approximate=True)


def _dot(a, b):
    return jnp.dot(a, b, preferred_element_type=F32)


def _w(u32_val):
    return pltpu.bitcast(u32_val, BF16)


def _kernel(x_hbm, mem0_ref, wq_hbm, wk_hbm, wv_hbm, wo_hbm, w1_hbm, w2_hbm,
            w3_hbm, w4_hbm, out_hbm,
            wqkv, wo, w1, w2, w3, w4, xbuf, lnx, ring, obuf, abuf, mem, h1buf,
            outbuf, sem_x, sem_qkv, sem_wo, sem_w, sem_out):
    NPAIR = H // 2
    XP = (S - P0) // NPAIR

    def x_head():
        return pltpu.make_async_copy(x_hbm.at[pl.ds(0, P0), :],
                                     xbuf.at[pl.ds(0, P0), :], sem_x.at[0])

    def x_piece(i):
        r = pl.ds(pl.multiple_of(P0 + i * XP, 8), XP)
        return pltpu.make_async_copy(x_hbm.at[r, :], xbuf.at[r, :], sem_x.at[1])

    def qkv_copies(p):
        real = p < NPAIR
        src_p = jnp.minimum(p, NPAIR - 1)
        cps = []
        for wi, w_hbm in enumerate((wq_hbm, wk_hbm, wv_hbm)):
            wu = w_hbm.bitcast(U32)
            for par in range(2):
                slot = jnp.where(real, wi * H + 2 * p + par,
                                 3 * H + (p - NPAIR) * 6 + 2 * wi + par)
                cps.append(pltpu.make_async_copy(
                    wu.at[:, par, src_p, :], wqkv.at[slot], sem_qkv.at[p]))
        return cps

    def w_copy(i):
        src, dst = ((w1_hbm, w1), (w2_hbm, w2), (w3_hbm, w3), (w4_hbm, w4))[i]
        return pltpu.make_async_copy(src.bitcast(U32), dst, sem_w.at[i])

    WO_ROWS = H * E // 2 // NPAIR

    def wo_piece(i):
        r = pl.ds(pl.multiple_of(i * WO_ROWS, WO_ROWS), WO_ROWS)
        return pltpu.make_async_copy(wo_hbm.bitcast(U32).at[r, :], wo.at[r, :],
                                     sem_wo.at[0])

    x_head().start()
    for c in qkv_copies(0):
        c.start(priority=1)

    mem[...] = mem0_ref[...].astype(F32)

    x_head().wait()
    lnx[...] = _ln(xbuf[0:P0, :].astype(F32)).astype(BF16)
    for c in qkv_copies(1):
        c.start(priority=1)

    def prologue(p, carry):
        for c in qkv_copies(p):
            c.wait()

        wo_piece(p).start()
        x_piece(p).start()
        xp = lnx[...]
        for wi in range(3):
            s0 = wi * H + 2 * p
            a = wqkv[s0]
            b = wqkv[s0 + 1]
            c0 = (a & jnp.uint32(0xFFFF)) | (b << 16)
            c1 = (a >> 16) | (b & jnp.uint32(0xFFFF0000))
            wqkv[s0] = c0
            wqkv[s0 + 1] = c1
            ring[s0, 0:P0, :] = _dot(xp, _w(c0)).astype(BF16)
            ring[s0 + 1, 0:P0, :] = _dot(xp, _w(c1)).astype(BF16)

        for c in qkv_copies(p + 2):
            c.start(priority=1)
        return carry

    with jax.named_scope('ph1_prologue'):
        jax.lax.fori_loop(0, NPAIR, prologue, 0)

    for i in range(NPAIR):
        x_piece(i).wait()
        wo_piece(i).wait()
    for i in range(4):
        w_copy(i).start()

    LP = 2 * (SEG + M)
    row = jax.lax.broadcasted_iota(jnp.int32, (LP, LP), 0)
    col = jax.lax.broadcasted_iota(jnp.int32, (LP, LP), 1)

    def head_of(i):
        return jnp.where(i < 2 * SEG, i // SEG, (i - 2 * SEG) // M)

    same_head = head_of(row) == head_of(col)
    allowed = same_head & ((col >= 2 * SEG) | (row >= 2 * SEG)
                           | (col % SEG <= row % SEG))
    scale = E ** (-0.5)
    bias = jnp.where(allowed, 0.0,
                     jnp.where(same_head, NEG / scale, -jnp.inf)).astype(F32)
    exp_c = scale * 1.4426950408889634

    ring_u = ring.bitcast(U32)
    obuf_u = obuf.bitcast(U32)

    def rows16(ref_u, slot, start, n):
        if isinstance(start, int):
            r = pl.ds(start // 2, n // 2)
        else:
            r = pl.ds(pl.multiple_of(start // 2, 8), n // 2)
        return pltpu.bitcast(ref_u[slot, r, :], BF16)

    def step_tokens(s):
        t0 = pl.multiple_of(jnp.minimum(P0 + TPS * s, S - TPS), 8)
        return t0, _ln(xbuf[pl.ds(t0, TPS), :].astype(F32))

    def step(s, tok):
        _, tok_next = step_tokens(s + 1)
        t0 = pl.multiple_of(P0 + TPS * s, 8)
        xs = jnp.concatenate([mem[...], tok], axis=0).astype(BF16)
        wpos = [pl.multiple_of((t0 + 8 * g) % RING, 8) for g in range(3)]
        rpos = pl.multiple_of((SEG * s) % RING, SEG)
        opos = pl.multiple_of(SEG * s, SEG)
        ord_ = pl.multiple_of(s * TPS, 8)
        qkv = {}
        soft = {}
        lhs_o = {}
        NP = H // 2

        def do_proj(j, wi):
            toks, mems = [], []
            for h in (2 * j, 2 * j + 1):
                y = _dot(xs, _w(wqkv[wi * H + h]))
                for g in range(3):
                    ring[wi * H + h, pl.ds(wpos[g], 8), :] = (
                        y[8 + 8 * g:16 + 8 * g].astype(BF16))
                toks.append(rows16(ring_u, wi * H + h, rpos, SEG))
                mems.append(y[0:8])
            mpart = jnp.concatenate(mems, axis=0).astype(BF16)
            qkv.setdefault(j, []).append(
                jnp.concatenate(toks + [mpart], axis=0))

        def do_scores(j):
            q, k, _ = qkv[j]
            sc = jax.lax.dot_general(q, k, (((1,), (1,)), ((), ())),
                                     preferred_element_type=F32) + bias
            mx = jnp.max(sc, axis=-1, keepdims=True)
            pe = jnp.exp2((sc - mx) * exp_c)
            inv = _recip(jnp.sum(pe, axis=-1, keepdims=True))
            soft[j] = (pe.astype(BF16), inv)

        def do_pv(j):
            pe, inv = soft[j]
            o = _dot(pe, qkv[j][2]) * inv
            for i, h in enumerate((2 * j, 2 * j + 1)):
                obuf[h, pl.ds(opos, SEG), :] = (
                    o[i * SEG:(i + 1) * SEG].astype(BF16))
                oprev = obuf[h, pl.ds(ord_, TPS), :].astype(F32)
                om = o[2 * SEG + i * M:2 * SEG + (i + 1) * M]
                lhs_o[h] = jnp.concatenate([om, oprev], axis=0).astype(BF16)

        def do_wo(h0, h1):
            la = jnp.concatenate([lhs_o[h] for h in range(h0, h1)], axis=1)
            return _dot(la, _w(wo[h0 * E // 2:h1 * E // 2, :]))

        res = None
        for i in range(NP):
            for op in ORDER:
                if op in 'qkv':
                    do_proj(i, 'qkv'.index(op))
                elif op == 's' and i - LAG_S >= 0:
                    do_scores(i - LAG_S)
                elif op == 'p' and i - LAG_S - LAG_P >= 0:
                    do_pv(i - LAG_S - LAG_P)
                elif op == 'w' and i in MAIN_W:
                    r = do_wo(*MAIN_W[i])
                    res = r if res is None else res + r
        for kind, a, b in TAIL:
            if kind == 's':
                do_scores(a)
            elif kind == 'p':
                do_pv(a)
            else:
                res = res + do_wo(a, b)
        mem[...] = res[0:M]
        abuf[pl.ds(ord_, TPS), :] = res[M:]
        return tok_next

    with jax.named_scope('ph2_steps'):
        jax.lax.fori_loop(0, NSEG, step, step_tokens(0)[1], unroll=STEP_UNROLL)

    def wo_tail(j, carry):
        cs = pl.ds(pl.multiple_of(j * 128, 128), 128)
        lo_ = jnp.concatenate([rows16(obuf_u, h, OTAIL, S - OTAIL)
                               for h in range(H)], axis=1)
        abuf[OTAIL:S, cs] = _dot(lo_, _w(wo[:, cs]))
        return carry

    with jax.named_scope('ph3_wo'):
        jax.lax.fori_loop(0, D // 128, wo_tail, 0, unroll=2)

    for i in range(4):
        w_copy(i).wait()
    for p in range(NPAIR, NPAIR + 2):
        for c in qkv_copies(p):
            c.wait()

    h1buf[0:8, :] = jnp.zeros((8, D), F32)
    h1buf[S + 8:S + 16, :] = jnp.zeros((8, D), F32)

    def resid(r):
        return xbuf[r, :].astype(F32) + abuf[r, :]

    QC = CH // 4

    def pass1_input(q):
        r = pl.ds(pl.multiple_of(q * QC, QC), QC)
        return _ln(_ln(resid(r))).astype(BF16)

    def pass1(c, t):
        for j in range(4):
            q = 4 * c + j
            y = _dot(t, _w(w1[...]))
            t = pass1_input(jnp.minimum(q + 1, S // QC - 1))
            h1buf[pl.ds(pl.multiple_of(q * QC + 8, 8), QC), :] = _gelu(y)
        return t

    with jax.named_scope('ph3_pass1'):
        jax.lax.fori_loop(0, S // CH, pass1, pass1_input(0))

    def out_copy(c):
        r = pl.ds(pl.multiple_of(c * HC, HC), HC)
        return pltpu.make_async_copy(outbuf.at[r, :], out_hbm.at[r, :],
                                     sem_out.at[c])

    def shifted(c0):
        win = h1buf[pl.ds(pl.multiple_of(c0, 8), HC + 16), :]
        qd = D // 4
        return jnp.concatenate([
            win[7:7 + HC, 0 * qd:1 * qd],
            win[9:9 + HC, 1 * qd:2 * qd],
            win[6:6 + HC, 2 * qd:3 * qd],
            win[10:10 + HC, 3 * qd:4 * qd]], axis=1).astype(BF16)

    def pass2(c, carry):
        halves = (2 * c, 2 * c + 1)
        rows = [pl.ds(pl.multiple_of(i * HC, HC), HC) for i in halves]
        hs = [_dot(shifted(i * HC), _w(w2[...])) for i in halves]
        hh = [resid(r) for r in rows]
        x1 = [_ln(h) + d for h, d in zip(hh, hs)]
        u = [_gelu(_dot(_ln(v).astype(BF16), _w(w3[...]))).astype(BF16)
             for v in x1]
        for i in range(2):
            y = _dot(u[i], _w(w4[...]))
            outbuf[rows[i], :] = (hh[i] + (x1[i] + y)).astype(BF16)
            out_copy(halves[i]).start()
        return carry

    with jax.named_scope('ph3_pass2'):
        jax.lax.fori_loop(0, S // CH, pass2, 0)
    for c in range(S // HC):
        out_copy(c).wait()


@functools.partial(jax.jit, static_argnames=("A_seg_len",))
def pallas_sequential_preLN__memory_aug_recurrent_mem_tr__mixer_s_mlp__prompt_kernel(
    A_x: jax.Array,
    A_mem0: jax.Array,
    A_Wq: jax.Array,
    A_Wk: jax.Array,
    A_Wv: jax.Array,
    A_Wo: jax.Array,
    A_seg_len,
    B_x: jax.Array,
    B_w1: jax.Array,
    B_w2: jax.Array,
    B_w3: jax.Array,
    B_w4: jax.Array,
):
    assert A_seg_len == SEG and A_x.shape == (1, S, D)
    x = A_x.reshape(S, D)
    mem0 = A_mem0.reshape(M, D)
    wq = A_Wq.reshape(D // 2, 2, H, E)
    wk = A_Wk.reshape(D // 2, 2, H, E)
    wv = A_Wv.reshape(D // 2, 2, H, E)
    wo = A_Wo.reshape(H * E, D)

    hbm = pl.BlockSpec(memory_space=pl.ANY)
    vmem = pl.BlockSpec(memory_space=pltpu.VMEM)
    out = pl.pallas_call(
        _kernel,
        out_shape=jax.ShapeDtypeStruct((S, D), BF16),
        in_specs=[hbm, vmem] + [hbm] * 8,
        out_specs=hbm,
        scratch_shapes=[
            pltpu.VMEM((3 * H + 12, D // 2, E), U32),
            pltpu.VMEM((H * E // 2, D), U32),
            pltpu.VMEM((D // 2, D), U32),
            pltpu.VMEM((D // 2, D), U32),
            pltpu.VMEM((D // 2, FF), U32),
            pltpu.VMEM((FF // 2, D), U32),
            pltpu.VMEM((S, D), BF16),
            pltpu.VMEM((P0, D), BF16),
            pltpu.VMEM((3 * H, RING, E), BF16),
            pltpu.VMEM((H, S, E), BF16),
            pltpu.VMEM((S, D), F32),
            pltpu.VMEM((M, D), F32),
            pltpu.VMEM((S + 16, D), F32),
            pltpu.VMEM((S, D), BF16),
            pltpu.SemaphoreType.DMA((2,)),
            pltpu.SemaphoreType.DMA((H // 2 + 2,)),
            pltpu.SemaphoreType.DMA((1,)),
            pltpu.SemaphoreType.DMA((4,)),
            pltpu.SemaphoreType.DMA((S // HC,)),
        ],
        compiler_params=pltpu.CompilerParams(
            vmem_limit_bytes=126 * 1024 * 1024,
            disable_bounds_checks=True),
    )(x, mem0, wq, wk, wv, wo, B_w1, B_w2, B_w3, B_w4)
    return out.reshape(1, S, D)
```

```python
import functools

import jax
import jax.numpy as jnp
import jax.experimental.pallas as pl
import jax.experimental.pallas.tpu as pltpu

F32 = jnp.float32
BF16 = jnp.bfloat16
U32 = jnp.uint32

S = 2048
D = 1024
H = 32
E = 128
M = 8
SEG = 32
NSEG = S // SEG
FF = 3584
TPS = 24
P0 = S - TPS * NSEG
RING = 544
OTAIL = TPS * NSEG
CH = 256
HC = CH // 2
EPS = 1e-5
STEP_UNROLL = 2
LAG_S = 1
LAG_P = 2
ORDER = 'qksvpw'
MAIN_W = {10: (0, 8), 14: (8, 12)}
TAIL = (('w', 12, 14), ('s', 15, 0), ('w', 14, 16), ('p', 13, 0), ('w', 16, 22),
        ('p', 14, 0), ('w', 22, 24), ('p', 15, 0), ('w', 24, 30), ('w', 30, 32))
NEG = -1000000000.0


def _ln(x):
    m = jnp.mean(x, axis=-1, keepdims=True)
    xc = x - m
    v = jnp.mean(xc * xc, axis=-1, keepdims=True)
    return xc * jax.lax.rsqrt(v + EPS)


def _recip(x):
    r = pl.reciprocal(x, approx=True)
    return r * (2.0 - x * r)


def _gelu(x):
    return jax.nn.gelu(x, approximate=True)


def _dot(a, b):
    return jnp.dot(a, b, preferred_element_type=F32)


def _w(u32_val):
    return pltpu.bitcast(u32_val, BF16)


def _kernel(x_hbm, mem0_ref, wq_hbm, wk_hbm, wv_hbm, wo_hbm, w1_hbm, w2_hbm,
            w3_hbm, w4_hbm, out_hbm,
            wqkv, wo, w1, w2, w3, w4, xbuf, lnx, ring, obuf, abuf, mem, h1buf,
            outbuf, sem_x, sem_qkv, sem_wo, sem_w, sem_out):
    NPAIR = H // 2
    XP = (S - P0) // NPAIR

    def x_head():
        return pltpu.make_async_copy(x_hbm.at[pl.ds(0, P0), :],
                                     xbuf.at[pl.ds(0, P0), :], sem_x.at[0])

    def x_piece(i):
        r = pl.ds(pl.multiple_of(P0 + i * XP, 8), XP)
        return pltpu.make_async_copy(x_hbm.at[r, :], xbuf.at[r, :], sem_x.at[1])

    def qkv_copies(p):
        real = p < NPAIR
        src_p = jnp.minimum(p, NPAIR - 1)
        cps = []
        for wi, w_hbm in enumerate((wq_hbm, wk_hbm, wv_hbm)):
            wu = w_hbm.bitcast(U32)
            for par in range(2):
                slot = jnp.where(real, wi * H + 2 * p + par,
                                 3 * H + (p - NPAIR) * 6 + 2 * wi + par)
                cps.append(pltpu.make_async_copy(
                    wu.at[:, par, src_p, :], wqkv.at[slot], sem_qkv.at[p]))
        return cps

    def w_copy(i):
        src, dst = ((w1_hbm, w1), (w2_hbm, w2), (w3_hbm, w3), (w4_hbm, w4))[i]
        return pltpu.make_async_copy(src.bitcast(U32), dst, sem_w.at[i])

    WO_ROWS = H * E // 2 // NPAIR

    def wo_piece(i):
        r = pl.ds(pl.multiple_of(i * WO_ROWS, WO_ROWS), WO_ROWS)
        return pltpu.make_async_copy(wo_hbm.bitcast(U32).at[r, :], wo.at[r, :],
                                     sem_wo.at[0])

    x_head().start()
    for c in qkv_copies(0):
        c.start(priority=1)

    mem[...] = mem0_ref[...].astype(F32)

    x_head().wait()
    lnx[...] = _ln(xbuf[0:P0, :].astype(F32)).astype(BF16)
    for c in qkv_copies(1):
        c.start(priority=1)

    def prologue(p, carry):
        for c in qkv_copies(p):
            c.wait()

        wo_piece(p).start()
        x_piece(p).start()
        xp = lnx[...]
        for wi in range(3):
            s0 = wi * H + 2 * p
            a = wqkv[s0]
            b = wqkv[s0 + 1]
            c0 = (a & jnp.uint32(0xFFFF)) | (b << 16)
            c1 = (a >> 16) | (b & jnp.uint32(0xFFFF0000))
            wqkv[s0] = c0
            wqkv[s0 + 1] = c1
            ring[s0, 0:P0, :] = _dot(xp, _w(c0)).astype(BF16)
            ring[s0 + 1, 0:P0, :] = _dot(xp, _w(c1)).astype(BF16)

        for c in qkv_copies(p + 2):
            c.start(priority=1)
        return carry

    with jax.named_scope('ph1_prologue'):
        jax.lax.fori_loop(0, NPAIR, prologue, 0)

    for i in range(NPAIR):
        x_piece(i).wait()
        wo_piece(i).wait()
    for i in range(4):
        w_copy(i).start()

    LP = 2 * (SEG + M)
    row = jax.lax.broadcasted_iota(jnp.int32, (LP, LP), 0)
    col = jax.lax.broadcasted_iota(jnp.int32, (LP, LP), 1)

    def head_of(i):
        return jnp.where(i < 2 * SEG, i // SEG, (i - 2 * SEG) // M)

    same_head = head_of(row) == head_of(col)
    allowed = same_head & ((col >= 2 * SEG) | (row >= 2 * SEG)
                           | (col % SEG <= row % SEG))
    scale = E ** (-0.5)
    bias = jnp.where(allowed, 0.0,
                     jnp.where(same_head, NEG / scale, -jnp.inf)).astype(F32)
    exp_c = scale * 1.4426950408889634

    ring_u = ring.bitcast(U32)
    obuf_u = obuf.bitcast(U32)

    def rows16(ref_u, slot, start, n):
        if isinstance(start, int):
            r = pl.ds(start // 2, n // 2)
        else:
            r = pl.ds(pl.multiple_of(start // 2, 8), n // 2)
        return pltpu.bitcast(ref_u[slot, r, :], BF16)

    def step_tokens(s):
        t0 = pl.multiple_of(jnp.minimum(P0 + TPS * s, S - TPS), 8)
        return t0, _ln(xbuf[pl.ds(t0, TPS), :].astype(F32))

    def step(s, tok):
        _, tok_next = step_tokens(s + 1)
        t0 = pl.multiple_of(P0 + TPS * s, 8)
        xs = jnp.concatenate([mem[...], tok], axis=0).astype(BF16)
        wpos = [pl.multiple_of((t0 + 8 * g) % RING, 8) for g in range(3)]
        rpos = pl.multiple_of((SEG * s) % RING, SEG)
        opos = pl.multiple_of(SEG * s, SEG)
        ord_ = pl.multiple_of(s * TPS, 8)
        qkv = {}
        soft = {}
        lhs_o = {}
        NP = H // 2

        def do_proj(j, wi):
            toks, mems = [], []
            for h in (2 * j, 2 * j + 1):
                y = _dot(xs, _w(wqkv[wi * H + h]))
                for g in range(3):
                    ring[wi * H + h, pl.ds(wpos[g], 8), :] = (
                        y[8 + 8 * g:16 + 8 * g].astype(BF16))
                toks.append(rows16(ring_u, wi * H + h, rpos, SEG))
                mems.append(y[0:8])
            mpart = jnp.concatenate(mems, axis=0).astype(BF16)
            qkv.setdefault(j, []).append(
                jnp.concatenate(toks + [mpart], axis=0))

        def do_scores(j):
            q, k, _ = qkv[j]
            sc = jax.lax.dot_general(q, k, (((1,), (1,)), ((), ())),
                                     preferred_element_type=F32) + bias
            mx = jnp.max(sc, axis=-1, keepdims=True)
            pe = jnp.exp2((sc - mx) * exp_c)
            inv = _recip(jnp.sum(pe, axis=-1, keepdims=True))
            soft[j] = (pe.astype(BF16), inv)

        def do_pv(j):
            pe, inv = soft[j]
            o = _dot(pe, qkv[j][2]) * inv
            for i, h in enumerate((2 * j, 2 * j + 1)):
                obuf[h, pl.ds(opos, SEG), :] = (
                    o[i * SEG:(i + 1) * SEG].astype(BF16))
                oprev = obuf[h, pl.ds(ord_, TPS), :].astype(F32)
                om = o[2 * SEG + i * M:2 * SEG + (i + 1) * M]
                lhs_o[h] = jnp.concatenate([om, oprev], axis=0).astype(BF16)

        def do_wo(h0, h1):
            la = jnp.concatenate([lhs_o[h] for h in range(h0, h1)], axis=1)
            return _dot(la, _w(wo[h0 * E // 2:h1 * E // 2, :]))

        res = None
        for i in range(NP):
            for op in ORDER:
                if op in 'qkv':
                    do_proj(i, 'qkv'.index(op))
                elif op == 's' and i - LAG_S >= 0:
                    do_scores(i - LAG_S)
                elif op == 'p' and i - LAG_S - LAG_P >= 0:
                    do_pv(i - LAG_S - LAG_P)
                elif op == 'w' and i in MAIN_W:
                    r = do_wo(*MAIN_W[i])
                    res = r if res is None else res + r
        for kind, a, b in TAIL:
            if kind == 's':
                do_scores(a)
            elif kind == 'p':
                do_pv(a)
            else:
                res = res + do_wo(a, b)
        mem[...] = res[0:M]
        abuf[pl.ds(ord_, TPS), :] = res[M:]
        return tok_next

    with jax.named_scope('ph2_steps'):
        jax.lax.fori_loop(0, NSEG, step, step_tokens(0)[1], unroll=STEP_UNROLL)

    def wo_tail(j, carry):
        cs = pl.ds(pl.multiple_of(j * 128, 128), 128)
        lo_ = jnp.concatenate([rows16(obuf_u, h, OTAIL, S - OTAIL)
                               for h in range(H)], axis=1)
        abuf[OTAIL:S, cs] = _dot(lo_, _w(wo[:, cs]))
        return carry

    with jax.named_scope('ph3_wo'):
        jax.lax.fori_loop(0, D // 128, wo_tail, 0, unroll=2)

    for i in range(4):
        w_copy(i).wait()
    for p in range(NPAIR, NPAIR + 2):
        for c in qkv_copies(p):
            c.wait()

    h1buf[0:8, :] = jnp.zeros((8, D), F32)
    h1buf[S + 8:S + 16, :] = jnp.zeros((8, D), F32)

    def resid(r):
        return xbuf[r, :].astype(F32) + abuf[r, :]

    QC = CH // 4

    def pass1_input(q):
        r = pl.ds(pl.multiple_of(q * QC, QC), QC)
        return _ln(_ln(resid(r))).astype(BF16)

    def pass1(c, t):
        for j in range(4):
            q = 4 * c + j
            y = _dot(t, _w(w1[...]))
            t = pass1_input(jnp.minimum(q + 1, S // QC - 1))
            h1buf[pl.ds(pl.multiple_of(q * QC + 8, 8), QC), :] = _gelu(y)
        return t

    with jax.named_scope('ph3_pass1'):
        jax.lax.fori_loop(0, S // CH, pass1, pass1_input(0))

    def out_copy(c):
        r = pl.ds(pl.multiple_of(c * HC, HC), HC)
        return pltpu.make_async_copy(outbuf.at[r, :], out_hbm.at[r, :],
                                     sem_out.at[c])

    def shifted(c0):
        win = h1buf[pl.ds(pl.multiple_of(c0, 8), HC + 16), :]
        qd = D // 4
        return jnp.concatenate([
            win[7:7 + HC, 0 * qd:1 * qd],
            win[9:9 + HC, 1 * qd:2 * qd],
            win[6:6 + HC, 2 * qd:3 * qd],
            win[10:10 + HC, 3 * qd:4 * qd]], axis=1).astype(BF16)

    def pass2(c, carry):
        halves = (2 * c, 2 * c + 1)
        rows = [pl.ds(pl.multiple_of(i * HC, HC), HC) for i in halves]
        hs = [_dot(shifted(i * HC), _w(w2[...])) for i in halves]
        hh = [resid(r) for r in rows]
        x1 = [_ln(h) + d for h, d in zip(hh, hs)]
        u = [_gelu(_dot(_ln(v).astype(BF16), _w(w3[...]))).astype(BF16)
             for v in x1]
        for i in range(2):
            y = _dot(u[i], _w(w4[...]))
            outbuf[rows[i], :] = (hh[i] + (x1[i] + y)).astype(BF16)
            out_copy(halves[i]).start()
        return carry

    with jax.named_scope('ph3_pass2'):
        jax.lax.fori_loop(0, S // CH, pass2, 0)
    for c in range(S // HC):
        out_copy(c).wait()


@functools.partial(jax.jit, static_argnames=("A_seg_len",))
def pallas_sequential_preLN__memory_aug_recurrent_mem_tr__mixer_s_mlp__prompt_kernel(
    A_x: jax.Array,
    A_mem0: jax.Array,
    A_Wq: jax.Array,
    A_Wk: jax.Array,
    A_Wv: jax.Array,
    A_Wo: jax.Array,
    A_seg_len,
    B_x: jax.Array,
    B_w1: jax.Array,
    B_w2: jax.Array,
    B_w3: jax.Array,
    B_w4: jax.Array,
):
    assert A_seg_len == SEG and A_x.shape == (1, S, D)
    x = A_x.reshape(S, D)
    mem0 = A_mem0.reshape(M, D)
    wq = A_Wq.reshape(D // 2, 2, H, E)
    wk = A_Wk.reshape(D // 2, 2, H, E)
    wv = A_Wv.reshape(D // 2, 2, H, E)
    wo = A_Wo.reshape(H * E, D)

    hbm = pl.BlockSpec(memory_space=pl.ANY)
    vmem = pl.BlockSpec(memory_space=pltpu.VMEM)
    out = pl.pallas_call(
        _kernel,
        out_shape=jax.ShapeDtypeStruct((S, D), BF16),
        in_specs=[hbm, vmem] + [hbm] * 8,
        out_specs=hbm,
        scratch_shapes=[
            pltpu.VMEM((3 * H + 12, D // 2, E), U32),
            pltpu.VMEM((H * E // 2, D), U32),
            pltpu.VMEM((D // 2, D), U32),
            pltpu.VMEM((D // 2, D), U32),
            pltpu.VMEM((D // 2, FF), U32),
            pltpu.VMEM((FF // 2, D), U32),
            pltpu.VMEM((S, D), BF16),
            pltpu.VMEM((P0, D), BF16),
            pltpu.VMEM((3 * H, RING, E), BF16),
            pltpu.VMEM((H, S, E), BF16),
            pltpu.VMEM((S, D), F32),
            pltpu.VMEM((M, D), F32),
            pltpu.VMEM((S + 16, D), F32),
            pltpu.VMEM((S, D), BF16),
            pltpu.SemaphoreType.DMA((2,)),
            pltpu.SemaphoreType.DMA((H // 2 + 2,)),
            pltpu.SemaphoreType.DMA((1,)),
            pltpu.SemaphoreType.DMA((4,)),
            pltpu.SemaphoreType.DMA((S // HC,)),
        ],
        compiler_params=pltpu.CompilerParams(
            vmem_limit_bytes=126 * 1024 * 1024,
            disable_bounds_checks=True),
    )(x, mem0, wq, wk, wv, wo, B_w1, B_w2, B_w3, B_w4)
    return out.reshape(1, S, D)
```

```python
import functools

import jax
import jax.numpy as jnp
import jax.experimental.pallas as pl
import jax.experimental.pallas.tpu as pltpu

F32 = jnp.float32
BF16 = jnp.bfloat16
U32 = jnp.uint32

S = 2048
D = 1024
H = 32
E = 128
M = 8
SEG = 32
NSEG = S // SEG
FF = 3584
TPS = 24
P0 = S - TPS * NSEG
RING = 576
OTAIL = TPS * NSEG
CH = 256
HC = CH // 2
EPS = 1e-5
LAG_S = 1
LAG_P = 2
ORDER = 'qksvpw'
MAIN_W = {10: (0, 8), 14: (8, 12)}
TAIL = (('w', 12, 14), ('s', 15, 0), ('w', 14, 16), ('p', 13, 0), ('w', 16, 22),
        ('p', 14, 0), ('w', 22, 24), ('p', 15, 0), ('w', 24, 30), ('w', 30, 32))
NEG = -1000000000.0


def _ln(x):
    m = jnp.mean(x, axis=-1, keepdims=True)
    xc = x - m
    v = jnp.mean(xc * xc, axis=-1, keepdims=True)
    return xc * jax.lax.rsqrt(v + EPS)


def _recip(x):
    r = pl.reciprocal(x, approx=True)
    return r * (2.0 - x * r)


def _gelu(x):
    return jax.nn.gelu(x, approximate=True)


def _dot(a, b):
    return jnp.dot(a, b, preferred_element_type=F32)


def _w(u32_val):
    return pltpu.bitcast(u32_val, BF16)


def _kernel(x_hbm, mem0_ref, wq_hbm, wk_hbm, wv_hbm, wo_hbm, w1_hbm, w2_hbm,
            w3_hbm, w4_hbm, out_hbm,
            wqkv, wo, w1, w2, w3, w4, xbuf, lnx, ring, obuf, abuf, mem, h1buf,
            outbuf, sem_x, sem_qkv, sem_wo, sem_w, sem_out):
    NPAIR = H // 2
    XP = (S - P0) // NPAIR

    def x_head():
        return pltpu.make_async_copy(x_hbm.at[pl.ds(0, P0), :],
                                     xbuf.at[pl.ds(0, P0), :], sem_x.at[0])

    def x_piece(i):
        r = pl.ds(pl.multiple_of(P0 + i * XP, 8), XP)
        return pltpu.make_async_copy(x_hbm.at[r, :], xbuf.at[r, :], sem_x.at[1])

    def qkv_copies(p):
        real = p < NPAIR
        src_p = jnp.minimum(p, NPAIR - 1)
        cps = []
        for wi, w_hbm in enumerate((wq_hbm, wk_hbm, wv_hbm)):
            wu = w_hbm.bitcast(U32)
            for par in range(2):
                slot = jnp.where(real, wi * H + 2 * p + par,
                                 3 * H + (p - NPAIR) * 6 + 2 * wi + par)
                cps.append(pltpu.make_async_copy(
                    wu.at[:, par, src_p, :], wqkv.at[slot], sem_qkv.at[p]))
        return cps

    def w_copy(i):
        src, dst = ((w1_hbm, w1), (w2_hbm, w2), (w3_hbm, w3), (w4_hbm, w4))[i]
        return pltpu.make_async_copy(src.bitcast(U32), dst, sem_w.at[i])

    WO_ROWS = H * E // 2 // NPAIR

    def wo_piece(i):
        r = pl.ds(pl.multiple_of(i * WO_ROWS, WO_ROWS), WO_ROWS)
        return pltpu.make_async_copy(wo_hbm.bitcast(U32).at[r, :], wo.at[r, :],
                                     sem_wo.at[0])

    x_head().start()
    for c in qkv_copies(0):
        c.start(priority=1)

    mem[...] = mem0_ref[...].astype(F32)

    x_head().wait()
    lnx[...] = _ln(xbuf[0:P0, :].astype(F32)).astype(BF16)
    for c in qkv_copies(1):
        c.start(priority=1)

    def prologue(p, carry):
        for c in qkv_copies(p):
            c.wait()

        wo_piece(p).start()
        x_piece(p).start()
        xp = lnx[...]
        for wi in range(3):
            s0 = wi * H + 2 * p
            a = wqkv[s0]
            b = wqkv[s0 + 1]
            c0 = (a & jnp.uint32(0xFFFF)) | (b << 16)
            c1 = (a >> 16) | (b & jnp.uint32(0xFFFF0000))
            wqkv[s0] = c0
            wqkv[s0 + 1] = c1
            ring[s0, 0:P0, :] = _dot(xp, _w(c0)).astype(BF16)
            ring[s0 + 1, 0:P0, :] = _dot(xp, _w(c1)).astype(BF16)

        for c in qkv_copies(p + 2):
            c.start(priority=1)
        return carry

    with jax.named_scope('ph1_prologue'):
        jax.lax.fori_loop(0, NPAIR, prologue, 0)

    for i in range(NPAIR):
        x_piece(i).wait()
        wo_piece(i).wait()
    for i in range(4):
        w_copy(i).start()

    LP = 2 * (SEG + M)
    row = jax.lax.broadcasted_iota(jnp.int32, (LP, LP), 0)
    col = jax.lax.broadcasted_iota(jnp.int32, (LP, LP), 1)

    def head_of(i):
        return jnp.where(i < 2 * SEG, i // SEG, (i - 2 * SEG) // M)

    same_head = head_of(row) == head_of(col)
    allowed = same_head & ((col >= 2 * SEG) | (row >= 2 * SEG)
                           | (col % SEG <= row % SEG))
    scale = E ** (-0.5)
    bias = jnp.where(allowed, 0.0,
                     jnp.where(same_head, NEG / scale, -jnp.inf)).astype(F32)
    exp_c = scale * 1.4426950408889634

    ring_u = ring.bitcast(U32)
    obuf_u = obuf.bitcast(U32)


    def step_tokens(s):
        t0 = pl.multiple_of(jnp.minimum(P0 + TPS * s, S - TPS), 8)
        return t0, _ln(xbuf[pl.ds(t0, TPS), :].astype(F32))

    def step(k, par, tok):
        s = 2 * k + par
        _, tok_next = step_tokens(s + 1)
        t0 = pl.multiple_of(P0 + TPS * s, 8)
        xs = jnp.concatenate([mem[...], tok], axis=0).astype(BF16)
        wpos = [pl.multiple_of((t0 + 8 * g) % RING, 8) for g in range(3)]
        rbase = pl.multiple_of((SEG * k) % (RING // 2), SEG)
        opos = pl.multiple_of(SEG * s, SEG)
        ord_ = pl.multiple_of(s * TPS, 8)
        qkv = {}
        soft = {}
        lhs_o = {}
        NP = H // 2

        def do_proj(j, wi):
            toks, mems = [], []
            for h in (2 * j, 2 * j + 1):
                y = _dot(xs, _w(wqkv[wi * H + h]))
                for g in range(3):
                    ring[wi * H + h, pl.ds(wpos[g], 8), :] = (
                        y[8 + 8 * g:16 + 8 * g].astype(BF16))
                two_segs = ring_u.at[wi * H + h, pl.ds(rbase, SEG), :]
                toks.append(pltpu.bitcast(
                    two_segs[par * SEG // 2:(par + 1) * SEG // 2, :], BF16))
                mems.append(y[0:8])
            mpart = jnp.concatenate(mems, axis=0).astype(BF16)
            qkv.setdefault(j, []).append(
                jnp.concatenate(toks + [mpart], axis=0))

        def do_scores(j):
            q, k, _ = qkv[j]
            sc = jax.lax.dot_general(q, k, (((1,), (1,)), ((), ())),
                                     preferred_element_type=F32) + bias
            mx = jnp.max(sc, axis=-1, keepdims=True)
            pe = jnp.exp2((sc - mx) * exp_c)
            inv = _recip(jnp.sum(pe, axis=-1, keepdims=True))
            soft[j] = (pe.astype(BF16), inv)

        def do_pv(j):
            pe, inv = soft[j]
            o = _dot(pe, qkv[j][2]) * inv
            for i, h in enumerate((2 * j, 2 * j + 1)):
                obuf[h, pl.ds(opos, SEG), :] = (
                    o[i * SEG:(i + 1) * SEG].astype(BF16))
                oprev = obuf[h, pl.ds(ord_, TPS), :].astype(F32)
                om = o[2 * SEG + i * M:2 * SEG + (i + 1) * M]
                lhs_o[h] = jnp.concatenate([om, oprev], axis=0).astype(BF16)

        def do_wo(h0, h1):
            la = jnp.concatenate([lhs_o[h] for h in range(h0, h1)], axis=1)
            return _dot(la, _w(wo[h0 * E // 2:h1 * E // 2, :]))

        res = None
        for i in range(NP):
            for op in ORDER:
                if op in 'qkv':
                    do_proj(i, 'qkv'.index(op))
                elif op == 's' and i - LAG_S >= 0:
                    do_scores(i - LAG_S)
                elif op == 'p' and i - LAG_S - LAG_P >= 0:
                    do_pv(i - LAG_S - LAG_P)
                elif op == 'w' and i in MAIN_W:
                    r = do_wo(*MAIN_W[i])
                    res = r if res is None else res + r
        for kind, a, b in TAIL:
            if kind == 's':
                do_scores(a)
            elif kind == 'p':
                do_pv(a)
            else:
                res = res + do_wo(a, b)
        mem[...] = res[0:M]
        abuf[pl.ds(ord_, TPS), :] = res[M:]
        return tok_next

    def two_steps(k, tok):
        return step(k, 1, step(k, 0, tok))

    with jax.named_scope('ph2_steps'):
        jax.lax.fori_loop(0, NSEG // 2, two_steps, step_tokens(0)[1])

    def wo_tail(j, carry):
        cs = pl.ds(pl.multiple_of(j * 128, 128), 128)
        lo_ = jnp.concatenate(
            [pltpu.bitcast(obuf_u[h, OTAIL // 2:S // 2, :], BF16)
             for h in range(H)], axis=1)
        abuf[OTAIL:S, cs] = _dot(lo_, _w(wo[:, cs]))
        return carry

    with jax.named_scope('ph3_wo'):
        jax.lax.fori_loop(0, D // 128, wo_tail, 0, unroll=2)

    for i in range(4):
        w_copy(i).wait()
    for p in range(NPAIR, NPAIR + 2):
        for c in qkv_copies(p):
            c.wait()

    h1buf[0:8, :] = jnp.zeros((8, D), F32)
    h1buf[S + 8:S + 16, :] = jnp.zeros((8, D), F32)

    def resid(r):
        return xbuf[r, :].astype(F32) + abuf[r, :]

    QC = CH // 4

    def pass1_input(q):
        r = pl.ds(pl.multiple_of(q * QC, QC), QC)
        return _ln(_ln(resid(r))).astype(BF16)

    def pass1(c, t):
        for j in range(4):
            q = 4 * c + j
            y = _dot(t, _w(w1[...]))
            t = pass1_input(jnp.minimum(q + 1, S // QC - 1))
            h1buf[pl.ds(pl.multiple_of(q * QC + 8, 8), QC), :] = _gelu(y)
        return t

    with jax.named_scope('ph3_pass1'):
        jax.lax.fori_loop(0, S // CH, pass1, pass1_input(0))

    def out_copy(c):
        r = pl.ds(pl.multiple_of(c * HC, HC), HC)
        return pltpu.make_async_copy(outbuf.at[r, :], out_hbm.at[r, :],
                                     sem_out.at[c])

    def shifted(c0):
        win = h1buf[pl.ds(pl.multiple_of(c0, 8), HC + 16), :]
        qd = D // 4
        return jnp.concatenate([
            win[7:7 + HC, 0 * qd:1 * qd],
            win[9:9 + HC, 1 * qd:2 * qd],
            win[6:6 + HC, 2 * qd:3 * qd],
            win[10:10 + HC, 3 * qd:4 * qd]], axis=1).astype(BF16)

    def pass2(c, carry):
        halves = (2 * c, 2 * c + 1)
        rows = [pl.ds(pl.multiple_of(i * HC, HC), HC) for i in halves]
        hs = [_dot(shifted(i * HC), _w(w2[...])) for i in halves]
        hh = [resid(r) for r in rows]
        x1 = [_ln(h) + d for h, d in zip(hh, hs)]
        u = [_gelu(_dot(_ln(v).astype(BF16), _w(w3[...]))).astype(BF16)
             for v in x1]
        for i in range(2):
            y = _dot(u[i], _w(w4[...]))
            outbuf[rows[i], :] = (hh[i] + (x1[i] + y)).astype(BF16)
            out_copy(halves[i]).start()
        return carry

    with jax.named_scope('ph3_pass2'):
        jax.lax.fori_loop(0, S // CH, pass2, 0)
    for c in range(S // HC):
        out_copy(c).wait()


@functools.partial(jax.jit, static_argnames=("A_seg_len",))
def pallas_sequential_preLN__memory_aug_recurrent_mem_tr__mixer_s_mlp__prompt_kernel(
    A_x: jax.Array,
    A_mem0: jax.Array,
    A_Wq: jax.Array,
    A_Wk: jax.Array,
    A_Wv: jax.Array,
    A_Wo: jax.Array,
    A_seg_len,
    B_x: jax.Array,
    B_w1: jax.Array,
    B_w2: jax.Array,
    B_w3: jax.Array,
    B_w4: jax.Array,
):
    assert A_seg_len == SEG and A_x.shape == (1, S, D)
    x = A_x.reshape(S, D)
    mem0 = A_mem0.reshape(M, D)
    wq = A_Wq.reshape(D // 2, 2, H, E)
    wk = A_Wk.reshape(D // 2, 2, H, E)
    wv = A_Wv.reshape(D // 2, 2, H, E)
    wo = A_Wo.reshape(H * E, D)

    hbm = pl.BlockSpec(memory_space=pl.ANY)
    vmem = pl.BlockSpec(memory_space=pltpu.VMEM)
    out = pl.pallas_call(
        _kernel,
        out_shape=jax.ShapeDtypeStruct((S, D), BF16),
        in_specs=[hbm, vmem] + [hbm] * 8,
        out_specs=hbm,
        scratch_shapes=[
            pltpu.VMEM((3 * H + 12, D // 2, E), U32),
            pltpu.VMEM((H * E // 2, D), U32),
            pltpu.VMEM((D // 2, D), U32),
            pltpu.VMEM((D // 2, D), U32),
            pltpu.VMEM((D // 2, FF), U32),
            pltpu.VMEM((FF // 2, D), U32),
            pltpu.VMEM((S, D), BF16),
            pltpu.VMEM((P0, D), BF16),
            pltpu.VMEM((3 * H, RING, E), BF16),
            pltpu.VMEM((H, S, E), BF16),
            pltpu.VMEM((S, D), F32),
            pltpu.VMEM((M, D), F32),
            pltpu.VMEM((S + 16, D), F32),
            pltpu.VMEM((S, D), BF16),
            pltpu.SemaphoreType.DMA((2,)),
            pltpu.SemaphoreType.DMA((H // 2 + 2,)),
            pltpu.SemaphoreType.DMA((1,)),
            pltpu.SemaphoreType.DMA((4,)),
            pltpu.SemaphoreType.DMA((S // HC,)),
        ],
        compiler_params=pltpu.CompilerParams(
            vmem_limit_bytes=126 * 1024 * 1024,
            disable_bounds_checks=True),
    )(x, mem0, wq, wk, wv, wo, B_w1, B_w2, B_w3, B_w4)
    return out.reshape(1, S, D)
```

```python
import functools

import jax
import jax.numpy as jnp
import jax.experimental.pallas as pl
import jax.experimental.pallas.tpu as pltpu

F32 = jnp.float32
BF16 = jnp.bfloat16
U32 = jnp.uint32

S = 2048
D = 1024
H = 32
E = 128
M = 8
SEG = 32
NSEG = S // SEG
FF = 3584
TPS = 24
P0 = S - TPS * NSEG
RING = 576
OTAIL = TPS * NSEG
CH = 256
HC = CH // 2
EPS = 1e-5
LAG_S = 1
LAG_P = 2
ORDER = 'qksvpw'
MAIN_W = {10: (0, 8), 14: (8, 12)}
TAIL = (('w', 12, 14), ('s', 15, 0), ('w', 14, 16), ('p', 13, 0), ('w', 16, 20),
        ('p', 14, 0), ('w', 20, 24), ('p', 15, 0), ('w', 24, 30), ('w', 30, 32))
NEG = -1000000000.0


def _ln(x):
    m = jnp.mean(x, axis=-1, keepdims=True)
    xc = x - m
    v = jnp.mean(xc * xc, axis=-1, keepdims=True)
    return xc * jax.lax.rsqrt(v + EPS)


def _recip(x):
    r = pl.reciprocal(x, approx=True)
    return r * (2.0 - x * r)


def _gelu(x):
    return jax.nn.gelu(x, approximate=True)


def _dot(a, b):
    return jnp.dot(a, b, preferred_element_type=F32)


def _w(u32_val):
    return pltpu.bitcast(u32_val, BF16)


def _kernel(x_hbm, mem0_hbm, wq_hbm, wk_hbm, wv_hbm, wo_hbm, w1_hbm, w2_hbm,
            w3_hbm, w4_hbm, out_hbm,
            wqkv, wo, w1, w2, w3, w4, xbuf, lnx, ring, obuf, abuf, mem, h1buf,
            outbuf, mem0buf, sem_x, sem_qkv, sem_wo, sem_w, sem_out):
    NPAIR = H // 2
    XP = (S - P0) // NPAIR

    def x_head():
        return pltpu.make_async_copy(x_hbm.at[pl.ds(0, P0), :],
                                     xbuf.at[pl.ds(0, P0), :], sem_x.at[0])

    def x_piece(i):
        r = pl.ds(pl.multiple_of(P0 + i * XP, 8), XP)
        return pltpu.make_async_copy(x_hbm.at[r, :], xbuf.at[r, :], sem_x.at[1])

    def qkv_copies(p):
        real = p < NPAIR
        src_p = jnp.minimum(p, NPAIR - 1)
        cps = []
        for wi, w_hbm in enumerate((wq_hbm, wk_hbm, wv_hbm)):
            wu = w_hbm.bitcast(U32)
            for par in range(2):
                slot = jnp.where(real, wi * H + 2 * p + par,
                                 3 * H + (p - NPAIR) * 6 + 2 * wi + par)
                cps.append(pltpu.make_async_copy(
                    wu.at[:, par, src_p, :], wqkv.at[slot], sem_qkv.at[p]))
        return cps

    def w_copy(i):
        src, dst = ((w1_hbm, w1), (w2_hbm, w2), (w3_hbm, w3), (w4_hbm, w4))[i]
        return pltpu.make_async_copy(src.bitcast(U32), dst, sem_w.at[i])

    WO_ROWS = H * E // 2 // NPAIR

    def wo_piece(i):
        r = pl.ds(pl.multiple_of(i * WO_ROWS, WO_ROWS), WO_ROWS)
        return pltpu.make_async_copy(wo_hbm.bitcast(U32).at[r, :], wo.at[r, :],
                                     sem_wo.at[0])

    x_head().start()
    for c in qkv_copies(0):
        c.start(priority=1)

    mem0_copy = pltpu.make_async_copy(mem0_hbm, mem0buf, sem_x.at[2])
    mem0_copy.start()

    x_head().wait()
    lnx[...] = _ln(xbuf[0:P0, :].astype(F32)).astype(BF16)
    for c in qkv_copies(1):
        c.start(priority=1)

    def prologue(p, carry):
        for c in qkv_copies(p):
            c.wait()

        wo_piece(p).start()
        x_piece(p).start()
        xp = lnx[...]
        for wi in range(3):
            s0 = wi * H + 2 * p
            a = wqkv[s0]
            b = wqkv[s0 + 1]
            c0 = (a & jnp.uint32(0xFFFF)) | (b << 16)
            c1 = (a >> 16) | (b & jnp.uint32(0xFFFF0000))
            wqkv[s0] = c0
            wqkv[s0 + 1] = c1
            ring[s0, 0:P0, :] = _dot(xp, _w(c0)).astype(BF16)
            ring[s0 + 1, 0:P0, :] = _dot(xp, _w(c1)).astype(BF16)

        for c in qkv_copies(p + 2):
            c.start(priority=1)
        return carry

    with jax.named_scope('ph1_prologue'):
        jax.lax.fori_loop(0, NPAIR, prologue, 0)

    mem0_copy.wait()
    mem[...] = mem0buf[...].astype(F32)
    for i in range(NPAIR):
        x_piece(i).wait()
        wo_piece(i).wait()
    for i in range(4):
        w_copy(i).start()

    LP = 2 * (SEG + M)
    row = jax.lax.broadcasted_iota(jnp.int32, (LP, LP), 0)
    col = jax.lax.broadcasted_iota(jnp.int32, (LP, LP), 1)

    def head_of(i):
        return jnp.where(i < 2 * SEG, i // SEG, (i - 2 * SEG) // M)

    same_head = head_of(row) == head_of(col)
    allowed = same_head & ((col >= 2 * SEG) | (row >= 2 * SEG)
                           | (col % SEG <= row % SEG))
    scale = E ** (-0.5)
    bias = jnp.where(allowed, 0.0,
                     jnp.where(same_head, NEG / scale, -jnp.inf)).astype(F32)
    exp_c = scale * 1.4426950408889634

    ring_u = ring.bitcast(U32)
    obuf_u = obuf.bitcast(U32)


    def step_tokens(s):
        t0 = pl.multiple_of(jnp.minimum(P0 + TPS * s, S - TPS), 8)
        return t0, _ln(xbuf[pl.ds(t0, TPS), :].astype(F32))

    def step(k, par, tok):
        s = 2 * k + par
        _, tok_next = step_tokens(s + 1)
        t0 = pl.multiple_of(P0 + TPS * s, 8)
        xs = jnp.concatenate([mem[...], tok], axis=0).astype(BF16)
        wpos = [pl.multiple_of((t0 + 8 * g) % RING, 8) for g in range(3)]
        rbase = pl.multiple_of((SEG * k) % (RING // 2), SEG)
        opos = pl.multiple_of(SEG * s, SEG)
        ord_ = pl.multiple_of(s * TPS, 8)
        qkv = {}
        soft = {}
        lhs_o = {}
        NP = H // 2

        def do_proj(j, wi):
            toks, mems = [], []
            for h in (2 * j, 2 * j + 1):
                y = _dot(xs, _w(wqkv[wi * H + h]))
                for g in range(3):
                    ring[wi * H + h, pl.ds(wpos[g], 8), :] = (
                        y[8 + 8 * g:16 + 8 * g].astype(BF16))
                two_segs = ring_u.at[wi * H + h, pl.ds(rbase, SEG), :]
                toks.append(pltpu.bitcast(
                    two_segs[par * SEG // 2:(par + 1) * SEG // 2, :], BF16))
                mems.append(y[0:8])
            mpart = jnp.concatenate(mems, axis=0).astype(BF16)
            qkv.setdefault(j, []).append(
                jnp.concatenate(toks + [mpart], axis=0))

        def do_scores(j):
            q, k, _ = qkv[j]
            sc = jax.lax.dot_general(q, k, (((1,), (1,)), ((), ())),
                                     preferred_element_type=F32) + bias
            mx = jnp.max(sc, axis=-1, keepdims=True)
            pe = jnp.exp2((sc - mx) * exp_c)
            inv = _recip(jnp.sum(pe, axis=-1, keepdims=True))
            soft[j] = (pe.astype(BF16), inv)

        def do_pv(j):
            pe, inv = soft[j]
            o = _dot(pe, qkv[j][2]) * inv
            for i, h in enumerate((2 * j, 2 * j + 1)):
                obuf[h, pl.ds(opos, SEG), :] = (
                    o[i * SEG:(i + 1) * SEG].astype(BF16))
                oprev = obuf[h, pl.ds(ord_, TPS), :].astype(F32)
                om = o[2 * SEG + i * M:2 * SEG + (i + 1) * M]
                lhs_o[h] = jnp.concatenate([om, oprev], axis=0).astype(BF16)

        def do_wo(h0, h1):
            la = jnp.concatenate([lhs_o[h] for h in range(h0, h1)], axis=1)
            return _dot(la, _w(wo[h0 * E // 2:h1 * E // 2, :]))

        res = None
        for i in range(NP):
            for op in ORDER:
                if op in 'qkv':
                    do_proj(i, 'qkv'.index(op))
                elif op == 's' and i - LAG_S >= 0:
                    do_scores(i - LAG_S)
                elif op == 'p' and i - LAG_S - LAG_P >= 0:
                    do_pv(i - LAG_S - LAG_P)
                elif op == 'w' and i in MAIN_W:
                    r = do_wo(*MAIN_W[i])
                    res = r if res is None else res + r
        for kind, a, b in TAIL:
            if kind == 's':
                do_scores(a)
            elif kind == 'p':
                do_pv(a)
            else:
                res = res + do_wo(a, b)
        mem[...] = res[0:M]
        abuf[pl.ds(ord_, TPS), :] = res[M:]
        return tok_next

    def two_steps(k, tok):
        return step(k, 1, step(k, 0, tok))

    with jax.named_scope('ph2_steps'):
        jax.lax.fori_loop(0, NSEG // 2, two_steps, step_tokens(0)[1])

    def wo_tail(j, carry):
        cs = pl.ds(pl.multiple_of(j * 128, 128), 128)
        lo_ = jnp.concatenate(
            [pltpu.bitcast(obuf_u[h, OTAIL // 2:S // 2, :], BF16)
             for h in range(H)], axis=1)
        abuf[OTAIL:S, cs] = _dot(lo_, _w(wo[:, cs]))
        return carry

    with jax.named_scope('ph3_wo'):
        jax.lax.fori_loop(0, D // 128, wo_tail, 0, unroll=2)

    for i in range(4):
        w_copy(i).wait()
    for p in range(NPAIR, NPAIR + 2):
        for c in qkv_copies(p):
            c.wait()

    h1buf[0:8, :] = jnp.zeros((8, D), F32)
    h1buf[S + 8:S + 16, :] = jnp.zeros((8, D), F32)

    def resid(r):
        return xbuf[r, :].astype(F32) + abuf[r, :]

    QC = CH // 4

    def pass1_input(q):
        r = pl.ds(pl.multiple_of(q * QC, QC), QC)
        return _ln(_ln(resid(r))).astype(BF16)

    def pass1(c, t):
        for j in range(4):
            q = 4 * c + j
            y = _dot(t, _w(w1[...]))
            t = pass1_input(jnp.minimum(q + 1, S // QC - 1))
            h1buf[pl.ds(pl.multiple_of(q * QC + 8, 8), QC), :] = _gelu(y)
        return t

    with jax.named_scope('ph3_pass1'):
        jax.lax.fori_loop(0, S // CH, pass1, pass1_input(0))

    def out_copy(c):
        r = pl.ds(pl.multiple_of(c * HC, HC), HC)
        return pltpu.make_async_copy(outbuf.at[r, :], out_hbm.at[r, :],
                                     sem_out.at[c])

    def shifted(c0):
        win = h1buf[pl.ds(pl.multiple_of(c0, 8), HC + 16), :]
        qd = D // 4
        return jnp.concatenate([
            win[7:7 + HC, 0 * qd:1 * qd],
            win[9:9 + HC, 1 * qd:2 * qd],
            win[6:6 + HC, 2 * qd:3 * qd],
            win[10:10 + HC, 3 * qd:4 * qd]], axis=1).astype(BF16)

    def pass2(c, carry):
        halves = (2 * c, 2 * c + 1)
        rows = [pl.ds(pl.multiple_of(i * HC, HC), HC) for i in halves]
        hs = [_dot(shifted(i * HC), _w(w2[...])) for i in halves]
        hh = [resid(r) for r in rows]
        x1 = [_ln(h) + d for h, d in zip(hh, hs)]
        u = [_gelu(_dot(_ln(v).astype(BF16), _w(w3[...]))).astype(BF16)
             for v in x1]
        for i in range(2):
            y = _dot(u[i], _w(w4[...]))
            outbuf[rows[i], :] = (hh[i] + (x1[i] + y)).astype(BF16)
            out_copy(halves[i]).start()
        return carry

    with jax.named_scope('ph3_pass2'):
        jax.lax.fori_loop(0, S // CH, pass2, 0)
    for c in range(S // HC):
        out_copy(c).wait()


@functools.partial(jax.jit, static_argnames=("A_seg_len",))
def pallas_sequential_preLN__memory_aug_recurrent_mem_tr__mixer_s_mlp__prompt_kernel(
    A_x: jax.Array,
    A_mem0: jax.Array,
    A_Wq: jax.Array,
    A_Wk: jax.Array,
    A_Wv: jax.Array,
    A_Wo: jax.Array,
    A_seg_len,
    B_x: jax.Array,
    B_w1: jax.Array,
    B_w2: jax.Array,
    B_w3: jax.Array,
    B_w4: jax.Array,
):
    assert A_seg_len == SEG and A_x.shape == (1, S, D)
    x = A_x.reshape(S, D)
    mem0 = A_mem0.reshape(M, D)
    wq = A_Wq.reshape(D // 2, 2, H, E)
    wk = A_Wk.reshape(D // 2, 2, H, E)
    wv = A_Wv.reshape(D // 2, 2, H, E)
    wo = A_Wo.reshape(H * E, D)

    hbm = pl.BlockSpec(memory_space=pl.ANY)
    out = pl.pallas_call(
        _kernel,
        out_shape=jax.ShapeDtypeStruct((S, D), BF16),
        in_specs=[hbm] * 10,
        out_specs=hbm,
        scratch_shapes=[
            pltpu.VMEM((3 * H + 12, D // 2, E), U32),
            pltpu.VMEM((H * E // 2, D), U32),
            pltpu.VMEM((D // 2, D), U32),
            pltpu.VMEM((D // 2, D), U32),
            pltpu.VMEM((D // 2, FF), U32),
            pltpu.VMEM((FF // 2, D), U32),
            pltpu.VMEM((S, D), BF16),
            pltpu.VMEM((P0, D), BF16),
            pltpu.VMEM((3 * H, RING, E), BF16),
            pltpu.VMEM((H, S, E), BF16),
            pltpu.VMEM((S, D), F32),
            pltpu.VMEM((M, D), F32),
            pltpu.VMEM((S + 16, D), F32),
            pltpu.VMEM((S, D), BF16),
            pltpu.VMEM((M, D), BF16),
            pltpu.SemaphoreType.DMA((3,)),
            pltpu.SemaphoreType.DMA((H // 2 + 2,)),
            pltpu.SemaphoreType.DMA((1,)),
            pltpu.SemaphoreType.DMA((4,)),
            pltpu.SemaphoreType.DMA((S // HC,)),
        ],
        compiler_params=pltpu.CompilerParams(
            vmem_limit_bytes=126 * 1024 * 1024,
            disable_bounds_checks=True),
    )(x, mem0, wq, wk, wv, wo, B_w1, B_w2, B_w3, B_w4)
    return out.reshape(1, S, D)
```
